```python
import jax
import jax.numpy as jnp

def _softmax(x, axis=-1):
    return jax.nn.softmax(x, axis=axis)

def _gelu(x):
    return jax.nn.gelu(x, approximate=True)

def _silu(x):
    return jax.nn.silu(x)

def _sigmoid(x):
    return jax.nn.sigmoid(x)

def _layernorm(x, axis=-1, eps=1e-05):
    m = jnp.mean(x, axis=axis, keepdims=True)
    v = jnp.var(x, axis=axis, keepdims=True)
    return (x - m) / jnp.sqrt(v + eps)

def _scatter_add(tgt, idx, src, axis=0):
    return tgt.at[idx].add(src)

def _segment_sum(src, seg, n):
    return jax.ops.segment_sum(src, seg, n)

class _Rng:

    def __init__(self, key):
        self._k = key

    def _next(self):
        self._k, sub = jax.random.split(self._k)
        return sub

    def normal(self, shape):
        return jax.random.normal(self._next(), shape, dtype=jnp.bfloat16)

    def randint(self, lo, hi, shape):
        return jax.random.randint(self._next(), shape, lo, hi, dtype=jnp.int32)

    def uniform(self, shape, lo=0.0, hi=1.0):
        return jax.random.uniform(self._next(), shape, jnp.bfloat16, lo, hi)

    def permutation(self, n):
        return jax.random.permutation(self._next(), n)
kernel_name = 'concat_heads__memory_aug_recurrent_mem_tr__ssm_conv_h3__prompt'

def setup_inputs():
    _rng = _Rng(jax.random.key(int.from_bytes(__import__("os").urandom(4), "little")))
    _w = lambda a: (lambda t: t.astype(jnp.bfloat16) if jnp.issubdtype(t.dtype, jnp.floating) else t)(jnp.asarray(a))

    def _A_setup():
        B, S, Dm = (1, 2048, 1024)
        H, Dh = (32, 128)
        M, seg = (8, 32)
        seg = min(seg, S)
        S = S // seg * seg
        return {'x': _w((lambda *s: _rng.normal(s) * 0.05)(B, S, Dm)), 'mem0': _w((lambda *s: _rng.normal(s) * 0.05)(B, M, Dm)), 'Wq': _w((lambda *s: _rng.normal(s) * 0.05)(Dm, H, Dh) * Dm ** (-0.5)), 'Wk': _w((lambda *s: _rng.normal(s) * 0.05)(Dm, H, Dh) * Dm ** (-0.5)), 'Wv': _w((lambda *s: _rng.normal(s) * 0.05)(Dm, H, Dh) * Dm ** (-0.5)), 'Wo': _w((lambda *s: _rng.normal(s) * 0.05)(H, Dh, Dm) * (H * Dh) ** (-0.5)), 'seg_len': seg}
    _A_in = _A_setup()

    def _B_setup():
        B, S, D = (1, 2048, 1024)
        ks = 4
        return {'q': _w((lambda *s: _rng.normal(s) * 0.05)(B, S, D)), 'k': _w((lambda *s: _rng.normal(s) * 0.05)(B, S, D)), 'v': _w((lambda *s: _rng.normal(s) * 0.05)(B, S, D)), 'shift_k': _w((lambda *s: _rng.normal(s) * 0.05)(D, ks) * 0.5), 'ssm_k': _w((lambda *s: _rng.normal(s) * 0.05)(D, S) * (1.0 / S ** 0.5)), 'ssm_D': _w((lambda *s: _rng.normal(s) * 0.05)(D))}
    _B_in = _B_setup()
    return {'A_x': _A_in['x'], 'A_mem0': _A_in['mem0'], 'A_Wq': _A_in['Wq'], 'A_Wk': _A_in['Wk'], 'A_Wv': _A_in['Wv'], 'A_Wo': _A_in['Wo'], 'A_seg_len': _A_in['seg_len'], 'B_q': _B_in['q'], 'B_k': _B_in['k'], 'B_v': _B_in['v'], 'B_shift_k': _B_in['shift_k'], 'B_ssm_k': _B_in['ssm_k'], 'B_ssm_D': _B_in['ssm_D']}

def reference(A_x, A_mem0, A_Wq, A_Wk, A_Wv, A_Wo, A_seg_len, B_q, B_k, B_v, B_shift_k, B_ssm_k, B_ssm_D):

    def _A_ref(x, mem0, Wq, Wk, Wv, Wo, seg_len):
        B, S, Dm = x.shape
        H, Dh = (Wq.shape[1], Wq.shape[2])
        M = mem0.shape[1]
        scale = Dh ** (-0.5)
        n_seg = S // seg_len
        L = M + seg_len
        idx = jnp.arange(L)
        mask = (idx[:, None] < M) | (idx[:, None] >= idx[None, :])
        mem = mem0
        outs = []
        for s in range(n_seg):
            xs = x[:, s * seg_len:(s + 1) * seg_len, :].copy()
            h = jnp.concatenate([mem, xs], axis=1)
            q = jnp.einsum('btd,dhe->bhte', h, Wq)
            k = jnp.einsum('btd,dhe->bhte', h, Wk)
            v = jnp.einsum('btd,dhe->bhte', h, Wv)
            scores = jnp.einsum('bhqe,bhke->bhqk', q, k) * scale
            scores = jnp.where(mask[None, None], scores, -1000000000.0)
            p = _softmax(scores, axis=-1)
            o = jnp.einsum('bhqk,bhke->bhqe', p, v)
            o = jnp.einsum('bhte,hed->btd', o, Wo)
            mem = o[:, :M, :].copy()
            outs.append(o[:, M:, :])
        return jnp.concatenate(outs, axis=1)

    def _B_ref(q, k, v, shift_k, ssm_k, ssm_D):
        B, S, D = q.shape
        ks = shift_k.shape[-1]
        k_pad = jnp.pad(k, ((0, 0), (ks - 1, 0), (0, 0)))
        k_shift = jnp.zeros_like(k)
        for t in range(ks):
            k_shift = k_shift + k_pad[:, t:t + S, :] * shift_k[:, ks - 1 - t][None, None, :]
        kv = k_shift * v
        L = 2 * S
        kv_pad = jnp.pad(kv, ((0, 0), (0, S), (0, 0)))
        kf_pad = jnp.pad(ssm_k, ((0, 0), (0, S)))
        kv_f = (lambda x, axes=(-2, -1): jnp.fft.rfft2(x.astype(jnp.float32), axes=axes))(kv_pad[:, None, :, :], axes=(1, 2))
        kf_f = (lambda x, axes=(-2, -1): jnp.fft.rfft2(x.astype(jnp.float32), axes=axes))(kf_pad[:, None, :], axes=(1, 2))
        kf_f = (lambda x, *d: x.transpose(*d))(kf_f, 1, 2, 0)
        y_f = kv_f * kf_f[None, :, :, :]
        y = (lambda x, s, axes=(-2, -1): jnp.fft.irfft2(x, s=s, axes=axes).astype(jnp.bfloat16))(y_f, (1, L), axes=(1, 2))[:, 0, :S, :]
        y = y + kv * ssm_D[None, None, :]
        return q * y
    a = _A_ref(A_x, A_mem0, A_Wq, A_Wk, A_Wv, A_Wo, A_seg_len)
    b = _B_ref(B_q, B_k, B_v, B_shift_k, B_ssm_k, B_ssm_D)
    return jnp.concatenate([a, b], axis=-1)
```

```python
import math

import jax
import jax.numpy as jnp
import numpy as np
from jax.experimental import pallas as pl
from jax.experimental.pallas import tpu as pltpu

F32 = jnp.float32
BF16 = jnp.bfloat16
U32 = jnp.uint32

N1, N2 = 32, 64
SEQ = N1 * N2
SX = N2 + 4
SZ = N2 + 4
ST = 2 * N2 + 4
CB = 128


def _dft_tables():
    theta = np.pi / (2 * SEQ)
    k1 = np.arange(N1)[:, None]
    n1 = np.arange(N1)[None, :]
    fwd = np.zeros((N2, 2 * N1, 128), np.float64)
    inv = np.zeros((N2, N1, 128), np.float64)
    for n2 in range(N2):
        ph = theta * (4 * k1 + 1) * (N2 * n1 + n2)
        fwd[n2, :N1, :N1] = np.cos(ph)
        fwd[n2, N1:, :N1] = np.sin(ph)
        inv[n2, :, :N1] = np.cos(ph).T / SEQ
        inv[n2, :, N1:2 * N1] = np.sin(ph).T / SEQ
    k2 = np.arange(N2)[:, None]
    n2 = np.arange(N2)[None, :]
    ph = 2 * np.pi * k2 * n2 / N2
    c, s = np.cos(ph), np.sin(ph)
    f2 = np.block([[c, -s], [s, c]])
    g2 = np.block([[c.T, s.T], [-s.T, c.T]])
    as_bf16 = lambda a: a.astype(np.float32).astype(BF16)
    return as_bf16(fwd), as_bf16(inv), as_bf16(np.stack([f2, g2]))


def _dot(a, b):
    return jnp.dot(a, b, preferred_element_type=F32)


def _dot_nt(a, b):
    return jax.lax.dot_general(a, b, (((1,), (1,)), ((), ())), preferred_element_type=F32)


def _make_kernel(n_heads, d_head, d_model, n_mem, seg, n_seg):
    n_rows = n_mem + seg
    n_cb = d_model // CB
    n_hp = n_heads // 2
    scale = d_head ** (-0.5)
    exp_scale = scale * math.log2(math.e)
    x_chunks = 8
    x_rows = SEQ // x_chunks
    steps_per_chunk = x_rows // seg

    def kernel(sh_ref, d_ref, mem_ref,
               x_hbm, wq_hbm, wk_hbm, wv_hbm, wo_hbm,
               q_hbm, k_hbm, v_hbm, h_hbm, tf_hbm, ti_hbm, t2_hbm,
               out_hbm,
               hs, ks, vs, qs, ob, kf, xs, ht, zx, zh, tt, yp, tf, ti, t2, sh32, d32,
               stage, wqkv, wo, xin, oa, hbuf, qbuf, kbuf, vbuf, obuf,
               sem_b, sem_t, sem_w, sem_o, sem_x, sem_ob, sem_oa):

        def b_copies(cb):
            c0 = cb * CB if isinstance(cb, int) else pl.multiple_of(cb * CB, CB)
            return [
                pltpu.make_async_copy(h_hbm.at[pl.ds(c0, CB), :], hs.at[cb], sem_b.at[0, cb]),
                pltpu.make_async_copy(k_hbm.at[:, pl.ds(c0, CB)], ks.at[cb], sem_b.at[1, cb]),
                pltpu.make_async_copy(v_hbm.at[:, pl.ds(c0, CB)], vs.at[cb], sem_b.at[2, cb]),
                pltpu.make_async_copy(q_hbm.at[:, pl.ds(c0, CB)], qs.at[cb], sem_b.at[3, cb]),
            ]

        def t_copies():
            return [pltpu.make_async_copy(tf_hbm, tf, sem_t.at[0]),
                    pltpu.make_async_copy(ti_hbm, ti, sem_t.at[1]),
                    pltpu.make_async_copy(t2_hbm, t2, sem_t.at[2])]

        def w_copies(m):
            w32 = (wq_hbm, wk_hbm, wv_hbm)[m].bitcast(U32)
            return [pltpu.make_async_copy(w32.at[:, hp, :], stage.at[m * n_hp + hp], sem_w.at[m])
                    for hp in range(n_hp)]

        def o_copies():
            wo32 = wo_hbm.bitcast(U32)
            return [pltpu.make_async_copy(wo32.at[:, pl.ds(j * 128, 128)], wo.at[j], sem_o)
                    for j in range(d_model // 128)]

        def x_copy(c):
            return pltpu.make_async_copy(x_hbm.at[pl.ds(c * x_rows, x_rows), :],
                                         xin.at[pl.ds(c * x_rows, x_rows), :], sem_x.at[c])

        def ob_copy(cb):
            c0 = cb * CB if isinstance(cb, int) else pl.multiple_of(cb * CB, CB)
            return pltpu.make_async_copy(ob.at[cb], out_hbm.at[:, pl.ds(d_model + c0, CB)], sem_ob)

        def oa_copy(s):
            r0 = s * seg if isinstance(s, int) else pl.multiple_of(s * seg, seg)
            return pltpu.make_async_copy(oa.at[pl.ds(r0, seg), :],
                                         out_hbm.at[pl.ds(r0, seg), pl.ds(0, d_model)], sem_oa)

        for c in b_copies(0):
            c.start()
        for c in t_copies():
            c.start()
        for cb in range(1, n_cb):
            for c in b_copies(cb):
                c.start()
        for m in range(3):
            for c in w_copies(m):
                c.start()
        x_copy(0).start()
        for c in o_copies():
            c.start()
        for c in range(1, x_chunks):
            x_copy(c).start()

        kf[0:8, :] = jnp.zeros((8, CB), F32)
        sh32[...] = sh_ref[...].astype(F32)
        d32[...] = d_ref[...].astype(F32)
        hbuf[0:n_mem, :] = mem_ref[...].astype(F32)
        eye = (jax.lax.broadcasted_iota(jnp.int32, (128, 128), 0)
               == jax.lax.broadcasted_iota(jnp.int32, (128, 128), 1)).astype(BF16)

        group = 4

        def load_z(z, k1):
            return jnp.concatenate([z[pl.ds(k1, N2, stride=SZ), :],
                                    z[pl.ds(N1 + k1, N2, stride=SZ), :]], axis=0).astype(BF16)

        def b_block(cb, carry):
            c0 = pl.multiple_of(cb * CB, CB)
            for c in b_copies(cb):
                c.wait()
            for j in range(SEQ // 128):
                r = _dot_nt(eye, hs[cb, :, j * 128:(j + 1) * 128])
                ht[pl.ds((2 * j) * SX, N2), :] = r[0:N2]
                ht[pl.ds((2 * j + 1) * SX, N2), :] = r[N2:2 * N2]
            kf[8:8 + SEQ, :] = ks[cb].astype(F32)
            taps = sh32[:, pl.ds(c0, CB)]
            for n1 in range(N1):
                acc = kf[pl.ds(8 + n1 * N2, N2), :] * taps[0:1]
                for i in range(1, 4):
                    acc = acc + kf[pl.ds(8 - i + n1 * N2, N2), :] * taps[i:i + 1]
                xs[pl.ds(n1 * SX, N2), :] = acc * vs[cb, pl.ds(n1 * N2, N2), :].astype(F32)
            for n2 in range(N2):
                a = tf[n2, :, 0:N1]
                zx[pl.ds(n2 * SZ, 2 * N1), :] = _dot(a, xs[pl.ds(n2, N1, stride=SX), :].astype(BF16))
                zh[pl.ds(n2 * SZ, 2 * N1), :] = _dot(a, ht[pl.ds(n2, N1, stride=SX), :].astype(BF16))
            f2 = t2[0]
            g2 = t2[1]

            def stage2(g):
                zz = []
                for k1 in range(g * group, (g + 1) * group):
                    zz += [load_z(zx, k1), load_z(zh, k1)]
                return _dot(f2, jnp.concatenate(zz, axis=1))

            def stage3(g, r):
                ys = []
                for i in range(group):
                    xf = r[:, (2 * i) * 128:(2 * i + 1) * 128]
                    hf = r[:, (2 * i + 1) * 128:(2 * i + 2) * 128]
                    xr, xi, hr, hi = xf[:N2], xf[N2:], hf[:N2], hf[N2:]
                    ys.append(jnp.concatenate([xr * hr - xi * hi, xr * hi + xi * hr], axis=0).astype(BF16))
                t = _dot(g2, jnp.concatenate(ys, axis=1))
                for i in range(group):
                    tt[pl.ds((g * group + i) * ST, 2 * N2), :] = t[:, i * 128:(i + 1) * 128]

            n_groups = N1 // group
            r = stage2(0)
            for g in range(n_groups):
                r_next = stage2(g + 1) if g + 1 < n_groups else None
                stage3(g, r)
                r = r_next
            for n2 in range(N2):
                t = jnp.concatenate([tt[pl.ds(n2, N1, stride=ST), :],
                                     tt[pl.ds(N2 + n2, N1, stride=ST), :]], axis=0).astype(BF16)
                yp[pl.ds(n2, N1, stride=SX), :] = _dot(ti[n2, :, 0:2 * N1], t)
            dv = d32[pl.ds(cb, 1), :]
            for n1 in range(N1):
                y = yp[pl.ds(n1 * SX, N2), :] + xs[pl.ds(n1 * SX, N2), :] * dv
                ob[cb, pl.ds(n1 * N2, N2), :] = (y * qs[cb, pl.ds(n1 * N2, N2), :].astype(F32)).astype(BF16)
            ob_copy(cb).start()
            return carry

        for c in t_copies():
            c.wait()
        jax.lax.fori_loop(0, n_cb, b_block, 0)

        for m in range(3):
            for c in w_copies(m):
                c.wait()

            def relayout(hp, carry, m=m):
                even = stage[m * n_hp + hp, pl.ds(0, d_model // 2, stride=2), :]
                odd = stage[m * n_hp + hp, pl.ds(1, d_model // 2, stride=2), :]
                wqkv[(2 * hp) * 3 + m] = (even & U32(0xFFFF)) | (odd << 16)
                wqkv[(2 * hp + 1) * 3 + m] = (even >> 16) | (odd & U32(0xFFFF0000))
                return carry

            jax.lax.fori_loop(0, n_hp, relayout, 0)

        def wtile(ref, i):
            return pltpu.bitcast(ref[i], BF16)

        x_copy(0).wait()
        for c in o_copies():
            c.wait()

        def step(s, carry):
            @pl.when(jnp.logical_and(s % steps_per_chunk == 0, s > 0))
            def _():
                x_copy_dyn = pltpu.make_async_copy(
                    x_hbm.at[pl.ds(0, x_rows), :], xin.at[pl.ds(0, x_rows), :], sem_x.at[s // steps_per_chunk])
                x_copy_dyn.wait()

            row = jax.lax.broadcasted_iota(jnp.int32, (n_rows, n_rows), 0)
            col = jax.lax.broadcasted_iota(jnp.int32, (n_rows, n_rows), 1)
            mask = (row < n_mem) | (row >= col)
            r0 = pl.multiple_of(s * seg, seg)
            hbuf[n_mem:n_rows, :] = xin[pl.ds(r0, seg), :].astype(F32)
            hl = hbuf[...]
            for h in range(n_heads):
                qbuf[h] = _dot(hl, wtile(wqkv, 3 * h))
                kbuf[h, 0:n_rows] = _dot(hl, wtile(wqkv, 3 * h + 1)).astype(BF16)
                vbuf[h, 0:n_rows] = _dot(hl, wtile(wqkv, 3 * h + 2)).astype(BF16)
            for h in range(n_heads):
                sc = _dot_nt(qbuf[h], kbuf[h, 0:n_rows])
                sc = jnp.where(mask, sc, -1e9 / scale)
                e = jnp.exp2((sc - jnp.max(sc, axis=-1, keepdims=True)) * exp_scale)
                den = jnp.sum(e, axis=-1, keepdims=True)
                inv = pl.reciprocal(den, approx=True)
                inv = inv * (2.0 - den * inv)
                obuf[:, h * d_head:(h + 1) * d_head] = _dot(e, vbuf[h, 0:n_rows]) * inv
            ol = obuf[...]
            for j in range(d_model // 128):
                y = _dot(ol, wtile(wo, j))
                hbuf[0:n_mem, j * 128:(j + 1) * 128] = y[0:n_mem]
                oa[pl.ds(r0, seg), j * 128:(j + 1) * 128] = y[n_mem:n_rows].astype(BF16)
            oa_copy(s).start()
            return carry

        jax.lax.fori_loop(0, n_seg, step, 0)

        for cb in range(n_cb):
            ob_copy(cb).wait()
        for s in range(n_seg):
            oa_copy(s).wait()

    return kernel


def _forward(x, mem0, wq, wk, wv, wo, seg_len, q, k, v, shift_k, ssm_k, ssm_d):
    _, seq, d_model = x.shape
    _, n_heads, d_head = wq.shape
    n_mem = mem0.shape[1]
    seg = seg_len
    n_seg = seq // seg
    n_rows = n_mem + seg
    n_cb = d_model // CB
    assert seq == SEQ and d_model == 1024 and d_head == 128 and n_rows % 8 == 0
    tf, ti, t2 = _dft_tables()

    any_spec = pl.BlockSpec(memory_space=pl.ANY)
    vmem_spec = pl.BlockSpec(memory_space=pltpu.VMEM)
    kv_rows = -(-n_rows // 16) * 16
    scratch = [
        pltpu.VMEM((n_cb, CB, seq), BF16),
        pltpu.VMEM((n_cb, seq, CB), BF16),
        pltpu.VMEM((n_cb, seq, CB), BF16),
        pltpu.VMEM((n_cb, seq, CB), BF16),
        pltpu.VMEM((n_cb, seq, CB), BF16),
        pltpu.VMEM((8 + seq, CB), F32),
        pltpu.VMEM((N1 * SX, CB), F32),
        pltpu.VMEM((N1 * SX, CB), F32),
        pltpu.VMEM((N2 * SZ, CB), F32),
        pltpu.VMEM((N2 * SZ, CB), F32),
        pltpu.VMEM((N1 * ST, CB), F32),
        pltpu.VMEM((N1 * SX, CB), F32),
        pltpu.VMEM(tf.shape, BF16),
        pltpu.VMEM(ti.shape, BF16),
        pltpu.VMEM(t2.shape, BF16),
        pltpu.VMEM((4, d_model), F32),
        pltpu.VMEM((n_cb, CB), F32),
        pltpu.VMEM((3 * n_heads // 2, d_model, d_head), U32),
        pltpu.VMEM((3 * n_heads, d_model // 2, d_head), U32),
        pltpu.VMEM((d_model // 128, n_heads * d_head // 2, 128), U32),
        pltpu.VMEM((seq, d_model), BF16),
        pltpu.VMEM((seq, d_model), BF16),
        pltpu.VMEM((n_rows, d_model), F32),
        pltpu.VMEM((n_heads, n_rows, d_head), F32),
        pltpu.VMEM((n_heads, kv_rows, d_head), BF16),
        pltpu.VMEM((n_heads, kv_rows, d_head), BF16),
        pltpu.VMEM((n_rows, n_heads * d_head), F32),
        pltpu.SemaphoreType.DMA((4, n_cb)),
        pltpu.SemaphoreType.DMA((3,)),
        pltpu.SemaphoreType.DMA((3,)),
        pltpu.SemaphoreType.DMA(()),
        pltpu.SemaphoreType.DMA((8,)),
        pltpu.SemaphoreType.DMA(()),
        pltpu.SemaphoreType.DMA(()),
    ]
    out = pl.pallas_call(
        _make_kernel(n_heads, d_head, d_model, n_mem, seg, n_seg),
        out_shape=jax.ShapeDtypeStruct((seq, 2 * d_model), BF16),
        in_specs=[vmem_spec] * 3 + [any_spec] * 12,
        out_specs=any_spec,
        scratch_shapes=scratch,
        compiler_params=pltpu.CompilerParams(vmem_limit_bytes=120 * 1024 * 1024),
    )(shift_k.T, ssm_d.reshape(n_cb, CB), mem0.reshape(n_mem, d_model),
      x.reshape(seq, d_model), wq, wk, wv, wo.reshape(n_heads * d_head, d_model),
      q.reshape(seq, d_model), k.reshape(seq, d_model), v.reshape(seq, d_model), ssm_k,
      tf, ti, t2)
    return out.reshape(1, seq, 2 * d_model)


def pallas_concat_heads__memory_aug_recurrent_mem_tr__ssm_conv_h3__prompt_kernel(
        A_x, A_mem0, A_Wq, A_Wk, A_Wv, A_Wo, A_seg_len, B_q, B_k, B_v, B_shift_k, B_ssm_k, B_ssm_D):
    return _forward(A_x, A_mem0, A_Wq, A_Wk, A_Wv, A_Wo, int(A_seg_len), B_q, B_k, B_v,
                    B_shift_k, B_ssm_k, B_ssm_D)
```

```python
import math

import jax
import jax.numpy as jnp
import numpy as np
from jax.experimental import pallas as pl
from jax.experimental.pallas import tpu as pltpu

F32 = jnp.float32
BF16 = jnp.bfloat16
U32 = jnp.uint32

N1, N2 = 32, 64
SEQ = N1 * N2
SX = N2 + 4
SZ = N2 + 4
ST = 2 * N2 + 4
CB = 128


def _dft_tables():
    theta = np.pi / (2 * SEQ)
    k1 = np.arange(N1)[:, None]
    n1 = np.arange(N1)[None, :]
    fwd = np.zeros((N2, 2 * N1, 128), np.float64)
    inv = np.zeros((N2, N1, 128), np.float64)
    for n2 in range(N2):
        ph = theta * (4 * k1 + 1) * (N2 * n1 + n2)
        fwd[n2, :N1, :N1] = np.cos(ph)
        fwd[n2, N1:, :N1] = np.sin(ph)
        inv[n2, :, :N1] = np.cos(ph).T / SEQ
        inv[n2, :, N1:2 * N1] = np.sin(ph).T / SEQ
    k2 = np.arange(N2)[:, None]
    n2 = np.arange(N2)[None, :]
    ph = 2 * np.pi * k2 * n2 / N2
    c, s = np.cos(ph), np.sin(ph)
    f2 = np.block([[c, -s], [s, c]])
    g2 = np.block([[c.T, s.T], [-s.T, c.T]])
    as_bf16 = lambda a: a.astype(np.float32).astype(BF16)
    return as_bf16(fwd), as_bf16(inv), as_bf16(np.stack([f2, g2]))


def _dot(a, b):
    return jnp.dot(a, b, preferred_element_type=F32)


def _dot_nt(a, b):
    return jax.lax.dot_general(a, b, (((1,), (1,)), ((), ())), preferred_element_type=F32)


def _make_kernel(n_heads, d_head, d_model, n_mem, seg, n_seg):
    n_rows = n_mem + seg
    n_cb = d_model // CB
    n_hp = n_heads // 2
    scale = d_head ** (-0.5)
    exp_scale = scale * math.log2(math.e)
    x_chunks = 8
    x_rows = SEQ // x_chunks
    steps_per_chunk = x_rows // seg
    out_slots = 4

    def kernel(sh_ref, d_ref, mem_ref,
               x_hbm, wq_hbm, wk_hbm, wv_hbm, wo_hbm,
               q_hbm, k_hbm, v_hbm, h_hbm, tf_hbm, ti_hbm, t2_hbm,
               out_hbm,
               hs, ks, vs, ob, kf, xs, ht, zx, zh, tt, yp, tf, ti, t2, sh32, d32,
               stage, wqkv, wo, xin, qin, ost, hbuf, qbuf, kbuf, vbuf, obuf,
               sem_b, sem_t, sem_w, sem_o, sem_x, sem_q, sem_out):

        def b_copies(cb):
            c0 = cb * CB if isinstance(cb, int) else pl.multiple_of(cb * CB, CB)
            return [
                pltpu.make_async_copy(h_hbm.at[pl.ds(c0, CB), :], hs.at[cb], sem_b.at[0, cb]),
                pltpu.make_async_copy(k_hbm.at[:, pl.ds(c0, CB)], ks.at[cb], sem_b.at[1, cb]),
                pltpu.make_async_copy(v_hbm.at[:, pl.ds(c0, CB)], vs.at[cb], sem_b.at[2, cb]),
            ]

        def t_copies():
            return [pltpu.make_async_copy(tf_hbm, tf, sem_t.at[0]),
                    pltpu.make_async_copy(ti_hbm, ti, sem_t.at[1]),
                    pltpu.make_async_copy(t2_hbm, t2, sem_t.at[2])]

        def w_copies(m):
            w32 = (wq_hbm, wk_hbm, wv_hbm)[m].bitcast(U32)
            return [pltpu.make_async_copy(w32.at[:, hp, :], stage.at[m * n_hp + hp], sem_w.at[m])
                    for hp in range(n_hp)]

        def o_copies():
            wo32 = wo_hbm.bitcast(U32)
            return [pltpu.make_async_copy(wo32.at[:, pl.ds(j * 128, 128)], wo.at[j], sem_o)
                    for j in range(d_model // 128)]

        def row_copy(src, dst, sem, c):
            r0 = c * x_rows if isinstance(c, int) else pl.multiple_of(c * x_rows, x_rows)
            return pltpu.make_async_copy(src.at[pl.ds(r0, x_rows), :], dst.at[pl.ds(r0, x_rows), :], sem.at[c])

        def x_copy(c):
            return row_copy(x_hbm, xin, sem_x, c)

        def q_copy(c):
            return row_copy(q_hbm, qin, sem_q, c)

        def out_copy(s):
            r0 = s * seg if isinstance(s, int) else pl.multiple_of(s * seg, seg)
            return pltpu.make_async_copy(ost.at[s % out_slots], out_hbm.at[pl.ds(r0, seg), :], sem_out.at[s % out_slots])

        for c in b_copies(0):
            c.start()
        for c in t_copies():
            c.start()
        for cb in range(1, n_cb):
            for c in b_copies(cb):
                c.start()
        late = w_copies(0) + w_copies(1) + w_copies(2) + [x_copy(0)] + o_copies() + [q_copy(0)]
        per_block = 12

        kf[0:8, :] = jnp.zeros((8, CB), F32)
        sh32[...] = sh_ref[...].astype(F32)
        d32[...] = d_ref[...].astype(F32)
        hbuf[0:n_mem, :] = mem_ref[...].astype(F32)
        eye = (jax.lax.broadcasted_iota(jnp.int32, (128, 128), 0)
               == jax.lax.broadcasted_iota(jnp.int32, (128, 128), 1)).astype(BF16)

        group = 4

        def load_z(z, k1):
            return jnp.concatenate([z[pl.ds(k1, N2, stride=SZ), :],
                                    z[pl.ds(N1 + k1, N2, stride=SZ), :]], axis=0).astype(BF16)

        def b_block(cb, carry):
            c0 = pl.multiple_of(cb * CB, CB)
            for c in b_copies(cb):
                c.wait()
            for i in range(n_cb):
                @pl.when(cb == i)
                def _(i=i):
                    for c in late[i * per_block:(i + 1) * per_block]:
                        c.start()
            for j in range(SEQ // 128):
                r = _dot_nt(eye, hs[cb, :, j * 128:(j + 1) * 128])
                ht[pl.ds((2 * j) * SX, N2), :] = r[0:N2]
                ht[pl.ds((2 * j + 1) * SX, N2), :] = r[N2:2 * N2]
            kf[8:8 + SEQ, :] = ks[cb].astype(F32)
            taps = sh32[:, pl.ds(c0, CB)]
            for n1 in range(N1):
                acc = kf[pl.ds(8 + n1 * N2, N2), :] * taps[0:1]
                for i in range(1, 4):
                    acc = acc + kf[pl.ds(8 - i + n1 * N2, N2), :] * taps[i:i + 1]
                xs[pl.ds(n1 * SX, N2), :] = acc * vs[cb, pl.ds(n1 * N2, N2), :].astype(F32)
            for n2 in range(N2):
                a = tf[n2, :, 0:N1]
                zx[pl.ds(n2 * SZ, 2 * N1), :] = _dot(a, xs[pl.ds(n2, N1, stride=SX), :].astype(BF16))
                zh[pl.ds(n2 * SZ, 2 * N1), :] = _dot(a, ht[pl.ds(n2, N1, stride=SX), :].astype(BF16))
            f2 = t2[0]
            g2 = t2[1]

            def stage2(g):
                zz = []
                for k1 in range(g * group, (g + 1) * group):
                    zz += [load_z(zx, k1), load_z(zh, k1)]
                return _dot(f2, jnp.concatenate(zz, axis=1))

            def stage3(g, r):
                ys = []
                for i in range(group):
                    xf = r[:, (2 * i) * 128:(2 * i + 1) * 128]
                    hf = r[:, (2 * i + 1) * 128:(2 * i + 2) * 128]
                    xr, xi, hr, hi = xf[:N2], xf[N2:], hf[:N2], hf[N2:]
                    ys.append(jnp.concatenate([xr * hr - xi * hi, xr * hi + xi * hr], axis=0).astype(BF16))
                t = _dot(g2, jnp.concatenate(ys, axis=1))
                for i in range(group):
                    tt[pl.ds((g * group + i) * ST, 2 * N2), :] = t[:, i * 128:(i + 1) * 128]

            n_groups = N1 // group
            r = stage2(0)
            for g in range(n_groups):
                r_next = stage2(g + 1) if g + 1 < n_groups else None
                stage3(g, r)
                r = r_next
            for n2 in range(N2):
                t = jnp.concatenate([tt[pl.ds(n2, N1, stride=ST), :],
                                     tt[pl.ds(N2 + n2, N1, stride=ST), :]], axis=0).astype(BF16)
                yp[pl.ds(n2, N1, stride=SX), :] = _dot(ti[n2, :, 0:2 * N1], t)
            dv = d32[pl.ds(cb, 1), :]
            for n1 in range(N1):
                y = yp[pl.ds(n1 * SX, N2), :] + xs[pl.ds(n1 * SX, N2), :] * dv
                ob[cb, pl.ds(n1 * N2, N2), :] = y.astype(BF16)
            return carry

        for c in t_copies():
            c.wait()
        jax.lax.fori_loop(0, n_cb, b_block, 0)

        for m in range(3):
            for c in w_copies(m):
                c.wait()

            def relayout(hp, carry, m=m):
                even = stage[m * n_hp + hp, pl.ds(0, d_model // 2, stride=2), :]
                odd = stage[m * n_hp + hp, pl.ds(1, d_model // 2, stride=2), :]
                wqkv[(2 * hp) * 3 + m] = (even & U32(0xFFFF)) | (odd << 16)
                wqkv[(2 * hp + 1) * 3 + m] = (even >> 16) | (odd & U32(0xFFFF0000))
                return carry

            jax.lax.fori_loop(0, n_hp, relayout, 0)

        def wtile(ref, i):
            return pltpu.bitcast(ref[i], BF16)

        def step(s, first):
            if first:
                x_copy(0).wait()
            else:
                @pl.when(s % steps_per_chunk == 0)
                def _():
                    x_copy(s // steps_per_chunk).wait()
                    q_copy(s // steps_per_chunk).wait()

                @pl.when(s >= out_slots)
                def _():
                    out_copy(s - out_slots).wait()

            @pl.when(jnp.logical_and(s % steps_per_chunk == 0, s + steps_per_chunk < n_seg))
            def _():
                nxt = jnp.minimum(s // steps_per_chunk + 1, x_chunks - 1)
                x_copy(nxt).start()
                q_copy(nxt).start()

            row = jax.lax.broadcasted_iota(jnp.int32, (n_rows, n_rows), 0)
            col = jax.lax.broadcasted_iota(jnp.int32, (n_rows, n_rows), 1)
            mask = (row < n_mem) | (row >= col)
            r0 = s * seg if first else pl.multiple_of(s * seg, seg)
            slot = s % out_slots
            hbuf[n_mem:n_rows, :] = xin[pl.ds(r0, seg), :].astype(F32)
            hl = hbuf[...]
            for h in range(n_heads):
                qbuf[h] = _dot(hl, wtile(wqkv, 3 * h))
                kbuf[h, 0:n_rows] = _dot(hl, wtile(wqkv, 3 * h + 1)).astype(BF16)
                vbuf[h, 0:n_rows] = _dot(hl, wtile(wqkv, 3 * h + 2)).astype(BF16)
            for h in range(n_heads):
                sc = _dot_nt(qbuf[h], kbuf[h, 0:n_rows])
                sc = jnp.where(mask, sc, -1e9 / scale)
                e = jnp.exp2((sc - jnp.max(sc, axis=-1, keepdims=True)) * exp_scale)
                den = jnp.sum(e, axis=-1, keepdims=True)
                inv = pl.reciprocal(den, approx=True)
                inv = inv * (2.0 - den * inv)
                obuf[:, h * d_head:(h + 1) * d_head] = _dot(e, vbuf[h, 0:n_rows]) * inv
            if first:
                for c in o_copies():
                    c.wait()
                q_copy(0).wait()
            ol = obuf[...]
            for j in range(d_model // 128):
                y = _dot(ol, wtile(wo, j))
                hbuf[0:n_mem, j * 128:(j + 1) * 128] = y[0:n_mem]
                ost[slot, :, j * 128:(j + 1) * 128] = y[n_mem:n_rows].astype(BF16)
            for cb in range(n_cb):
                gate = qin[pl.ds(r0, seg), cb * CB:(cb + 1) * CB].astype(F32)
                ost[slot, :, d_model + cb * CB:d_model + (cb + 1) * CB] = (
                    ob[cb, pl.ds(r0, seg), :].astype(F32) * gate).astype(BF16)
            out_copy(s).start()

        def step_body(s, carry):
            step(s, False)
            return carry

        step(0, True)
        jax.lax.fori_loop(1, n_seg, step_body, 0)
        for s in range(n_seg - out_slots, n_seg):
            out_copy(s).wait()

    return kernel


def _forward(x, mem0, wq, wk, wv, wo, seg_len, q, k, v, shift_k, ssm_k, ssm_d):
    _, seq, d_model = x.shape
    _, n_heads, d_head = wq.shape
    n_mem = mem0.shape[1]
    seg = seg_len
    n_seg = seq // seg
    n_rows = n_mem + seg
    n_cb = d_model // CB
    assert seq == SEQ and d_model == 1024 and d_head == 128 and n_rows % 8 == 0
    tf, ti, t2 = _dft_tables()

    any_spec = pl.BlockSpec(memory_space=pl.ANY)
    vmem_spec = pl.BlockSpec(memory_space=pltpu.VMEM)
    kv_rows = -(-n_rows // 16) * 16
    scratch = [
        pltpu.VMEM((n_cb, CB, seq), BF16),
        pltpu.VMEM((n_cb, seq, CB), BF16),
        pltpu.VMEM((n_cb, seq, CB), BF16),
        pltpu.VMEM((n_cb, seq, CB), BF16),
        pltpu.VMEM((8 + seq, CB), F32),
        pltpu.VMEM((N1 * SX, CB), F32),
        pltpu.VMEM((N1 * SX, CB), F32),
        pltpu.VMEM((N2 * SZ, CB), F32),
        pltpu.VMEM((N2 * SZ, CB), F32),
        pltpu.VMEM((N1 * ST, CB), F32),
        pltpu.VMEM((N1 * SX, CB), F32),
        pltpu.VMEM(tf.shape, BF16),
        pltpu.VMEM(ti.shape, BF16),
        pltpu.VMEM(t2.shape, BF16),
        pltpu.VMEM((4, d_model), F32),
        pltpu.VMEM((n_cb, CB), F32),
        pltpu.VMEM((3 * n_heads // 2, d_model, d_head), U32),
        pltpu.VMEM((3 * n_heads, d_model // 2, d_head), U32),
        pltpu.VMEM((d_model // 128, n_heads * d_head // 2, 128), U32),
        pltpu.VMEM((seq, d_model), BF16),
        pltpu.VMEM((seq, d_model), BF16),
        pltpu.VMEM((4, seg, 2 * d_model), BF16),
        pltpu.VMEM((n_rows, d_model), F32),
        pltpu.VMEM((n_heads, n_rows, d_head), F32),
        pltpu.VMEM((n_heads, kv_rows, d_head), BF16),
        pltpu.VMEM((n_heads, kv_rows, d_head), BF16),
        pltpu.VMEM((n_rows, n_heads * d_head), F32),
        pltpu.SemaphoreType.DMA((3, n_cb)),
        pltpu.SemaphoreType.DMA((3,)),
        pltpu.SemaphoreType.DMA((3,)),
        pltpu.SemaphoreType.DMA(()),
        pltpu.SemaphoreType.DMA((8,)),
        pltpu.SemaphoreType.DMA((8,)),
        pltpu.SemaphoreType.DMA((4,)),
    ]
    out = pl.pallas_call(
        _make_kernel(n_heads, d_head, d_model, n_mem, seg, n_seg),
        out_shape=jax.ShapeDtypeStruct((seq, 2 * d_model), BF16),
        in_specs=[vmem_spec] * 3 + [any_spec] * 12,
        out_specs=any_spec,
        scratch_shapes=scratch,
        compiler_params=pltpu.CompilerParams(vmem_limit_bytes=120 * 1024 * 1024),
    )(shift_k.T, ssm_d.reshape(n_cb, CB), mem0.reshape(n_mem, d_model),
      x.reshape(seq, d_model), wq, wk, wv, wo.reshape(n_heads * d_head, d_model),
      q.reshape(seq, d_model), k.reshape(seq, d_model), v.reshape(seq, d_model), ssm_k,
      tf, ti, t2)
    return out.reshape(1, seq, 2 * d_model)


def pallas_concat_heads__memory_aug_recurrent_mem_tr__ssm_conv_h3__prompt_kernel(
        A_x, A_mem0, A_Wq, A_Wk, A_Wv, A_Wo, A_seg_len, B_q, B_k, B_v, B_shift_k, B_ssm_k, B_ssm_D):
    return _forward(A_x, A_mem0, A_Wq, A_Wk, A_Wv, A_Wo, int(A_seg_len), B_q, B_k, B_v,
                    B_shift_k, B_ssm_k, B_ssm_D)
```

```python
import math

import jax
import jax.numpy as jnp
import numpy as np
from jax.experimental import pallas as pl
from jax.experimental.pallas import tpu as pltpu

F32 = jnp.float32
BF16 = jnp.bfloat16
U32 = jnp.uint32

N1, N2 = 32, 64
SEQ = N1 * N2
SX = N2 + 4
SZ = N2 + 4
ST = 2 * N2 + 4
CB = 128


def _dft_tables():
    theta = np.pi / (2 * SEQ)
    k1 = np.arange(N1)[:, None]
    n1 = np.arange(N1)[None, :]
    fwd = np.zeros((N2, 2 * N1, 128), np.float64)
    inv = np.zeros((N2, N1, 128), np.float64)
    for n2 in range(N2):
        ph = theta * (4 * k1 + 1) * (N2 * n1 + n2)
        fwd[n2, :N1, :N1] = np.cos(ph)
        fwd[n2, N1:, :N1] = np.sin(ph)
        inv[n2, :, :N1] = np.cos(ph).T / SEQ
        inv[n2, :, N1:2 * N1] = np.sin(ph).T / SEQ
    k2 = np.arange(N2)[:, None]
    n2 = np.arange(N2)[None, :]
    ph = 2 * np.pi * k2 * n2 / N2
    c, s = np.cos(ph), np.sin(ph)
    f2 = np.block([[c, -s], [s, c]])
    g2 = np.block([[c.T, s.T], [-s.T, c.T]])
    as_bf16 = lambda a: a.astype(np.float32).astype(BF16)
    return as_bf16(fwd), as_bf16(inv), as_bf16(np.stack([f2, g2]))


_CFG = dict(group=4, lag_s=1, lag_v=1, wo_split=24, gate_at=1)


def _step_order(n_heads, n_out_tiles):
    g, a, b = _CFG["group"], _CFG["lag_s"], _CFG["lag_v"]
    split = _CFG["wo_split"]
    n_groups = n_heads // g
    total = n_groups + a + b
    early = [("W", j, 0, split) for j in range(n_out_tiles)] if split < n_heads else []
    ops = []
    for t in range(total):
        if t < n_groups:
            ops += [("P", h) for h in range(t * g, (t + 1) * g)]
        if t == _CFG["gate_at"]:
            ops.append(("G",))
        if 0 <= t - a < n_groups:
            ops += [("S", h) for h in range((t - a) * g, (t - a + 1) * g)]
        if 0 <= t - a - b < n_groups:
            ops += [("V", h) for h in range((t - a - b) * g, (t - a - b + 1) * g)]
        if early and (t - a - b + 1) * g >= split:
            n = -(-len(early) // (total - t))
            ops += early[:n]
            early = early[n:]
    ops += early
    ops += [("W", j, split if split < n_heads else 0, n_heads) for j in range(n_out_tiles)]
    return ops


def _dot(a, b):
    return jnp.dot(a, b, preferred_element_type=F32)


def _dot_nt(a, b):
    return jax.lax.dot_general(a, b, (((1,), (1,)), ((), ())), preferred_element_type=F32)


def _make_kernel(n_heads, d_head, d_model, n_mem, seg, n_seg):
    n_rows = n_mem + seg
    n_cb = d_model // CB
    n_hp = n_heads // 2
    scale = d_head ** (-0.5)
    exp_scale = scale * math.log2(math.e)
    x_chunks = 8
    x_rows = SEQ // x_chunks
    steps_per_chunk = x_rows // seg
    order = _step_order(n_heads, d_model // 128)

    def kernel(sh_ref, d_ref, mem_ref,
               x_hbm, wq_hbm, wk_hbm, wv_hbm, wo_hbm,
               q_hbm, k_hbm, v_hbm, h_hbm, tf_hbm, ti_hbm, t2_hbm,
               out_hbm,
               hs, ks, vs, ob, kf, xs, ht, zx, zh, tt, yp, tf, ti, t2, sh32, d32,
               stage, wqkv, wo, xin, qin, ost, hbuf, qbuf, kbuf, vbuf, obuf, pbuf, ibuf, ybuf,
               sem_b, sem_t, sem_w, sem_o, sem_x, sem_q, sem_out):

        def b_copies(cb):
            c0 = cb * CB if isinstance(cb, int) else pl.multiple_of(cb * CB, CB)
            return [
                pltpu.make_async_copy(h_hbm.at[pl.ds(c0, CB), :], hs.at[cb], sem_b.at[0, cb]),
                pltpu.make_async_copy(k_hbm.at[:, pl.ds(c0, CB)], ks.at[cb], sem_b.at[1, cb]),
                pltpu.make_async_copy(v_hbm.at[:, pl.ds(c0, CB)], vs.at[cb], sem_b.at[2, cb]),
            ]

        def t_copies():
            return [pltpu.make_async_copy(tf_hbm, tf, sem_t.at[0]),
                    pltpu.make_async_copy(ti_hbm, ti, sem_t.at[1]),
                    pltpu.make_async_copy(t2_hbm, t2, sem_t.at[2])]

        def w_copies(m):
            w32 = (wq_hbm, wk_hbm, wv_hbm)[m].bitcast(U32)
            return [pltpu.make_async_copy(w32.at[:, hp, :], stage.at[m * n_hp + hp], sem_w.at[m])
                    for hp in range(n_hp)]

        def o_copies():
            wo32 = wo_hbm.bitcast(U32)
            return [pltpu.make_async_copy(wo32.at[:, pl.ds(j * 128, 128)], wo.at[j], sem_o)
                    for j in range(d_model // 128)]

        def row_copy(src, dst, sem, c):
            r0 = c * x_rows if isinstance(c, int) else pl.multiple_of(c * x_rows, x_rows)
            return pltpu.make_async_copy(src.at[pl.ds(r0, x_rows), :], dst.at[pl.ds(r0, x_rows), :], sem.at[c])

        def x_copy(c):
            return row_copy(x_hbm, xin, sem_x, c)

        def q_copy(c):
            return row_copy(q_hbm, qin, sem_q, c)

        def out_copy(s):
            r0 = s * seg if isinstance(s, int) else pl.multiple_of(s * seg, seg)
            return pltpu.make_async_copy(ost.at[s], out_hbm.at[pl.ds(r0, seg), :], sem_out)

        for c in b_copies(0):
            c.start()
        for c in t_copies():
            c.start()
        for cb in range(1, n_cb):
            for c in b_copies(cb):
                c.start()
        late = w_copies(0) + w_copies(1) + w_copies(2) + [x_copy(0)] + o_copies() + [q_copy(0)]
        for c in range(1, x_chunks):
            late += [x_copy(c), q_copy(c)]
        per_block = 12

        kf[0:8, :] = jnp.zeros((8, CB), F32)
        sh32[...] = sh_ref[...].astype(F32)
        d32[...] = d_ref[...].astype(F32)
        hbuf[0:n_mem, :] = mem_ref[...].astype(F32)
        eye = (jax.lax.broadcasted_iota(jnp.int32, (128, 128), 0)
               == jax.lax.broadcasted_iota(jnp.int32, (128, 128), 1)).astype(BF16)

        group = 4

        def load_z(z, k1):
            return jnp.concatenate([z[pl.ds(k1, N2, stride=SZ), :],
                                    z[pl.ds(N1 + k1, N2, stride=SZ), :]], axis=0).astype(BF16)

        def b_block(cb, carry):
            c0 = pl.multiple_of(cb * CB, CB)
            for c in b_copies(cb):
                c.wait()
            for i in range(n_cb):
                @pl.when(cb == i)
                def _(i=i):
                    for c in late[i * per_block:(i + 1) * per_block]:
                        c.start()
            for j in range(SEQ // 128):
                r = _dot_nt(eye, hs[cb, :, j * 128:(j + 1) * 128])
                ht[pl.ds((2 * j) * SX, N2), :] = r[0:N2]
                ht[pl.ds((2 * j + 1) * SX, N2), :] = r[N2:2 * N2]
            kf[8:8 + SEQ, :] = ks[cb].astype(F32)
            taps = sh32[:, pl.ds(c0, CB)]
            for n1 in range(N1):
                acc = kf[pl.ds(8 + n1 * N2, N2), :] * taps[0:1]
                for i in range(1, 4):
                    acc = acc + kf[pl.ds(8 - i + n1 * N2, N2), :] * taps[i:i + 1]
                xs[pl.ds(n1 * SX, N2), :] = acc * vs[cb, pl.ds(n1 * N2, N2), :].astype(F32)
            for n2 in range(N2):
                a = tf[n2, :, 0:N1]
                zx[pl.ds(n2 * SZ, 2 * N1), :] = _dot(a, xs[pl.ds(n2, N1, stride=SX), :].astype(BF16))
                zh[pl.ds(n2 * SZ, 2 * N1), :] = _dot(a, ht[pl.ds(n2, N1, stride=SX), :].astype(BF16))
            f2 = t2[0]
            g2 = t2[1]

            def stage2(g):
                zz = []
                for k1 in range(g * group, (g + 1) * group):
                    zz += [load_z(zx, k1), load_z(zh, k1)]
                return _dot(f2, jnp.concatenate(zz, axis=1))

            def stage3(g, r):
                ys = []
                for i in range(group):
                    xf = r[:, (2 * i) * 128:(2 * i + 1) * 128]
                    hf = r[:, (2 * i + 1) * 128:(2 * i + 2) * 128]
                    xr, xi, hr, hi = xf[:N2], xf[N2:], hf[:N2], hf[N2:]
                    ys.append(jnp.concatenate([xr * hr - xi * hi, xr * hi + xi * hr], axis=0).astype(BF16))
                t = _dot(g2, jnp.concatenate(ys, axis=1))
                for i in range(group):
                    tt[pl.ds((g * group + i) * ST, 2 * N2), :] = t[:, i * 128:(i + 1) * 128]

            n_groups = N1 // group
            r = stage2(0)
            for g in range(n_groups):
                r_next = stage2(g + 1) if g + 1 < n_groups else None
                stage3(g, r)
                r = r_next
            for n2 in range(N2):
                t = jnp.concatenate([tt[pl.ds(n2, N1, stride=ST), :],
                                     tt[pl.ds(N2 + n2, N1, stride=ST), :]], axis=0).astype(BF16)
                yp[pl.ds(n2, N1, stride=SX), :] = _dot(ti[n2, :, 0:2 * N1], t)
            dv = d32[pl.ds(cb, 1), :]
            for n1 in range(N1):
                y = yp[pl.ds(n1 * SX, N2), :] + xs[pl.ds(n1 * SX, N2), :] * dv
                ob[cb, pl.ds(n1 * N2, N2), :] = y.astype(BF16)
            return carry

        for c in t_copies():
            c.wait()
        jax.lax.fori_loop(0, n_cb, b_block, 0)

        for m in range(3):
            for c in w_copies(m):
                c.wait()

            def relayout(hp, carry, m=m):
                even = stage[m * n_hp + hp, pl.ds(0, d_model // 2, stride=2), :]
                odd = stage[m * n_hp + hp, pl.ds(1, d_model // 2, stride=2), :]
                wqkv[(2 * hp) * 3 + m] = (even & U32(0xFFFF)) | (odd << 16)
                wqkv[(2 * hp + 1) * 3 + m] = (even >> 16) | (odd & U32(0xFFFF0000))
                return carry

            jax.lax.fori_loop(0, n_hp, relayout, 0)

        def wtile(ref, i):
            return pltpu.bitcast(ref[i], BF16)

        def step(s, first):
            if first:
                x_copy(0).wait()
            row = jax.lax.broadcasted_iota(jnp.int32, (n_rows, n_rows), 0)
            col = jax.lax.broadcasted_iota(jnp.int32, (n_rows, n_rows), 1)
            mask = (row < n_mem) | (row >= col)
            r0 = s * seg if first else pl.multiple_of(s * seg, seg)
            slot = s
            hbuf[n_mem:n_rows, :] = xin[pl.ds(r0, seg), :].astype(F32)
            hl = hbuf[...]
            waited = False
            for op in order:
                if op[0] == "P":
                    h = op[1]
                    qbuf[h] = _dot(hl, wtile(wqkv, 3 * h))
                    kbuf[h, 0:n_rows] = _dot(hl, wtile(wqkv, 3 * h + 1)).astype(BF16)
                    vbuf[h, 0:n_rows] = _dot(hl, wtile(wqkv, 3 * h + 2)).astype(BF16)
                elif op[0] == "S":
                    h = op[1]
                    sc = _dot_nt(qbuf[h], kbuf[h, 0:n_rows])
                    sc = jnp.where(mask, sc, -1e9 / scale)
                    e = jnp.exp2((sc - jnp.max(sc, axis=-1, keepdims=True)) * exp_scale)
                    den = jnp.sum(e, axis=-1, keepdims=True)
                    inv = pl.reciprocal(den, approx=True)
                    pbuf[h, :, 0:n_rows] = e
                    ibuf[h] = jnp.broadcast_to(inv * (2.0 - den * inv), (n_rows, d_head))
                elif op[0] == "V":
                    h = op[1]
                    obuf[:, h * d_head:(h + 1) * d_head] = (
                        _dot(pbuf[h, :, 0:n_rows], vbuf[h, 0:n_rows]) * ibuf[h])
                elif op[0] == "W":
                    _, j, lo, hi = op
                    if first and not waited:
                        for c in o_copies():
                            c.wait()
                        waited = True
                    w = pltpu.bitcast(wo[j, lo * d_head // 2:hi * d_head // 2, :], BF16)
                    y = _dot(obuf[:, lo * d_head:hi * d_head], w)
                    if lo > 0:
                        y = y + ybuf[j]
                    if hi < n_heads:
                        ybuf[j] = y
                    else:
                        hbuf[0:n_mem, j * 128:(j + 1) * 128] = y[0:n_mem]
                        ost[slot, :, j * 128:(j + 1) * 128] = y[n_mem:n_rows].astype(BF16)
                else:
                    if first:
                        q_copy(0).wait()
                    for cb in range(n_cb):
                        gate = qin[pl.ds(r0, seg), cb * CB:(cb + 1) * CB].astype(F32)
                        ost[slot, :, d_model + cb * CB:d_model + (cb + 1) * CB] = (
                            ob[cb, pl.ds(r0, seg), :].astype(F32) * gate).astype(BF16)
            out_copy(s).start()

        def step_body(s, carry):
            step(s, False)
            return carry

        def chunk_body(c, carry):
            @pl.when(c > 0)
            def _():
                x_copy(c).wait()
                q_copy(c).wait()
            jax.lax.fori_loop(jnp.maximum(c * steps_per_chunk, 1), (c + 1) * steps_per_chunk, step_body, 0)
            return carry

        step(0, True)
        jax.lax.fori_loop(0, x_chunks, chunk_body, 0)
        for s in range(n_seg):
            out_copy(s).wait()

    return kernel


def _forward(x, mem0, wq, wk, wv, wo, seg_len, q, k, v, shift_k, ssm_k, ssm_d):
    _, seq, d_model = x.shape
    _, n_heads, d_head = wq.shape
    n_mem = mem0.shape[1]
    seg = seg_len
    n_seg = seq // seg
    n_rows = n_mem + seg
    n_cb = d_model // CB
    assert seq == SEQ and d_model == 1024 and d_head == 128 and n_rows % 8 == 0
    tf, ti, t2 = _dft_tables()

    any_spec = pl.BlockSpec(memory_space=pl.ANY)
    vmem_spec = pl.BlockSpec(memory_space=pltpu.VMEM)
    kv_rows = -(-n_rows // 16) * 16
    scratch = [
        pltpu.VMEM((n_cb, CB, seq), BF16),
        pltpu.VMEM((n_cb, seq, CB), BF16),
        pltpu.VMEM((n_cb, seq, CB), BF16),
        pltpu.VMEM((n_cb, seq, CB), BF16),
        pltpu.VMEM((8 + seq, CB), F32),
        pltpu.VMEM((N1 * SX, CB), F32),
        pltpu.VMEM((N1 * SX, CB), F32),
        pltpu.VMEM((N2 * SZ, CB), F32),
        pltpu.VMEM((N2 * SZ, CB), F32),
        pltpu.VMEM((N1 * ST, CB), F32),
        pltpu.VMEM((N1 * SX, CB), F32),
        pltpu.VMEM(tf.shape, BF16),
        pltpu.VMEM(ti.shape, BF16),
        pltpu.VMEM(t2.shape, BF16),
        pltpu.VMEM((4, d_model), F32),
        pltpu.VMEM((n_cb, CB), F32),
        pltpu.VMEM((3 * n_heads // 2, d_model, d_head), U32),
        pltpu.VMEM((3 * n_heads, d_model // 2, d_head), U32),
        pltpu.VMEM((d_model // 128, n_heads * d_head // 2, 128), U32),
        pltpu.VMEM((seq, d_model), BF16),
        pltpu.VMEM((seq, d_model), BF16),
        pltpu.VMEM((n_seg, seg, 2 * d_model), BF16),
        pltpu.VMEM((n_rows, d_model), F32),
        pltpu.VMEM((n_heads, n_rows, d_head), F32),
        pltpu.VMEM((n_heads, kv_rows, d_head), BF16),
        pltpu.VMEM((n_heads, kv_rows, d_head), BF16),
        pltpu.VMEM((n_rows, n_heads * d_head), F32),
        pltpu.VMEM((n_heads, n_rows, d_head), F32),
        pltpu.VMEM((n_heads, n_rows, d_head), F32),
        pltpu.VMEM((d_model // 128, n_rows, 128), F32),
        pltpu.SemaphoreType.DMA((3, n_cb)),
        pltpu.SemaphoreType.DMA((3,)),
        pltpu.SemaphoreType.DMA((3,)),
        pltpu.SemaphoreType.DMA(()),
        pltpu.SemaphoreType.DMA((8,)),
        pltpu.SemaphoreType.DMA((8,)),
        pltpu.SemaphoreType.DMA(()),
    ]
    out = pl.pallas_call(
        _make_kernel(n_heads, d_head, d_model, n_mem, seg, n_seg),
        out_shape=jax.ShapeDtypeStruct((seq, 2 * d_model), BF16),
        in_specs=[vmem_spec] * 3 + [any_spec] * 12,
        out_specs=any_spec,
        scratch_shapes=scratch,
        compiler_params=pltpu.CompilerParams(vmem_limit_bytes=120 * 1024 * 1024),
    )(shift_k.T, ssm_d.reshape(n_cb, CB), mem0.reshape(n_mem, d_model),
      x.reshape(seq, d_model), wq, wk, wv, wo.reshape(n_heads * d_head, d_model),
      q.reshape(seq, d_model), k.reshape(seq, d_model), v.reshape(seq, d_model), ssm_k,
      tf, ti, t2)
    return out.reshape(1, seq, 2 * d_model)


def pallas_concat_heads__memory_aug_recurrent_mem_tr__ssm_conv_h3__prompt_kernel(
        A_x, A_mem0, A_Wq, A_Wk, A_Wv, A_Wo, A_seg_len, B_q, B_k, B_v, B_shift_k, B_ssm_k, B_ssm_D):
    return _forward(A_x, A_mem0, A_Wq, A_Wk, A_Wv, A_Wo, int(A_seg_len), B_q, B_k, B_v,
                    B_shift_k, B_ssm_k, B_ssm_D)
```

```python
import math

import jax
import jax.numpy as jnp
import numpy as np
from jax.experimental import pallas as pl
from jax.experimental.pallas import tpu as pltpu

F32 = jnp.float32
BF16 = jnp.bfloat16
U32 = jnp.uint32

N1, N2 = 32, 64
SEQ = N1 * N2
SX = N2 + 4
SZ = N2 + 4
ST = 2 * N2 + 4
CB = 128


def _dft_tables():
    theta = np.pi / (2 * SEQ)
    k1 = np.arange(N1)[:, None]
    n1 = np.arange(N1)[None, :]
    fwd = np.zeros((N2, 2 * N1, 128), np.float64)
    inv = np.zeros((N2, N1, 128), np.float64)
    for n2 in range(N2):
        ph = theta * (4 * k1 + 1) * (N2 * n1 + n2)
        fwd[n2, :N1, :N1] = np.cos(ph)
        fwd[n2, N1:, :N1] = np.sin(ph)
        inv[n2, :, :N1] = np.cos(ph).T / SEQ
        inv[n2, :, N1:2 * N1] = np.sin(ph).T / SEQ
    k2 = np.arange(N2)[:, None]
    n2 = np.arange(N2)[None, :]
    ph = 2 * np.pi * k2 * n2 / N2
    c, s = np.cos(ph), np.sin(ph)
    f2 = np.block([[c, -s], [s, c]])
    g2 = np.block([[c.T, s.T], [-s.T, c.T]])
    as_bf16 = lambda a: a.astype(np.float32).astype(BF16)
    return as_bf16(fwd), as_bf16(inv), as_bf16(np.stack([f2, g2]))


_CFG = dict(group=8, lag_s=2, lag_v=3, wo_split=16, gate_at=1, x_early=0)


def _step_order(n_heads, n_out_tiles):
    g, a, b = _CFG["group"], _CFG["lag_s"], _CFG["lag_v"]
    split = _CFG["wo_split"]
    n_groups = n_heads // g
    total = n_groups + a + b
    early = [("W", j, 0, split) for j in range(n_out_tiles)] if split < n_heads else []
    ops = []
    for t in range(total):
        if t < n_groups:
            ops += [("P", h) for h in range(t * g, (t + 1) * g)]
        if _CFG["x_early"] and t == n_groups - 1:
            ops.append(("X",))
        if t == _CFG["gate_at"]:
            ops.append(("G",))
        if 0 <= t - a < n_groups:
            ops += [("S", h) for h in range((t - a) * g, (t - a + 1) * g)]
        if 0 <= t - a - b < n_groups:
            ops += [("V", h) for h in range((t - a - b) * g, (t - a - b + 1) * g)]
        if early and (t - a - b + 1) * g >= split:
            n = -(-len(early) // (total - t))
            ops += early[:n]
            early = early[n:]
    ops += early
    ops += [("W", j, split if split < n_heads else 0, n_heads) for j in range(n_out_tiles)]
    return ops


def _dot(a, b):
    return jnp.dot(a, b, preferred_element_type=F32)


def _dot_nt(a, b):
    return jax.lax.dot_general(a, b, (((1,), (1,)), ((), ())), preferred_element_type=F32)


def _make_kernel(n_heads, d_head, d_model, n_mem, seg, n_seg):
    n_rows = n_mem + seg
    n_cb = d_model // CB
    n_hp = n_heads // 2
    scale = d_head ** (-0.5)
    exp_scale = scale * math.log2(math.e)
    x_chunks = 8
    x_rows = SEQ // x_chunks
    steps_per_chunk = x_rows // seg
    order = _step_order(n_heads, d_model // 128)

    def kernel(sh_ref, d_ref, mem_ref,
               x_hbm, wq_hbm, wk_hbm, wv_hbm, wo_hbm,
               q_hbm, k_hbm, v_hbm, h_hbm, tf_hbm, ti_hbm, t2_hbm,
               out_hbm,
               hs, ks, vs, ob, kf, xs, ht, zx, zh, tt, yp, tf, ti, t2, sh32, d32,
               stage, wqkv, wo, xin, qin, ost, hbuf, qbuf, kbuf, vbuf, obuf, pbuf, ibuf, ybuf,
               sem_b, sem_t, sem_w, sem_o, sem_x, sem_q, sem_out):

        def b_copies(cb):
            c0 = cb * CB if isinstance(cb, int) else pl.multiple_of(cb * CB, CB)
            return [
                pltpu.make_async_copy(h_hbm.at[pl.ds(c0, CB), :], hs.at[cb], sem_b.at[0, cb]),
                pltpu.make_async_copy(k_hbm.at[:, pl.ds(c0, CB)], ks.at[cb], sem_b.at[1, cb]),
                pltpu.make_async_copy(v_hbm.at[:, pl.ds(c0, CB)], vs.at[cb], sem_b.at[2, cb]),
            ]

        def t_copies():
            return [pltpu.make_async_copy(tf_hbm, tf, sem_t.at[0]),
                    pltpu.make_async_copy(ti_hbm, ti, sem_t.at[1]),
                    pltpu.make_async_copy(t2_hbm, t2, sem_t.at[2])]

        def w_copies(m):
            w32 = (wq_hbm, wk_hbm, wv_hbm)[m].bitcast(U32)
            return [pltpu.make_async_copy(w32.at[:, hp, :], stage.at[m * n_hp + hp], sem_w.at[m])
                    for hp in range(n_hp)]

        def o_copies():
            wo32 = wo_hbm.bitcast(U32)
            return [pltpu.make_async_copy(wo32.at[:, pl.ds(j * 128, 128)], wo.at[j], sem_o)
                    for j in range(d_model // 128)]

        def row_copy(src, dst, sem, c):
            r0 = c * x_rows if isinstance(c, int) else pl.multiple_of(c * x_rows, x_rows)
            return pltpu.make_async_copy(src.at[pl.ds(r0, x_rows), :], dst.at[pl.ds(r0, x_rows), :], sem.at[c])

        def x_copy(c):
            return row_copy(x_hbm, xin, sem_x, c)

        def q_copy(c):
            return row_copy(q_hbm, qin, sem_q, c)

        def out_copy(s):
            r0 = s * seg if isinstance(s, int) else pl.multiple_of(s * seg, seg)
            return pltpu.make_async_copy(ost.at[s], out_hbm.at[pl.ds(r0, seg), :], sem_out)

        for c in b_copies(0):
            c.start()
        for c in t_copies():
            c.start()
        for cb in range(1, n_cb):
            for c in b_copies(cb):
                c.start()
        late = w_copies(0) + w_copies(1) + w_copies(2) + [x_copy(0)] + o_copies() + [q_copy(0)]
        for c in range(1, x_chunks):
            late += [x_copy(c), q_copy(c)]
        per_block = 12

        kf[0:8, :] = jnp.zeros((8, CB), F32)
        sh32[...] = sh_ref[...].astype(F32)
        d32[...] = d_ref[...].astype(F32)
        hbuf[0:n_mem, :] = mem_ref[...].astype(F32)
        eye = (jax.lax.broadcasted_iota(jnp.int32, (128, 128), 0)
               == jax.lax.broadcasted_iota(jnp.int32, (128, 128), 1)).astype(BF16)

        group = 4

        def load_z(z, k1):
            return jnp.concatenate([z[pl.ds(k1, N2, stride=SZ), :],
                                    z[pl.ds(N1 + k1, N2, stride=SZ), :]], axis=0).astype(BF16)

        def b_block(cb, carry):
            c0 = pl.multiple_of(cb * CB, CB)
            for c in b_copies(cb):
                c.wait()
            for i in range(n_cb):
                @pl.when(cb == i)
                def _(i=i):
                    for c in late[i * per_block:(i + 1) * per_block]:
                        c.start()
            for j in range(SEQ // 128):
                r = _dot_nt(eye, hs[cb, :, j * 128:(j + 1) * 128])
                ht[pl.ds((2 * j) * SX, N2), :] = r[0:N2]
                ht[pl.ds((2 * j + 1) * SX, N2), :] = r[N2:2 * N2]
            kf[8:8 + SEQ, :] = ks[cb].astype(F32)
            taps = sh32[:, pl.ds(c0, CB)]
            for n1 in range(N1):
                acc = kf[pl.ds(8 + n1 * N2, N2), :] * taps[0:1]
                for i in range(1, 4):
                    acc = acc + kf[pl.ds(8 - i + n1 * N2, N2), :] * taps[i:i + 1]
                xs[pl.ds(n1 * SX, N2), :] = acc * vs[cb, pl.ds(n1 * N2, N2), :].astype(F32)
            for n2 in range(N2):
                a = tf[n2, :, 0:N1]
                zx[pl.ds(n2 * SZ, 2 * N1), :] = _dot(a, xs[pl.ds(n2, N1, stride=SX), :].astype(BF16))
                zh[pl.ds(n2 * SZ, 2 * N1), :] = _dot(a, ht[pl.ds(n2, N1, stride=SX), :].astype(BF16))
            f2 = t2[0]
            g2 = t2[1]

            def stage2(g):
                zz = []
                for k1 in range(g * group, (g + 1) * group):
                    zz += [load_z(zx, k1), load_z(zh, k1)]
                return _dot(f2, jnp.concatenate(zz, axis=1))

            def stage3(g, r):
                ys = []
                for i in range(group):
                    xf = r[:, (2 * i) * 128:(2 * i + 1) * 128]
                    hf = r[:, (2 * i + 1) * 128:(2 * i + 2) * 128]
                    xr, xi, hr, hi = xf[:N2], xf[N2:], hf[:N2], hf[N2:]
                    ys.append(jnp.concatenate([xr * hr - xi * hi, xr * hi + xi * hr], axis=0).astype(BF16))
                t = _dot(g2, jnp.concatenate(ys, axis=1))
                for i in range(group):
                    tt[pl.ds((g * group + i) * ST, 2 * N2), :] = t[:, i * 128:(i + 1) * 128]

            n_groups = N1 // group
            r = stage2(0)
            for g in range(n_groups):
                r_next = stage2(g + 1) if g + 1 < n_groups else None
                stage3(g, r)
                r = r_next
            for n2 in range(N2):
                t = jnp.concatenate([tt[pl.ds(n2, N1, stride=ST), :],
                                     tt[pl.ds(N2 + n2, N1, stride=ST), :]], axis=0).astype(BF16)
                yp[pl.ds(n2, N1, stride=SX), :] = _dot(ti[n2, :, 0:2 * N1], t)
            dv = d32[pl.ds(cb, 1), :]
            for n1 in range(N1):
                y = yp[pl.ds(n1 * SX, N2), :] + xs[pl.ds(n1 * SX, N2), :] * dv
                ob[cb, pl.ds(n1 * N2, N2), :] = y.astype(BF16)
            return carry

        for c in t_copies():
            c.wait()
        jax.lax.fori_loop(0, n_cb, b_block, 0)

        for m in range(3):
            for c in w_copies(m):
                c.wait()

            def relayout(hp, carry, m=m):
                even = stage[m * n_hp + hp, pl.ds(0, d_model // 2, stride=2), :]
                odd = stage[m * n_hp + hp, pl.ds(1, d_model // 2, stride=2), :]
                wqkv[(2 * hp) * 3 + m] = (even & U32(0xFFFF)) | (odd << 16)
                wqkv[(2 * hp + 1) * 3 + m] = (even >> 16) | (odd & U32(0xFFFF0000))
                return carry

            jax.lax.fori_loop(0, n_hp, relayout, 0)

        def wtile(ref, i):
            return pltpu.bitcast(ref[i], BF16)

        def step(s, first):
            if first:
                x_copy(0).wait()
            row = jax.lax.broadcasted_iota(jnp.int32, (n_rows, n_rows), 0)
            col = jax.lax.broadcasted_iota(jnp.int32, (n_rows, n_rows), 1)
            mask = (row < n_mem) | (row >= col)
            r0 = s * seg if first else pl.multiple_of(s * seg, seg)
            slot = s
            if first or not _CFG["x_early"]:
                hbuf[n_mem:n_rows, :] = xin[pl.ds(r0, seg), :].astype(F32)
            hl = hbuf[...]
            waited = False
            for op in order:
                if op[0] == "P":
                    h = op[1]
                    qbuf[h] = _dot(hl, wtile(wqkv, 3 * h))
                    kbuf[h, 0:n_rows] = _dot(hl, wtile(wqkv, 3 * h + 1)).astype(BF16)
                    vbuf[h, 0:n_rows] = _dot(hl, wtile(wqkv, 3 * h + 2)).astype(BF16)
                elif op[0] == "X":
                    r1 = pl.multiple_of(jnp.minimum(s + 1, n_seg - 1) * seg, seg)
                    hbuf[n_mem:n_rows, :] = xin[pl.ds(r1, seg), :].astype(F32)
                elif op[0] == "S":
                    h = op[1]
                    sc = _dot_nt(qbuf[h], kbuf[h, 0:n_rows])
                    sc = jnp.where(mask, sc, -1e9 / scale)
                    e = jnp.exp2((sc - jnp.max(sc, axis=-1, keepdims=True)) * exp_scale)
                    den = jnp.sum(e, axis=-1, keepdims=True)
                    inv = pl.reciprocal(den, approx=True)
                    pbuf[h, :, 0:n_rows] = e
                    ibuf[h] = jnp.broadcast_to(inv * (2.0 - den * inv), (n_rows, d_head))
                elif op[0] == "V":
                    h = op[1]
                    obuf[:, h * d_head:(h + 1) * d_head] = (
                        _dot(pbuf[h, :, 0:n_rows], vbuf[h, 0:n_rows]) * ibuf[h])
                elif op[0] == "W":
                    _, j, lo, hi = op
                    if first and not waited:
                        for c in o_copies():
                            c.wait()
                        waited = True
                    w = pltpu.bitcast(wo[j, lo * d_head // 2:hi * d_head // 2, :], BF16)
                    y = _dot(obuf[:, lo * d_head:hi * d_head], w)
                    if lo > 0:
                        y = y + ybuf[j]
                    if hi < n_heads:
                        ybuf[j] = y
                    else:
                        hbuf[0:n_mem, j * 128:(j + 1) * 128] = y[0:n_mem]
                        ost[slot, :, j * 128:(j + 1) * 128] = y[n_mem:n_rows].astype(BF16)
                else:
                    if first:
                        q_copy(0).wait()
                    for cb in range(n_cb):
                        gate = qin[pl.ds(r0, seg), cb * CB:(cb + 1) * CB].astype(F32)
                        ost[slot, :, d_model + cb * CB:d_model + (cb + 1) * CB] = (
                            ob[cb, pl.ds(r0, seg), :].astype(F32) * gate).astype(BF16)
            out_copy(s).start()

        def step_body(s, carry):
            step(s, False)
            return carry

        def chunk_body(c, carry):
            @pl.when(c > 0)
            def _():
                q_copy(c).wait()

            @pl.when(c + 1 < x_chunks)
            def _():
                x_copy(jnp.minimum(c + 1, x_chunks - 1)).wait()
            jax.lax.fori_loop(jnp.maximum(c * steps_per_chunk, 1), (c + 1) * steps_per_chunk, step_body, 0)
            return carry

        step(0, True)
        jax.lax.fori_loop(0, x_chunks, chunk_body, 0)
        for s in range(n_seg):
            out_copy(s).wait()

    return kernel


def _forward(x, mem0, wq, wk, wv, wo, seg_len, q, k, v, shift_k, ssm_k, ssm_d):
    _, seq, d_model = x.shape
    _, n_heads, d_head = wq.shape
    n_mem = mem0.shape[1]
    seg = seg_len
    n_seg = seq // seg
    n_rows = n_mem + seg
    n_cb = d_model // CB
    assert seq == SEQ and d_model == 1024 and d_head == 128 and n_rows % 8 == 0
    tf, ti, t2 = _dft_tables()

    any_spec = pl.BlockSpec(memory_space=pl.ANY)
    vmem_spec = pl.BlockSpec(memory_space=pltpu.VMEM)
    kv_rows = -(-n_rows // 16) * 16
    scratch = [
        pltpu.VMEM((n_cb, CB, seq), BF16),
        pltpu.VMEM((n_cb, seq, CB), BF16),
        pltpu.VMEM((n_cb, seq, CB), BF16),
        pltpu.VMEM((n_cb, seq, CB), BF16),
        pltpu.VMEM((8 + seq, CB), F32),
        pltpu.VMEM((N1 * SX, CB), F32),
        pltpu.VMEM((N1 * SX, CB), F32),
        pltpu.VMEM((N2 * SZ, CB), F32),
        pltpu.VMEM((N2 * SZ, CB), F32),
        pltpu.VMEM((N1 * ST, CB), F32),
        pltpu.VMEM((N1 * SX, CB), F32),
        pltpu.VMEM(tf.shape, BF16),
        pltpu.VMEM(ti.shape, BF16),
        pltpu.VMEM(t2.shape, BF16),
        pltpu.VMEM((4, d_model), F32),
        pltpu.VMEM((n_cb, CB), F32),
        pltpu.VMEM((3 * n_heads // 2, d_model, d_head), U32),
        pltpu.VMEM((3 * n_heads, d_model // 2, d_head), U32),
        pltpu.VMEM((d_model // 128, n_heads * d_head // 2, 128), U32),
        pltpu.VMEM((seq, d_model), BF16),
        pltpu.VMEM((seq, d_model), BF16),
        pltpu.VMEM((n_seg, seg, 2 * d_model), BF16),
        pltpu.VMEM((n_rows, d_model), F32),
        pltpu.VMEM((n_heads, n_rows, d_head), F32),
        pltpu.VMEM((n_heads, kv_rows, d_head), BF16),
        pltpu.VMEM((n_heads, kv_rows, d_head), BF16),
        pltpu.VMEM((n_rows, n_heads * d_head), F32),
        pltpu.VMEM((n_heads, n_rows, d_head), F32),
        pltpu.VMEM((n_heads, n_rows, d_head), F32),
        pltpu.VMEM((d_model // 128, n_rows, 128), F32),
        pltpu.SemaphoreType.DMA((3, n_cb)),
        pltpu.SemaphoreType.DMA((3,)),
        pltpu.SemaphoreType.DMA((3,)),
        pltpu.SemaphoreType.DMA(()),
        pltpu.SemaphoreType.DMA((8,)),
        pltpu.SemaphoreType.DMA((8,)),
        pltpu.SemaphoreType.DMA(()),
    ]
    out = pl.pallas_call(
        _make_kernel(n_heads, d_head, d_model, n_mem, seg, n_seg),
        out_shape=jax.ShapeDtypeStruct((seq, 2 * d_model), BF16),
        in_specs=[vmem_spec] * 3 + [any_spec] * 12,
        out_specs=any_spec,
        scratch_shapes=scratch,
        compiler_params=pltpu.CompilerParams(vmem_limit_bytes=120 * 1024 * 1024),
    )(shift_k.T, ssm_d.reshape(n_cb, CB), mem0.reshape(n_mem, d_model),
      x.reshape(seq, d_model), wq, wk, wv, wo.reshape(n_heads * d_head, d_model),
      q.reshape(seq, d_model), k.reshape(seq, d_model), v.reshape(seq, d_model), ssm_k,
      tf, ti, t2)
    return out.reshape(1, seq, 2 * d_model)


def pallas_concat_heads__memory_aug_recurrent_mem_tr__ssm_conv_h3__prompt_kernel(
        A_x, A_mem0, A_Wq, A_Wk, A_Wv, A_Wo, A_seg_len, B_q, B_k, B_v, B_shift_k, B_ssm_k, B_ssm_D):
    return _forward(A_x, A_mem0, A_Wq, A_Wk, A_Wv, A_Wo, int(A_seg_len), B_q, B_k, B_v,
                    B_shift_k, B_ssm_k, B_ssm_D)
```

```python
import math

import jax
import jax.numpy as jnp
import numpy as np
from jax.experimental import pallas as pl
from jax.experimental.pallas import tpu as pltpu

F32 = jnp.float32
BF16 = jnp.bfloat16
U32 = jnp.uint32

N1, N2 = 32, 64
SEQ = N1 * N2
SP = N2 // 2 + 4
SZ = N1 + 4
ST = N2 + 4
SY = N2 + 4
CB = 128


def _dft_tables():
    theta = np.pi / (2 * SEQ)
    lane = np.arange(128)[None, :]
    hi, mid, lo = lane // 64, (lane % 64) // 2, lane % 2
    k1 = np.arange(N1)[:, None]
    fwd = np.zeros((N2 // 4, 2 * N1, 128))
    for g in range(N2 // 4):
        ph = theta * (4 * k1 + 1) * (N2 * mid + 4 * g + 2 * hi + lo)
        fwd[g, 0::2] = np.cos(ph)
        fwd[g, 1::2] = np.sin(ph)
    n1 = np.arange(N1)[:, None]
    inv = np.zeros((N2 // 2, N1, 128))
    for i in range(N2 // 2):
        ph = theta * (4 * mid + 1) * (N2 * n1 + 2 * i + hi)
        inv[i] = np.where(lo == 0, np.cos(ph), np.sin(ph)) / SEQ
    ph = 2 * np.pi * np.arange(N2)[:, None] * np.arange(N2)[None, :] / N2
    c, s = np.cos(ph), np.sin(ph)
    f2 = np.zeros((128, 128))
    f2[:N2, 0::2], f2[:N2, 1::2], f2[N2:, 0::2], f2[N2:, 1::2] = c, -s, s, c
    g2 = np.zeros((128, 128))
    g2[0::2, :N2], g2[0::2, N2:], g2[1::2, :N2], g2[1::2, N2:] = c.T, s.T, -s.T, c.T
    as_bf16 = lambda a: a.astype(np.float32).astype(BF16)
    return as_bf16(fwd), as_bf16(inv), as_bf16(np.stack([f2, g2]))


def _to_words(x):
    return pltpu.bitcast(x.astype(BF16), U32)


def _from_words(w):
    return pltpu.bitcast(w, BF16)


_CFG = dict(group=8, lag_s=2, lag_v=3, wo_split=16, gate_at=1, x_early=0, late_first=0, late_per_block=10, xlu_t=1, b_group=4, n_early=3)


def _step_order(n_heads, n_out_tiles):
    g, a, b = _CFG["group"], _CFG["lag_s"], _CFG["lag_v"]
    split = _CFG["wo_split"]
    n_groups = n_heads // g
    total = n_groups + a + b
    early = [("W", j, 0, split) for j in range(n_out_tiles)] if split < n_heads else []
    ops = []
    for t in range(total):
        if t < n_groups:
            ops += [("P", h) for h in range(t * g, (t + 1) * g)]
        if _CFG["x_early"] and t == n_groups - 1:
            ops.append(("X",))
        if t == _CFG["gate_at"]:
            ops.append(("G",))
        if 0 <= t - a < n_groups:
            ops += [("S", h) for h in range((t - a) * g, (t - a + 1) * g)]
        if 0 <= t - a - b < n_groups:
            ops += [("V", h) for h in range((t - a - b) * g, (t - a - b + 1) * g)]
        if early and (t - a - b + 1) * g >= split:
            n = -(-len(early) // (total - t))
            ops += early[:n]
            early = early[n:]
    ops += early
    ops += [("W", j, split if split < n_heads else 0, n_heads) for j in range(n_out_tiles)]
    return ops


def _dot(a, b):
    return jnp.dot(a, b, preferred_element_type=F32)


def _dot_nt(a, b):
    return jax.lax.dot_general(a, b, (((1,), (1,)), ((), ())), preferred_element_type=F32)


def _make_kernel(n_heads, d_head, d_model, n_mem, seg, n_seg):
    n_rows = n_mem + seg
    n_cb = d_model // CB
    n_hp = n_heads // 2
    scale = d_head ** (-0.5)
    exp_scale = scale * math.log2(math.e)
    x_chunks = 8
    x_rows = SEQ // x_chunks
    steps_per_chunk = x_rows // seg
    order = _step_order(n_heads, d_model // 128)

    def kernel(sh_ref, d_ref, mem_ref,
               x_hbm, wq_hbm, wk_hbm, wv_hbm, wo_hbm,
               q_hbm, k_hbm, v_hbm, h_hbm, tf_hbm, ti_hbm, t2_hbm,
               out_hbm,
               hs, ks, vs, ob, kf, xp, hp, zx, zh, tt, yp, tf, ti, t2, sh32, d32,
               stage, wqkv, wo, xin, qin, ost, hbuf, qbuf, kbuf, vbuf, obuf, pbuf, ibuf, ybuf,
               sem_b, sem_t, sem_w, sem_o, sem_h, sem_x, sem_q, sem_out):

        def b_copies(cb):
            c0 = cb * CB if isinstance(cb, int) else pl.multiple_of(cb * CB, CB)
            return [
                pltpu.make_async_copy(h_hbm.at[pl.ds(c0, CB), :], hs.at[cb], sem_b.at[0, cb]),
                pltpu.make_async_copy(k_hbm.at[:, pl.ds(c0, CB)], ks.at[cb], sem_b.at[1, cb]),
                pltpu.make_async_copy(v_hbm.at[:, pl.ds(c0, CB)], vs.at[cb], sem_b.at[2, cb]),
            ]

        def t_copies():
            return [pltpu.make_async_copy(tf_hbm, tf, sem_t.at[0]),
                    pltpu.make_async_copy(ti_hbm, ti, sem_t.at[1]),
                    pltpu.make_async_copy(t2_hbm, t2, sem_t.at[2])]

        def w_copies(m):
            w32 = (wq_hbm, wk_hbm, wv_hbm)[m].bitcast(U32)
            return [pltpu.make_async_copy(w32.at[:, hp, :], stage.at[m * n_hp + hp], sem_w.at[m])
                    for hp in range(n_hp)]

        def o_copies(i):
            wo32 = wo_hbm.bitcast(U32)
            half = n_heads * d_head // 4
            return [pltpu.make_async_copy(wo32.at[pl.ds(i * half, half), pl.ds(j * 128, 128)],
                                          wo.at[j, pl.ds(i * half, half), :], sem_o.at[i])
                    for j in range(d_model // 128)]

        def row_copy(src, dst, sem, c):
            r0 = c * x_rows if isinstance(c, int) else pl.multiple_of(c * x_rows, x_rows)
            return pltpu.make_async_copy(src.at[pl.ds(r0, x_rows), :], dst.at[pl.ds(r0, x_rows), :], sem.at[c])

        def head_copies(k):
            lo, n = (0, seg) if k == 0 else (seg, x_rows - seg)
            return [pltpu.make_async_copy(src.at[pl.ds(lo, n), :], dst.at[pl.ds(lo, n), :], sem_h.at[2 * k + i])
                    for i, (src, dst) in enumerate(((x_hbm, xin), (q_hbm, qin)))]

        def x_copy(c):
            return row_copy(x_hbm, xin, sem_x, c)

        def q_copy(c):
            return row_copy(q_hbm, qin, sem_q, c)

        def out_copy(s):
            r0 = s * seg if isinstance(s, int) else pl.multiple_of(s * seg, seg)
            return pltpu.make_async_copy(ost.at[s], out_hbm.at[pl.ds(r0, seg), :], sem_out)

        n_early = _CFG["n_early"]
        for c in t_copies():
            c.start()
        for cb in range(n_early):
            for c in b_copies(cb):
                c.start()
        late = []
        for cb in range(n_early, n_cb):
            late += b_copies(cb)
        n_b_late = len(late)
        late += w_copies(0) + w_copies(1) + w_copies(2) + head_copies(0) + o_copies(0) + o_copies(1)
        per_block = _CFG["late_per_block"]
        first_block = _CFG["late_first"]

        kf[0:8, :] = jnp.zeros((8, CB), F32)
        sh32[...] = sh_ref[...].astype(F32)
        d32[...] = d_ref[...].astype(F32)
        hbuf[0:n_mem, :] = mem_ref[...].astype(F32)
        eye = (jax.lax.broadcasted_iota(jnp.int32, (128, 128), 0)
               == jax.lax.broadcasted_iota(jnp.int32, (128, 128), 1)).astype(BF16)

        group = _CFG["b_group"]

        def b_block(cb, carry):
            c0 = pl.multiple_of(cb * CB, CB)
            for c in b_copies(cb):
                c.wait()
            for i in range(n_cb - first_block):
                @pl.when(cb == i + first_block)
                def _(i=i):
                    lo = 0 if i == 0 else n_b_late + i * per_block
                    for c in late[lo:n_b_late + (i + 1) * per_block]:
                        c.start()
            lane = jax.lax.broadcasted_iota(jnp.int32, (1, 128), 1)
            for j in range(SEQ // 128):
                tile = hs[cb, :, j * 128:(j + 1) * 128]
                w = _to_words(tile.astype(F32).T if _CFG["xlu_t"] else _dot_nt(eye, tile))
                hp[pl.ds((2 * j) * SP, N2 // 2), :] = w[0:N2 // 2]
                hp[pl.ds((2 * j + 1) * SP, N2 // 2), :] = w[N2 // 2:N2]
            kf[8:8 + SEQ, :] = ks[cb].astype(F32)
            taps = sh32[:, pl.ds(c0, CB)]
            for n1 in range(N1):
                acc = kf[pl.ds(8 + n1 * N2, N2), :] * taps[0:1]
                for i in range(1, 4):
                    acc = acc + kf[pl.ds(8 - i + n1 * N2, N2), :] * taps[i:i + 1]
                xp[pl.ds(n1 * SP, N2 // 2), :] = _to_words(acc * vs[cb, pl.ds(n1 * N2, N2), :].astype(F32))
            for g in range(N2 // 4):
                m = tf[g]
                lhs = jnp.concatenate(
                    [jnp.where((lane // 64 == j // 2) & (lane % 2 == j % 2), m, jnp.zeros_like(m))
                     for j in range(4)], axis=0)

                def rhs(ref, g=g):
                    return _from_words(jnp.concatenate(
                        [ref[pl.ds(2 * g, N1, stride=SP), :], ref[pl.ds(2 * g + 1, N1, stride=SP), :]], axis=0))

                r = _dot(lhs, jnp.concatenate([rhs(xp), rhs(hp)], axis=1))
                wx, wh = _to_words(r[:, :128]), _to_words(r[:, 128:])
                for j in range(4):
                    zx[pl.ds((4 * g + j) * SZ, N1), :] = wx[N1 * j:N1 * j + N1]
                    zh[pl.ds((4 * g + j) * SZ, N1), :] = wh[N1 * j:N1 * j + N1]
            f2 = t2[0]
            g2 = t2[1]

            def stage2(g):
                zz = []
                for k1 in range(g * group, (g + 1) * group):
                    zz += [_from_words(zx[pl.ds(k1, N2, stride=SZ), :]),
                           _from_words(zh[pl.ds(k1, N2, stride=SZ), :])]
                return _dot(f2, jnp.concatenate(zz, axis=1))

            def stage3(g, r):
                ys = []
                for i in range(group):
                    xf = r[:, (2 * i) * 128:(2 * i + 1) * 128]
                    hf = r[:, (2 * i + 1) * 128:(2 * i + 2) * 128]
                    xr, xi, hr, hi = xf[:N2], xf[N2:], hf[:N2], hf[N2:]
                    ys.append(jnp.concatenate([xr * hr - xi * hi, xr * hi + xi * hr], axis=0).astype(BF16))
                t = _dot(g2, jnp.concatenate(ys, axis=1))
                for i in range(group):
                    tt[pl.ds((g * group + i) * ST, N2), :] = _to_words(t[:, i * 128:(i + 1) * 128])

            n_groups = N1 // group
            r = stage2(0)
            for g in range(n_groups):
                r_next = stage2(g + 1) if g + 1 < n_groups else None
                stage3(g, r)
                r = r_next
            for i in range(N2 // 2):
                m = ti[i]
                lhs = jnp.concatenate([jnp.where(lane < 64, m, jnp.zeros_like(m)),
                                       jnp.where(lane >= 64, m, jnp.zeros_like(m))], axis=0)
                y = _dot(lhs, _from_words(jnp.concatenate(
                    [tt[pl.ds(2 * i, N1, stride=ST), :], tt[pl.ds(2 * i + 1, N1, stride=ST), :]], axis=0)))
                yp[pl.ds(2 * i, N1, stride=SY), :] = y[0:N1]
                yp[pl.ds(2 * i + 1, N1, stride=SY), :] = y[N1:2 * N1]
            dv = d32[pl.ds(cb, 1), :]
            for n1 in range(N1):
                kv = _from_words(xp[pl.ds(n1 * SP, N2 // 2), :]).astype(F32)
                ob[cb, pl.ds(n1 * N2, N2), :] = (yp[pl.ds(n1 * SY, N2), :] + kv * dv).astype(BF16)
            return carry

        for c in t_copies():
            c.wait()
        jax.lax.fori_loop(0, n_cb, b_block, 0)
        for c in late[n_b_late + (n_cb - first_block) * per_block:]:
            c.start()

        for m in range(3):
            for c in w_copies(m):
                c.wait()

            def relayout(hp, carry, m=m):
                even = stage[m * n_hp + hp, pl.ds(0, d_model // 2, stride=2), :]
                odd = stage[m * n_hp + hp, pl.ds(1, d_model // 2, stride=2), :]
                wqkv[(2 * hp) * 3 + m] = (even & U32(0xFFFF)) | (odd << 16)
                wqkv[(2 * hp + 1) * 3 + m] = (even >> 16) | (odd & U32(0xFFFF0000))
                return carry

            jax.lax.fori_loop(0, n_hp, relayout, 0)

        def wtile(ref, i):
            return _from_words(ref[i])

        def step(s, first):
            if first:
                for c in head_copies(0):
                    c.wait()
            row = jax.lax.broadcasted_iota(jnp.int32, (n_rows, n_rows), 0)
            col = jax.lax.broadcasted_iota(jnp.int32, (n_rows, n_rows), 1)
            mask = (row < n_mem) | (row >= col)
            r0 = s * seg if first else pl.multiple_of(s * seg, seg)
            slot = s
            if first or not _CFG["x_early"]:
                hbuf[n_mem:n_rows, :] = xin[pl.ds(r0, seg), :].astype(F32)
            hl = hbuf[...]
            waited = [False, False]
            for op in order:
                if op[0] == "P":
                    h = op[1]
                    qbuf[h] = _dot(hl, wtile(wqkv, 3 * h))
                    kbuf[h, 0:n_rows] = _dot(hl, wtile(wqkv, 3 * h + 1)).astype(BF16)
                    vbuf[h, 0:n_rows] = _dot(hl, wtile(wqkv, 3 * h + 2)).astype(BF16)
                elif op[0] == "X":
                    r1 = pl.multiple_of(jnp.minimum(s + 1, n_seg - 1) * seg, seg)
                    hbuf[n_mem:n_rows, :] = xin[pl.ds(r1, seg), :].astype(F32)
                elif op[0] == "S":
                    h = op[1]
                    sc = _dot_nt(qbuf[h], kbuf[h, 0:n_rows])
                    sc = jnp.where(mask, sc, -1e9 / scale)
                    e = jnp.exp2((sc - jnp.max(sc, axis=-1, keepdims=True)) * exp_scale)
                    den = jnp.sum(e, axis=-1, keepdims=True)
                    inv = pl.reciprocal(den, approx=True)
                    pbuf[h, :, 0:n_rows] = e
                    ibuf[h] = jnp.broadcast_to(inv * (2.0 - den * inv), (n_rows, d_head))
                elif op[0] == "V":
                    h = op[1]
                    obuf[:, h * d_head:(h + 1) * d_head] = (
                        _dot(pbuf[h, :, 0:n_rows], vbuf[h, 0:n_rows]) * ibuf[h])
                elif op[0] == "W":
                    _, j, lo, hi = op
                    if first:
                        for i in range(2):
                            if not waited[i] and hi * 2 > i * n_heads:
                                for c in o_copies(i):
                                    c.wait()
                                waited[i] = True
                                if i == 1:
                                    for c in head_copies(1):
                                        c.start()
                                    for ch in range(1, x_chunks):
                                        x_copy(ch).start()
                                        q_copy(ch).start()
                    w = _from_words(wo[j, lo * d_head // 2:hi * d_head // 2, :])
                    y = _dot(obuf[:, lo * d_head:hi * d_head], w)
                    if lo > 0:
                        y = y + ybuf[j]
                    if hi < n_heads:
                        ybuf[j] = y
                    else:
                        hbuf[0:n_mem, j * 128:(j + 1) * 128] = y[0:n_mem]
                        ost[slot, :, j * 128:(j + 1) * 128] = y[n_mem:n_rows].astype(BF16)
                else:
                    for cb in range(n_cb):
                        gate = qin[pl.ds(r0, seg), cb * CB:(cb + 1) * CB].astype(F32)
                        ost[slot, :, d_model + cb * CB:d_model + (cb + 1) * CB] = (
                            ob[cb, pl.ds(r0, seg), :].astype(F32) * gate).astype(BF16)
            out_copy(s).start()

        def step_body(s, carry):
            step(s, False)
            return carry

        def chunk_body(c, carry):
            @pl.when(c > 0)
            def _():
                q_copy(c).wait()

            @pl.when(c + 1 < x_chunks)
            def _():
                x_copy(jnp.minimum(c + 1, x_chunks - 1)).wait()
            jax.lax.fori_loop(jnp.maximum(c * steps_per_chunk, 1), (c + 1) * steps_per_chunk, step_body, 0)
            return carry

        step(0, True)
        for c in head_copies(1):
            c.wait()
        jax.lax.fori_loop(0, x_chunks, chunk_body, 0)
        for s in range(n_seg):
            out_copy(s).wait()

    return kernel


def _forward(x, mem0, wq, wk, wv, wo, seg_len, q, k, v, shift_k, ssm_k, ssm_d):
    _, seq, d_model = x.shape
    _, n_heads, d_head = wq.shape
    n_mem = mem0.shape[1]
    seg = seg_len
    n_seg = seq // seg
    n_rows = n_mem + seg
    n_cb = d_model // CB
    assert seq == SEQ and d_model == 1024 and d_head == 128 and n_rows % 8 == 0
    tf, ti, t2 = _dft_tables()

    any_spec = pl.BlockSpec(memory_space=pl.ANY)
    vmem_spec = pl.BlockSpec(memory_space=pltpu.VMEM)
    kv_rows = -(-n_rows // 16) * 16
    scratch = [
        pltpu.VMEM((n_cb, CB, seq), BF16),
        pltpu.VMEM((n_cb, seq, CB), BF16),
        pltpu.VMEM((n_cb, seq, CB), BF16),
        pltpu.VMEM((n_cb, seq, CB), BF16),
        pltpu.VMEM((8 + seq, CB), F32),
        pltpu.VMEM((N1 * SP, CB), U32),
        pltpu.VMEM((N1 * SP, CB), U32),
        pltpu.VMEM((N2 * SZ, CB), U32),
        pltpu.VMEM((N2 * SZ, CB), U32),
        pltpu.VMEM((N1 * ST, CB), U32),
        pltpu.VMEM((N1 * SY, CB), F32),
        pltpu.VMEM(tf.shape, BF16),
        pltpu.VMEM(ti.shape, BF16),
        pltpu.VMEM(t2.shape, BF16),
        pltpu.VMEM((4, d_model), F32),
        pltpu.VMEM((n_cb, CB), F32),
        pltpu.VMEM((3 * n_heads // 2, d_model, d_head), U32),
        pltpu.VMEM((3 * n_heads, d_model // 2, d_head), U32),
        pltpu.VMEM((d_model // 128, n_heads * d_head // 2, 128), U32),
        pltpu.VMEM((seq, d_model), BF16),
        pltpu.VMEM((seq, d_model), BF16),
        pltpu.VMEM((n_seg, seg, 2 * d_model), BF16),
        pltpu.VMEM((n_rows, d_model), F32),
        pltpu.VMEM((n_heads, n_rows, d_head), F32),
        pltpu.VMEM((n_heads, kv_rows, d_head), BF16),
        pltpu.VMEM((n_heads, kv_rows, d_head), BF16),
        pltpu.VMEM((n_rows, n_heads * d_head), F32),
        pltpu.VMEM((n_heads, n_rows, d_head), F32),
        pltpu.VMEM((n_heads, n_rows, d_head), F32),
        pltpu.VMEM((d_model // 128, n_rows, 128), F32),
        pltpu.SemaphoreType.DMA((3, n_cb)),
        pltpu.SemaphoreType.DMA((3,)),
        pltpu.SemaphoreType.DMA((3,)),
        pltpu.SemaphoreType.DMA((2,)),
        pltpu.SemaphoreType.DMA((4,)),
        pltpu.SemaphoreType.DMA((8,)),
        pltpu.SemaphoreType.DMA((8,)),
        pltpu.SemaphoreType.DMA(()),
    ]
    out = pl.pallas_call(
        _make_kernel(n_heads, d_head, d_model, n_mem, seg, n_seg),
        out_shape=jax.ShapeDtypeStruct((seq, 2 * d_model), BF16),
        in_specs=[vmem_spec] * 3 + [any_spec] * 12,
        out_specs=any_spec,
        scratch_shapes=scratch,
        compiler_params=pltpu.CompilerParams(vmem_limit_bytes=120 * 1024 * 1024),
    )(shift_k.T, ssm_d.reshape(n_cb, CB), mem0.reshape(n_mem, d_model),
      x.reshape(seq, d_model), wq, wk, wv, wo.reshape(n_heads * d_head, d_model),
      q.reshape(seq, d_model), k.reshape(seq, d_model), v.reshape(seq, d_model), ssm_k,
      tf, ti, t2)
    return out.reshape(1, seq, 2 * d_model)


def pallas_concat_heads__memory_aug_recurrent_mem_tr__ssm_conv_h3__prompt_kernel(
        A_x, A_mem0, A_Wq, A_Wk, A_Wv, A_Wo, A_seg_len, B_q, B_k, B_v, B_shift_k, B_ssm_k, B_ssm_D):
    return _forward(A_x, A_mem0, A_Wq, A_Wk, A_Wv, A_Wo, int(A_seg_len), B_q, B_k, B_v,
                    B_shift_k, B_ssm_k, B_ssm_D)
```

```python
import math

import jax
import jax.numpy as jnp
import numpy as np
from jax.experimental import pallas as pl
from jax.experimental.pallas import tpu as pltpu

F32 = jnp.float32
BF16 = jnp.bfloat16
U32 = jnp.uint32

N1, N2 = 32, 64
SEQ = N1 * N2
SP = N2 // 2 + 4
SZ = N1 + 4
ST = N2 + 4
SY = N2 + 4
CB = 128


def _dft_tables():
    theta = np.pi / (2 * SEQ)
    lane = np.arange(128)[None, :]
    hi, mid, lo = lane // 64, (lane % 64) // 2, lane % 2
    k1 = np.arange(N1)[:, None]
    fwd = np.zeros((N2 // 4, 2 * N1, 128))
    for g in range(N2 // 4):
        ph = theta * (4 * k1 + 1) * (N2 * mid + 4 * g + 2 * hi + lo)
        fwd[g, 0::2] = np.cos(ph)
        fwd[g, 1::2] = np.sin(ph)
    n1 = np.arange(N1)[:, None]
    inv = np.zeros((N2 // 2, N1, 128))
    for i in range(N2 // 2):
        ph = theta * (4 * mid + 1) * (N2 * n1 + 2 * i + hi)
        inv[i] = np.where(lo == 0, np.cos(ph), np.sin(ph)) / SEQ
    ph = 2 * np.pi * np.arange(N2)[:, None] * np.arange(N2)[None, :] / N2
    c, s = np.cos(ph), np.sin(ph)
    f2 = np.zeros((128, 128))
    f2[:N2, 0::2], f2[:N2, 1::2], f2[N2:, 0::2], f2[N2:, 1::2] = c, -s, s, c
    g2 = np.zeros((128, 128))
    g2[0::2, :N2], g2[0::2, N2:], g2[1::2, :N2], g2[1::2, N2:] = c.T, s.T, -s.T, c.T
    as_bf16 = lambda a: a.astype(np.float32).astype(BF16)
    return as_bf16(fwd), as_bf16(inv), as_bf16(np.stack([f2, g2]))


def _to_words(x):
    return pltpu.bitcast(x.astype(BF16), U32)


def _from_words(w):
    return pltpu.bitcast(w, BF16)


_CFG = dict(group=8, lag_s=2, lag_v=3, wo_split=16, gate_at=1, late_first=0, late_per_block=10, xlu_t=1, b_group=4, n_early=3, unroll=3, chunk_steps=9)


def _step_order(n_heads, n_out_tiles):
    g, a, b = _CFG["group"], _CFG["lag_s"], _CFG["lag_v"]
    split = _CFG["wo_split"]
    n_groups = n_heads // g
    total = n_groups + a + b
    early = [("W", j, 0, split) for j in range(n_out_tiles)] if split < n_heads else []
    ops = []
    for t in range(total):
        if t < n_groups:
            ops += [("P", h) for h in range(t * g, (t + 1) * g)]
        if t == _CFG["gate_at"]:
            ops.append(("G",))
        if 0 <= t - a < n_groups:
            ops += [("S", h) for h in range((t - a) * g, (t - a + 1) * g)]
        if 0 <= t - a - b < n_groups:
            ops += [("V", h) for h in range((t - a - b) * g, (t - a - b + 1) * g)]
        if early and (t - a - b + 1) * g >= split:
            n = -(-len(early) // (total - t))
            ops += early[:n]
            early = early[n:]
    ops += early
    ops += [("W", j, split if split < n_heads else 0, n_heads) for j in range(n_out_tiles)]
    return ops


def _dot(a, b):
    return jnp.dot(a, b, preferred_element_type=F32)


def _dot_nt(a, b):
    return jax.lax.dot_general(a, b, (((1,), (1,)), ((), ())), preferred_element_type=F32)


def _make_kernel(n_heads, d_head, d_model, n_mem, seg, n_seg):
    n_rows = n_mem + seg
    n_cb = d_model // CB
    n_hp = n_heads // 2
    scale = d_head ** (-0.5)
    exp_scale = scale * math.log2(math.e)
    steps_per_chunk = _CFG["chunk_steps"]
    x_chunks = (n_seg - 1) // steps_per_chunk
    x_rows = steps_per_chunk * seg
    assert x_chunks * steps_per_chunk == n_seg - 1 and steps_per_chunk % _CFG["unroll"] == 0
    order = _step_order(n_heads, d_model // 128)

    def kernel(sh_ref, d_ref, mem_ref,
               x_hbm, wq_hbm, wk_hbm, wv_hbm, wo_hbm,
               q_hbm, k_hbm, v_hbm, h_hbm, tf_hbm, ti_hbm, t2_hbm,
               out_hbm,
               hs, ks, vs, ob, kf, xp, hp, zx, zh, tt, yp, tf, ti, t2, sh32, d32,
               stage, wqkv, wo, xin, qin, ost, hbuf, qbuf, kbuf, vbuf, obuf, pbuf, ibuf, ybuf,
               sem_b, sem_t, sem_w, sem_o, sem_h, sem_x, sem_q, sem_out):

        def b_copies(cb):
            c0 = cb * CB if isinstance(cb, int) else pl.multiple_of(cb * CB, CB)
            return [
                pltpu.make_async_copy(h_hbm.at[pl.ds(c0, CB), :], hs.at[cb], sem_b.at[0, cb]),
                pltpu.make_async_copy(k_hbm.at[:, pl.ds(c0, CB)], ks.at[cb], sem_b.at[1, cb]),
                pltpu.make_async_copy(v_hbm.at[:, pl.ds(c0, CB)], vs.at[cb], sem_b.at[2, cb]),
            ]

        def t_copies():
            return [pltpu.make_async_copy(tf_hbm, tf, sem_t.at[0]),
                    pltpu.make_async_copy(ti_hbm, ti, sem_t.at[1]),
                    pltpu.make_async_copy(t2_hbm, t2, sem_t.at[2])]

        def w_copies(m):
            w32 = (wq_hbm, wk_hbm, wv_hbm)[m].bitcast(U32)
            return [pltpu.make_async_copy(w32.at[:, hp, :], stage.at[m * n_hp + hp], sem_w.at[m])
                    for hp in range(n_hp)]

        def o_copies(i):
            wo32 = wo_hbm.bitcast(U32)
            half = n_heads * d_head // 4
            return [pltpu.make_async_copy(wo32.at[pl.ds(i * half, half), pl.ds(j * 128, 128)],
                                          wo.at[j, pl.ds(i * half, half), :], sem_o.at[i])
                    for j in range(d_model // 128)]

        def head_copies():
            return [pltpu.make_async_copy(src.at[pl.ds(0, seg), :], dst.at[pl.ds(0, seg), :], sem_h.at[i])
                    for i, (src, dst) in enumerate(((x_hbm, xin), (q_hbm, qin)))]

        def chunk_copies(c):
            r0 = seg + c * x_rows if isinstance(c, int) else pl.multiple_of(seg + c * x_rows, seg)
            return [pltpu.make_async_copy(src.at[pl.ds(r0, x_rows), :], dst.at[pl.ds(r0, x_rows), :], sem.at[c])
                    for src, dst, sem in ((x_hbm, xin, sem_x), (q_hbm, qin, sem_q))]

        def out_copy(s):
            r0 = s * seg if isinstance(s, int) else pl.multiple_of(s * seg, seg)
            return pltpu.make_async_copy(ost.at[s], out_hbm.at[pl.ds(r0, seg), :], sem_out)

        n_early = _CFG["n_early"]
        for c in t_copies():
            c.start()
        for cb in range(n_early):
            for c in b_copies(cb):
                c.start()
        late = []
        for cb in range(n_early, n_cb):
            late += b_copies(cb)
        n_b_late = len(late)
        late += w_copies(0) + w_copies(1) + w_copies(2) + head_copies() + o_copies(0) + o_copies(1)
        per_block = _CFG["late_per_block"]
        first_block = _CFG["late_first"]

        kf[0:8, :] = jnp.zeros((8, CB), F32)
        sh32[...] = sh_ref[...].astype(F32)
        d32[...] = d_ref[...].astype(F32)
        hbuf[0:n_mem, :] = mem_ref[...].astype(F32)
        eye = (jax.lax.broadcasted_iota(jnp.int32, (128, 128), 0)
               == jax.lax.broadcasted_iota(jnp.int32, (128, 128), 1)).astype(BF16)

        group = _CFG["b_group"]

        def b_block(cb, carry):
            c0 = pl.multiple_of(cb * CB, CB)
            for c in b_copies(cb):
                c.wait()
            for i in range(n_cb - first_block):
                @pl.when(cb == i + first_block)
                def _(i=i):
                    lo = 0 if i == 0 else n_b_late + i * per_block
                    for c in late[lo:n_b_late + (i + 1) * per_block]:
                        c.start()
            lane = jax.lax.broadcasted_iota(jnp.int32, (1, 128), 1)
            for j in range(SEQ // 128):
                tile = hs[cb, :, j * 128:(j + 1) * 128]
                w = _to_words(tile.astype(F32).T if _CFG["xlu_t"] else _dot_nt(eye, tile))
                hp[pl.ds((2 * j) * SP, N2 // 2), :] = w[0:N2 // 2]
                hp[pl.ds((2 * j + 1) * SP, N2 // 2), :] = w[N2 // 2:N2]
            kf[8:8 + SEQ, :] = ks[cb].astype(F32)
            taps = sh32[:, pl.ds(c0, CB)]
            for n1 in range(N1):
                acc = kf[pl.ds(8 + n1 * N2, N2), :] * taps[0:1]
                for i in range(1, 4):
                    acc = acc + kf[pl.ds(8 - i + n1 * N2, N2), :] * taps[i:i + 1]
                xp[pl.ds(n1 * SP, N2 // 2), :] = _to_words(acc * vs[cb, pl.ds(n1 * N2, N2), :].astype(F32))
            for g in range(N2 // 4):
                m = tf[g]
                lhs = jnp.concatenate(
                    [jnp.where((lane // 64 == j // 2) & (lane % 2 == j % 2), m, jnp.zeros_like(m))
                     for j in range(4)], axis=0)

                def rhs(ref, g=g):
                    return _from_words(jnp.concatenate(
                        [ref[pl.ds(2 * g, N1, stride=SP), :], ref[pl.ds(2 * g + 1, N1, stride=SP), :]], axis=0))

                r = _dot(lhs, jnp.concatenate([rhs(xp), rhs(hp)], axis=1))
                wx, wh = _to_words(r[:, :128]), _to_words(r[:, 128:])
                for j in range(4):
                    zx[pl.ds((4 * g + j) * SZ, N1), :] = wx[N1 * j:N1 * j + N1]
                    zh[pl.ds((4 * g + j) * SZ, N1), :] = wh[N1 * j:N1 * j + N1]
            f2 = t2[0]
            g2 = t2[1]

            def stage2(g):
                zz = []
                for k1 in range(g * group, (g + 1) * group):
                    zz += [_from_words(zx[pl.ds(k1, N2, stride=SZ), :]),
                           _from_words(zh[pl.ds(k1, N2, stride=SZ), :])]
                return _dot(f2, jnp.concatenate(zz, axis=1))

            def stage3(g, r):
                ys = []
                for i in range(group):
                    xf = r[:, (2 * i) * 128:(2 * i + 1) * 128]
                    hf = r[:, (2 * i + 1) * 128:(2 * i + 2) * 128]
                    xr, xi, hr, hi = xf[:N2], xf[N2:], hf[:N2], hf[N2:]
                    ys.append(jnp.concatenate([xr * hr - xi * hi, xr * hi + xi * hr], axis=0).astype(BF16))
                t = _dot(g2, jnp.concatenate(ys, axis=1))
                for i in range(group):
                    tt[pl.ds((g * group + i) * ST, N2), :] = _to_words(t[:, i * 128:(i + 1) * 128])

            n_groups = N1 // group
            r = stage2(0)
            for g in range(n_groups):
                r_next = stage2(g + 1) if g + 1 < n_groups else None
                stage3(g, r)
                r = r_next
            for i in range(N2 // 2):
                m = ti[i]
                lhs = jnp.concatenate([jnp.where(lane < 64, m, jnp.zeros_like(m)),
                                       jnp.where(lane >= 64, m, jnp.zeros_like(m))], axis=0)
                y = _dot(lhs, _from_words(jnp.concatenate(
                    [tt[pl.ds(2 * i, N1, stride=ST), :], tt[pl.ds(2 * i + 1, N1, stride=ST), :]], axis=0)))
                yp[pl.ds(2 * i, N1, stride=SY), :] = y[0:N1]
                yp[pl.ds(2 * i + 1, N1, stride=SY), :] = y[N1:2 * N1]
            dv = d32[pl.ds(cb, 1), :]
            for n1 in range(N1):
                kv = _from_words(xp[pl.ds(n1 * SP, N2 // 2), :]).astype(F32)
                ob[cb, pl.ds(n1 * N2, N2), :] = (yp[pl.ds(n1 * SY, N2), :] + kv * dv).astype(BF16)
            return carry

        for c in t_copies():
            c.wait()
        jax.lax.fori_loop(0, n_cb, b_block, 0)
        for c in late[n_b_late + (n_cb - first_block) * per_block:]:
            c.start()

        for m in range(3):
            for c in w_copies(m):
                c.wait()

            def relayout(hp, carry, m=m):
                even = stage[m * n_hp + hp, pl.ds(0, d_model // 2, stride=2), :]
                odd = stage[m * n_hp + hp, pl.ds(1, d_model // 2, stride=2), :]
                wqkv[(2 * hp) * 3 + m] = (even & U32(0xFFFF)) | (odd << 16)
                wqkv[(2 * hp + 1) * 3 + m] = (even >> 16) | (odd & U32(0xFFFF0000))
                return carry

            jax.lax.fori_loop(0, n_hp, relayout, 0)

        def wtile(ref, i):
            return _from_words(ref[i])

        def step(s, first):
            if first:
                for c in head_copies():
                    c.wait()
            row = jax.lax.broadcasted_iota(jnp.int32, (n_rows, n_rows), 0)
            col = jax.lax.broadcasted_iota(jnp.int32, (n_rows, n_rows), 1)
            mask = (row < n_mem) | (row >= col)
            r0 = s * seg if first else pl.multiple_of(s * seg, seg)
            slot = s
            hbuf[n_mem:n_rows, :] = xin[pl.ds(r0, seg), :].astype(F32)
            hl = hbuf[...]
            waited = [False, False]
            for op in order:
                if op[0] == "P":
                    h = op[1]
                    qbuf[h] = _dot(hl, wtile(wqkv, 3 * h))
                    kbuf[h, 0:n_rows] = _dot(hl, wtile(wqkv, 3 * h + 1)).astype(BF16)
                    vbuf[h, 0:n_rows] = _dot(hl, wtile(wqkv, 3 * h + 2)).astype(BF16)
                elif op[0] == "S":
                    h = op[1]
                    sc = _dot_nt(qbuf[h], kbuf[h, 0:n_rows])
                    sc = jnp.where(mask, sc, -1e9 / scale)
                    e = jnp.exp2((sc - jnp.max(sc, axis=-1, keepdims=True)) * exp_scale)
                    den = jnp.sum(e, axis=-1, keepdims=True)
                    inv = pl.reciprocal(den, approx=True)
                    pbuf[h, :, 0:n_rows] = e
                    ibuf[h] = jnp.broadcast_to(inv * (2.0 - den * inv), (n_rows, d_head))
                elif op[0] == "V":
                    h = op[1]
                    obuf[:, h * d_head:(h + 1) * d_head] = (
                        _dot(pbuf[h, :, 0:n_rows], vbuf[h, 0:n_rows]) * ibuf[h])
                elif op[0] == "W":
                    _, j, lo, hi = op
                    if first:
                        for i in range(2):
                            if not waited[i] and hi * 2 > i * n_heads:
                                for c in o_copies(i):
                                    c.wait()
                                waited[i] = True
                                if i == 1:
                                    for ch in range(x_chunks):
                                        for c in chunk_copies(ch):
                                            c.start()
                    w = _from_words(wo[j, lo * d_head // 2:hi * d_head // 2, :])
                    y = _dot(obuf[:, lo * d_head:hi * d_head], w)
                    if lo > 0:
                        y = y + ybuf[j]
                    if hi < n_heads:
                        ybuf[j] = y
                    else:
                        hbuf[0:n_mem, j * 128:(j + 1) * 128] = y[0:n_mem]
                        ost[slot, :, j * 128:(j + 1) * 128] = y[n_mem:n_rows].astype(BF16)
                else:
                    for cb in range(n_cb):
                        gate = qin[pl.ds(r0, seg), cb * CB:(cb + 1) * CB].astype(F32)
                        ost[slot, :, d_model + cb * CB:d_model + (cb + 1) * CB] = (
                            ob[cb, pl.ds(r0, seg), :].astype(F32) * gate).astype(BF16)
            out_copy(s).start()

        unroll = _CFG["unroll"]

        def chunk_body(c, carry):
            for cp in chunk_copies(c):
                cp.wait()

            def steps_body(i, carry):
                for u in range(unroll):
                    step(1 + c * steps_per_chunk + i * unroll + u, False)
                return carry

            if steps_per_chunk == unroll:
                steps_body(0, 0)
            else:
                jax.lax.fori_loop(0, steps_per_chunk // unroll, steps_body, 0)
            return carry

        step(0, True)
        jax.lax.fori_loop(0, x_chunks, chunk_body, 0)
        for s in range(n_seg):
            out_copy(s).wait()

    return kernel


def _forward(x, mem0, wq, wk, wv, wo, seg_len, q, k, v, shift_k, ssm_k, ssm_d):
    _, seq, d_model = x.shape
    _, n_heads, d_head = wq.shape
    n_mem = mem0.shape[1]
    seg = seg_len
    n_seg = seq // seg
    n_rows = n_mem + seg
    n_cb = d_model // CB
    assert seq == SEQ and d_model == 1024 and d_head == 128 and n_rows % 8 == 0
    tf, ti, t2 = _dft_tables()

    any_spec = pl.BlockSpec(memory_space=pl.ANY)
    vmem_spec = pl.BlockSpec(memory_space=pltpu.VMEM)
    kv_rows = -(-n_rows // 16) * 16
    scratch = [
        pltpu.VMEM((n_cb, CB, seq), BF16),
        pltpu.VMEM((n_cb, seq, CB), BF16),
        pltpu.VMEM((n_cb, seq, CB), BF16),
        pltpu.VMEM((n_cb, seq, CB), BF16),
        pltpu.VMEM((8 + seq, CB), F32),
        pltpu.VMEM((N1 * SP, CB), U32),
        pltpu.VMEM((N1 * SP, CB), U32),
        pltpu.VMEM((N2 * SZ, CB), U32),
        pltpu.VMEM((N2 * SZ, CB), U32),
        pltpu.VMEM((N1 * ST, CB), U32),
        pltpu.VMEM((N1 * SY, CB), F32),
        pltpu.VMEM(tf.shape, BF16),
        pltpu.VMEM(ti.shape, BF16),
        pltpu.VMEM(t2.shape, BF16),
        pltpu.VMEM((4, d_model), F32),
        pltpu.VMEM((n_cb, CB), F32),
        pltpu.VMEM((3 * n_heads // 2, d_model, d_head), U32),
        pltpu.VMEM((3 * n_heads, d_model // 2, d_head), U32),
        pltpu.VMEM((d_model // 128, n_heads * d_head // 2, 128), U32),
        pltpu.VMEM((seq, d_model), BF16),
        pltpu.VMEM((seq, d_model), BF16),
        pltpu.VMEM((n_seg, seg, 2 * d_model), BF16),
        pltpu.VMEM((n_rows, d_model), F32),
        pltpu.VMEM((n_heads, n_rows, d_head), F32),
        pltpu.VMEM((n_heads, kv_rows, d_head), BF16),
        pltpu.VMEM((n_heads, kv_rows, d_head), BF16),
        pltpu.VMEM((n_rows, n_heads * d_head), F32),
        pltpu.VMEM((n_heads, n_rows, d_head), F32),
        pltpu.VMEM((n_heads, n_rows, d_head), F32),
        pltpu.VMEM((d_model // 128, n_rows, 128), F32),
        pltpu.SemaphoreType.DMA((3, n_cb)),
        pltpu.SemaphoreType.DMA((3,)),
        pltpu.SemaphoreType.DMA((3,)),
        pltpu.SemaphoreType.DMA((2,)),
        pltpu.SemaphoreType.DMA((2,)),
        pltpu.SemaphoreType.DMA((n_seg,)),
        pltpu.SemaphoreType.DMA((n_seg,)),
        pltpu.SemaphoreType.DMA(()),
    ]
    out = pl.pallas_call(
        _make_kernel(n_heads, d_head, d_model, n_mem, seg, n_seg),
        out_shape=jax.ShapeDtypeStruct((seq, 2 * d_model), BF16),
        in_specs=[vmem_spec] * 3 + [any_spec] * 12,
        out_specs=any_spec,
        scratch_shapes=scratch,
        compiler_params=pltpu.CompilerParams(vmem_limit_bytes=120 * 1024 * 1024),
    )(shift_k.T, ssm_d.reshape(n_cb, CB), mem0.reshape(n_mem, d_model),
      x.reshape(seq, d_model), wq, wk, wv, wo.reshape(n_heads * d_head, d_model),
      q.reshape(seq, d_model), k.reshape(seq, d_model), v.reshape(seq, d_model), ssm_k,
      tf, ti, t2)
    return out.reshape(1, seq, 2 * d_model)


def pallas_concat_heads__memory_aug_recurrent_mem_tr__ssm_conv_h3__prompt_kernel(
        A_x, A_mem0, A_Wq, A_Wk, A_Wv, A_Wo, A_seg_len, B_q, B_k, B_v, B_shift_k, B_ssm_k, B_ssm_D):
    return _forward(A_x, A_mem0, A_Wq, A_Wk, A_Wv, A_Wo, int(A_seg_len), B_q, B_k, B_v,
                    B_shift_k, B_ssm_k, B_ssm_D)
```

```python
import functools
import math

import jax
import jax.numpy as jnp
import numpy as np
from jax.experimental import pallas as pl
from jax.experimental.pallas import tpu as pltpu

F32 = jnp.float32
BF16 = jnp.bfloat16
U32 = jnp.uint32

N1, N2 = 32, 64
SEQ = N1 * N2
SP = N2 // 2 + 4
SZ = N1 + 4
ST = N2 + 4
SY = N2 + 4
CB = 128


def _dft_tables():
    theta = np.pi / (2 * SEQ)
    lane = np.arange(128)[None, :]
    hi, mid, lo = lane // 64, (lane % 64) // 2, lane % 2
    k1 = np.arange(N1)[:, None]
    fwd = np.zeros((N2 // 4, 2 * N1, 128))
    for g in range(N2 // 4):
        ph = theta * (4 * k1 + 1) * (N2 * mid + 4 * g + 2 * hi + lo)
        fwd[g, 0::2] = np.cos(ph)
        fwd[g, 1::2] = np.sin(ph)
    n1 = np.arange(N1)[:, None]
    inv = np.zeros((N2 // 2, N1, 128))
    for i in range(N2 // 2):
        ph = theta * (4 * mid + 1) * (N2 * n1 + 2 * i + hi)
        inv[i] = np.where(lo == 0, np.cos(ph), np.sin(ph)) / SEQ
    ph = 2 * np.pi * np.arange(N2)[:, None] * np.arange(N2)[None, :] / N2
    c, s = np.cos(ph), np.sin(ph)
    f2 = np.zeros((128, 128))
    f2[:N2, 0::2], f2[:N2, 1::2], f2[N2:, 0::2], f2[N2:, 1::2] = c, -s, s, c
    g2 = np.zeros((128, 128))
    g2[0::2, :N2], g2[0::2, N2:], g2[1::2, :N2], g2[1::2, N2:] = c.T, s.T, -s.T, c.T

    def as_words(a):
        u = a.astype(np.float32).astype(BF16).view(np.uint16).astype(np.uint32)
        return u[..., 0::2, :] | (u[..., 1::2, :] << 16)

    return as_words(fwd), as_words(inv), as_words(np.stack([f2, g2]))


def _to_words(x):
    return pltpu.bitcast(x.astype(BF16), U32)


def _from_words(w):
    return pltpu.bitcast(w, BF16)


_CFG = dict(group=8, lag_s=2, lag_v=3, wo_split=16, gate_at=1, late_first=0, late_per_block=10, prep_early=4, b_group=4, n_early=3, n_first=2, unroll=3, chunk_steps=3, first_splits=(16, 26),
            n_pre=9, pre_unroll=16)


def _step_order(n_heads, n_out_tiles, first=False):
    g, a, b = _CFG["group"], _CFG["lag_s"], _CFG["lag_v"]
    split = _CFG["wo_split"]
    n_groups = n_heads // g
    total = n_groups + a + b
    early = [("W", j, 0, split) for j in range(n_out_tiles)] if split < n_heads else []
    ops = []
    for t in range(total):
        if t < n_groups:
            ops += [("P", h) for h in range(t * g, (t + 1) * g)]
        if t == _CFG["gate_at"]:
            ops.append(("G",))
        if 0 <= t - a < n_groups:
            ops += [("S", h) for h in range((t - a) * g, (t - a + 1) * g)]
        if 0 <= t - a - b < n_groups:
            ops += [("V", h) for h in range((t - a - b) * g, (t - a - b + 1) * g)]
        if early and (t - a - b + 1) * g >= split:
            n = -(-len(early) // (total - t))
            ops += early[:n]
            early = early[n:]
    ops += early
    bounds = [split if split < n_heads else 0]
    if first:
        bounds += [b for b in _CFG["first_splits"] if b > split]
    for lo, hi in zip(bounds, bounds[1:] + [n_heads]):
        ops += [("W", j, lo, hi) for j in range(n_out_tiles)]
    return ops


def _dot(a, b):
    return jnp.dot(a, b, preferred_element_type=F32)


def _dot_nt(a, b):
    return jax.lax.dot_general(a, b, (((1,), (1,)), ((), ())), preferred_element_type=F32)


def _make_kernel(n_heads, d_head, d_model, n_mem, seg, n_seg):
    n_rows = n_mem + seg
    n_cb = d_model // CB
    n_hp = n_heads // 2
    scale = d_head ** (-0.5)
    exp_scale = scale * math.log2(math.e)
    steps_per_chunk = _CFG["chunk_steps"]
    x_chunks = (n_seg - 1) // steps_per_chunk
    x_rows = steps_per_chunk * seg
    assert x_chunks * steps_per_chunk == n_seg - 1 and steps_per_chunk % _CFG["unroll"] == 0
    n_pre = _CFG["n_pre"]
    pre_rows = 8
    assert n_pre % steps_per_chunk == 0
    order = _step_order(n_heads, d_model // 128)
    order_first = _step_order(n_heads, d_model // 128, True)
    wo_bounds = [0] + list(_CFG["first_splits"]) + [n_heads]

    def kernel(sh_hbm, d_hbm, mem_hbm,
               x_hbm, wq_hbm, wk_hbm, wv_hbm, wo_hbm,
               q_hbm, k_hbm, v_hbm, h_hbm, tf_hbm, ti_hbm, t2_hbm,
               out_hbm,
               hs, ks, vs, ob, kf, xp, hp, zx, zh, tt, yp, tf, ti, t2, sh_ref, d_ref, mem_ref, sh32, d32,
               stage, wqkv, wo, xin, qin, ost, hbuf, qbuf, kbuf, vbuf, obuf, pbuf, ibuf, ybuf, xpre, xpre32, qkpre,
               sem_b, sem_t, sem_w, sem_o, sem_h, sem_p, sem_x, sem_q, sem_out):

        n_early = _CFG["n_early"]

        def h_copy(cb):
            c0 = cb * CB if isinstance(cb, int) else pl.multiple_of(cb * CB, CB)
            return pltpu.make_async_copy(h_hbm.at[pl.ds(c0, CB), :], hs.at[cb], sem_b.at[0, cb])

        def kv_copies(cb):
            if isinstance(cb, int):
                c0, width = cb * CB, (CB if cb < n_early else d_model - n_early * CB)
            else:
                c0, width = pl.multiple_of(cb * CB, CB), CB
            return [pltpu.make_async_copy(src.at[:, pl.ds(c0, width)], dst.at[:, pl.ds(c0, width)], sem_b.at[1 + i, cb])
                    for i, (src, dst) in enumerate(((k_hbm, ks), (v_hbm, vs)))]

        def t_copies():
            pairs = ((sh_hbm, sh_ref), (d_hbm, d_ref), (mem_hbm, mem_ref),
                     (tf_hbm, tf), (ti_hbm, ti), (t2_hbm, t2))
            return [pltpu.make_async_copy(src, dst, sem_t.at[i]) for i, (src, dst) in enumerate(pairs)]

        def w_copies(m):
            w32 = (wq_hbm, wk_hbm, wv_hbm)[m].bitcast(U32)
            return [pltpu.make_async_copy(w32.at[:, hp, :], stage.at[m * n_hp + hp], sem_w.at[m])
                    for hp in range(n_hp)]

        def o_copies(i):
            wo32 = wo_hbm.bitcast(U32)
            lo, hi = wo_bounds[i] * d_head // 2, wo_bounds[i + 1] * d_head // 2
            return [pltpu.make_async_copy(wo32.at[pl.ds(lo, hi - lo), pl.ds(j * 128, 128)],
                                          wo.at[j, pl.ds(lo, hi - lo), :], sem_o.at[i])
                    for j in range(d_model // 128)]

        def head_copies():
            return [pltpu.make_async_copy(src.at[pl.ds(0, seg), :], dst.at[pl.ds(0, seg), :], sem_h.at[i])
                    for i, (src, dst) in enumerate(((x_hbm, xin), (q_hbm, qin)))]

        def pre_copies():
            return [pltpu.make_async_copy(x_hbm.at[pl.ds((i + 1) * seg, pre_rows), :],
                                          xpre.at[pl.ds(i * pre_rows, pre_rows), :], sem_p) for i in range(n_pre)]

        def chunk_copies(c):
            r0 = seg + c * x_rows if isinstance(c, int) else pl.multiple_of(seg + c * x_rows, seg)
            return [pltpu.make_async_copy(src.at[pl.ds(r0, x_rows), :], dst.at[pl.ds(r0, x_rows), :], sem.at[c])
                    for src, dst, sem in ((x_hbm, xin, sem_x), (q_hbm, qin, sem_q))]

        def out_copy(s):
            r0 = s * seg if isinstance(s, int) else pl.multiple_of(s * seg, seg)
            return pltpu.make_async_copy(ost.at[s], out_hbm.at[pl.ds(r0, seg), :], sem_out)

        for c in t_copies():
            c.start()
        n_first = _CFG["n_first"]
        for cb in range(n_first):
            for c in [h_copy(cb)] + kv_copies(cb):
                c.start()
        second = []
        for cb in range(n_first, n_early):
            second += [h_copy(cb)] + kv_copies(cb)
        late = kv_copies(n_early) + [h_copy(cb) for cb in range(n_early, n_cb)]
        n_b_late = len(late)
        late += w_copies(0) + pre_copies() + w_copies(1) + w_copies(2) + head_copies()
        for i in range(len(wo_bounds) - 1):
            late += o_copies(i)
        per_block = _CFG["late_per_block"]
        first_block = _CFG["late_first"]

        kf[0:8, :] = jnp.zeros((8, CB), F32)

        group = _CFG["b_group"]

        def put(ref, row, x, slot=()):
            ref[(*slot, pl.ds(2 * row, x.shape[0]), slice(None))] = x.astype(BF16)

        def get(ref, row, n, stride=1, slot=()):
            return ref.bitcast(U32)[(*slot, pl.ds(row, n, stride=stride), slice(None))]

        def wait_inputs(cb):
            h_copy(cb).wait()

            @pl.when(cb < n_early)
            def _():
                for c in kv_copies(cb):
                    c.wait()

            @pl.when(cb == n_early)
            def _():
                for c in kv_copies(n_early):
                    c.wait()

        def prepare(cb, slot, piece):
            c0 = pl.multiple_of(cb * CB, CB)
            for j in range(2 * piece, 2 * piece + 2):
                r = hs[cb, :, j * 128:(j + 1) * 128].astype(F32).T
                put(hp, (2 * j) * SP, r[0:N2], (slot,))
                put(hp, (2 * j + 1) * SP, r[N2:2 * N2], (slot,))
            taps = sh32[:, pl.ds(c0, CB)]
            for n1 in range(4 * piece, 4 * piece + 4):
                kf[pl.ds(8 + n1 * N2, N2), :] = ks[pl.ds(n1 * N2, N2), pl.ds(c0, CB)].astype(F32)
                acc = kf[pl.ds(8 + n1 * N2, N2), :] * taps[0:1]
                for i in range(1, 4):
                    acc = acc + kf[pl.ds(8 - i + n1 * N2, N2), :] * taps[i:i + 1]
                put(xp, n1 * SP, acc * vs[pl.ds(n1 * N2, N2), pl.ds(c0, CB)].astype(F32), (slot,))

        def finish(cb, slot, piece):
            dv = d32[pl.ds(cb, 1), :]
            for n1 in range(4 * piece, 4 * piece + 4):
                kv = _from_words(get(xp, n1 * SP, N2 // 2, 1, (slot,))).astype(F32)
                ob[cb, pl.ds(n1 * N2, N2), :] = (yp[pl.ds(n1 * SY, N2), :] + kv * dv).astype(BF16)

        def b_block(cb, carry):
            @pl.when(cb + 1 < n_cb)
            def _():
                wait_inputs(cb + 1)

            for i in range(n_cb - first_block):
                @pl.when(cb == i + first_block)
                def _(i=i):
                    lo = 0 if i == 0 else n_b_late + i * per_block
                    for c in late[lo:n_b_late + (i + 1) * per_block]:
                        c.start()
            lane = jax.lax.broadcasted_iota(jnp.int32, (1, 128), 1)
            slot = cb % 2
            nxt = jnp.minimum(cb + 1, n_cb - 1)
            prv = jnp.maximum(cb - 1, 0)
            n_pieces = 8

            def side_work(piece):
                finish(prv, 1 - slot, piece)
                prepare(nxt, 1 - slot, piece)

            early_pieces = _CFG["prep_early"]
            for g in range(N2 // 4):
                m = tf[g]
                lhs = _from_words(jnp.concatenate(
                    [jnp.where((lane // 64 == j // 2) & (lane % 2 == j % 2), m, jnp.zeros_like(m))
                     for j in range(4)], axis=0))

                def rhs(ref, g=g):
                    return _from_words(jnp.concatenate(
                        [get(ref, 2 * g, N1, SP, (slot,)), get(ref, 2 * g + 1, N1, SP, (slot,))], axis=0))

                r = _dot(lhs, jnp.concatenate([rhs(xp), rhs(hp)], axis=1))
                for j in range(4):
                    put(zx, (4 * g + j) * SZ, r[2 * N1 * j:2 * N1 * (j + 1), :128])
                    put(zh, (4 * g + j) * SZ, r[2 * N1 * j:2 * N1 * (j + 1), 128:])
                if early_pieces and g % (16 // early_pieces) == 0:
                    side_work(g // (16 // early_pieces))
            f2 = _from_words(t2[0])
            g2 = _from_words(t2[1])

            def stage2(g):
                zz = []
                for k1 in range(g * group, (g + 1) * group):
                    zz += [_from_words(get(zx, k1, N2, SZ)), _from_words(get(zh, k1, N2, SZ))]
                return _dot(f2, jnp.concatenate(zz, axis=1))

            def stage3(g, r):
                ys = []
                for i in range(group):
                    xf = r[:, (2 * i) * 128:(2 * i + 1) * 128]
                    hf = r[:, (2 * i + 1) * 128:(2 * i + 2) * 128]
                    xr, xi, hr, hi = xf[:N2], xf[N2:], hf[:N2], hf[N2:]
                    ys.append(jnp.concatenate([xr * hr - xi * hi, xr * hi + xi * hr], axis=0).astype(BF16))
                t = _dot(g2, jnp.concatenate(ys, axis=1))
                for i in range(group):
                    put(tt, (g * group + i) * ST, t[:, i * 128:(i + 1) * 128])

            n_groups = N1 // group
            late_pieces = list(range(early_pieces, n_pieces))
            r = stage2(0)
            for g in range(n_groups):
                r_next = stage2(g + 1) if g + 1 < n_groups else None
                stage3(g, r)
                r = r_next
                for piece in late_pieces[g::n_groups]:
                    side_work(piece)
            for i in range(N2 // 2):
                m = ti[i]
                lhs = _from_words(jnp.concatenate([jnp.where(lane < 64, m, jnp.zeros_like(m)),
                                                   jnp.where(lane >= 64, m, jnp.zeros_like(m))], axis=0))
                y = _dot(lhs, _from_words(jnp.concatenate(
                    [get(tt, 2 * i, N1, ST), get(tt, 2 * i + 1, N1, ST)], axis=0)))
                yp[pl.ds(2 * i, N1, stride=SY), :] = y[0:N1]
                yp[pl.ds(2 * i + 1, N1, stride=SY), :] = y[N1:2 * N1]
            return carry

        for c in t_copies():
            c.wait()
        sh32[...] = sh_ref[...].astype(F32)
        d32[...] = d_ref[...].astype(F32)
        hbuf[0:n_mem, :] = mem_ref[...].astype(F32)
        wait_inputs(0)
        for c in second:
            c.start()
        for piece in range(8):
            prepare(0, 0, piece)
        jax.lax.fori_loop(0, n_cb, b_block, 0)
        for c in late[n_b_late + (n_cb - first_block) * per_block:]:
            c.start()
        for piece in range(8):
            finish(n_cb - 1, (n_cb - 1) % 2, piece)

        def wtile(ref, i):
            return _from_words(ref[i])

        def precompute():
            per = _CFG["pre_unroll"]

            def body(i, carry):
                xl = xpre32[...]
                for u in range(per):
                    h = i * per + u
                    for m in range(2):
                        qkpre[m, h] = _dot(xl, wtile(wqkv, 3 * h + m))
                return carry

            jax.lax.fori_loop(0, n_heads // per, body, 0)

        for m in range(3):
            if m == 2 and n_pre:
                for c in pre_copies():
                    c.wait()
                xpre32[...] = xpre[...].astype(F32)
                precompute()
            for c in w_copies(m):
                c.wait()

            def relayout(hp, carry, m=m):
                even = stage[m * n_hp + hp, pl.ds(0, d_model // 2, stride=2), :]
                odd = stage[m * n_hp + hp, pl.ds(1, d_model // 2, stride=2), :]
                wqkv[(2 * hp) * 3 + m] = (even & U32(0xFFFF)) | (odd << 16)
                wqkv[(2 * hp + 1) * 3 + m] = (even >> 16) | (odd & U32(0xFFFF0000))
                return carry

            jax.lax.fori_loop(0, n_hp, relayout, 0)

        def step(s, first, pre=False):
            if first:
                for c in head_copies():
                    c.wait()
            row = jax.lax.broadcasted_iota(jnp.int32, (n_rows, n_rows), 0)
            col = jax.lax.broadcasted_iota(jnp.int32, (n_rows, n_rows), 1)
            mask = (row < n_mem) | (row >= col)
            r0 = s * seg if first else pl.multiple_of(s * seg, seg)
            slot = s
            hbuf[n_mem:n_rows, :] = xin[pl.ds(r0, seg), :].astype(F32)
            hl = hbuf[...]
            if pre:
                hr = jnp.concatenate([hl[0:n_mem], hl[n_mem + pre_rows:n_rows]], axis=0)
                p0 = pl.multiple_of((s - 1) * pre_rows, pre_rows)
            waited = [False] * (len(wo_bounds) - 1)
            for op in (order_first if first else order):
                if op[0] == "P":
                    h = op[1]
                    if pre:
                        rq = _dot(hr, wtile(wqkv, 3 * h))
                        qbuf[h] = jnp.concatenate(
                            [rq[0:n_mem], qkpre[0, h, pl.ds(p0, pre_rows), :], rq[n_mem:]], axis=0)
                        rk = _dot(hr, wtile(wqkv, 3 * h + 1))
                        kbuf[h, 0:n_rows] = jnp.concatenate(
                            [rk[0:n_mem], qkpre[1, h, pl.ds(p0, pre_rows), :], rk[n_mem:]], axis=0).astype(BF16)
                    else:
                        qbuf[h] = _dot(hl, wtile(wqkv, 3 * h))
                        kbuf[h, 0:n_rows] = _dot(hl, wtile(wqkv, 3 * h + 1)).astype(BF16)
                    vbuf[h, 0:n_rows] = _dot(hl, wtile(wqkv, 3 * h + 2)).astype(BF16)
                elif op[0] == "S":
                    h = op[1]
                    sc = _dot_nt(qbuf[h], kbuf[h, 0:n_rows])
                    sc = jnp.where(mask, sc, -1e9 / scale)
                    e = jnp.exp2((sc - jnp.max(sc, axis=-1, keepdims=True)) * exp_scale)
                    den = jnp.sum(e, axis=-1, keepdims=True)
                    inv = pl.reciprocal(den, approx=True)
                    pbuf[h, :, 0:n_rows] = e
                    ibuf[h] = jnp.broadcast_to(inv * (2.0 - den * inv), (n_rows, d_head))
                elif op[0] == "V":
                    h = op[1]
                    obuf[:, h * d_head:(h + 1) * d_head] = (
                        _dot(pbuf[h, :, 0:n_rows], vbuf[h, 0:n_rows]) * ibuf[h])
                elif op[0] == "W":
                    _, j, lo, hi = op
                    if first:
                        for i in range(len(waited)):
                            if not waited[i] and hi > wo_bounds[i]:
                                for c in o_copies(i):
                                    c.wait()
                                waited[i] = True
                                if i == len(waited) - 1:
                                    for ch in range(x_chunks):
                                        for c in chunk_copies(ch):
                                            c.start()
                    w = _from_words(wo[j, lo * d_head // 2:hi * d_head // 2, :])
                    y = _dot(obuf[:, lo * d_head:hi * d_head], w)
                    if lo > 0:
                        y = y + ybuf[j]
                    if hi < n_heads:
                        ybuf[j] = y
                    else:
                        hbuf[0:n_mem, j * 128:(j + 1) * 128] = y[0:n_mem]
                        ost[slot, :, j * 128:(j + 1) * 128] = y[n_mem:n_rows].astype(BF16)
                else:
                    for cb in range(n_cb):
                        gate = qin[pl.ds(r0, seg), cb * CB:(cb + 1) * CB].astype(F32)
                        ost[slot, :, d_model + cb * CB:d_model + (cb + 1) * CB] = (
                            ob[cb, pl.ds(r0, seg), :].astype(F32) * gate).astype(BF16)
            out_copy(s).start()

        unroll = _CFG["unroll"]

        def chunk_body(c, carry, pre=False):
            for cp in chunk_copies(c):
                cp.wait()

            def steps_body(i, carry):
                for u in range(unroll):
                    step(1 + c * steps_per_chunk + i * unroll + u, False, pre)
                return carry

            if steps_per_chunk == unroll:
                steps_body(0, 0)
            else:
                jax.lax.fori_loop(0, steps_per_chunk // unroll, steps_body, 0)
            return carry

        step(0, True)
        pre_chunks = n_pre // steps_per_chunk
        if pre_chunks:
            jax.lax.fori_loop(0, pre_chunks, functools.partial(chunk_body, pre=True), 0)
        jax.lax.fori_loop(pre_chunks, x_chunks, chunk_body, 0)
        for s in range(n_seg):
            out_copy(s).wait()

    return kernel


def _forward(x, mem0, wq, wk, wv, wo, seg_len, q, k, v, shift_k, ssm_k, ssm_d):
    _, seq, d_model = x.shape
    _, n_heads, d_head = wq.shape
    n_mem = mem0.shape[1]
    seg = seg_len
    n_seg = seq // seg
    n_rows = n_mem + seg
    n_cb = d_model // CB
    assert seq == SEQ and d_model == 1024 and d_head == 128 and n_rows % 8 == 0
    tf, ti, t2 = _dft_tables()

    any_spec = pl.BlockSpec(memory_space=pl.ANY)
    kv_rows = -(-n_rows // 16) * 16
    scratch = [
        pltpu.VMEM((n_cb, CB, seq), BF16),
        pltpu.VMEM((seq, d_model), BF16),
        pltpu.VMEM((seq, d_model), BF16),
        pltpu.VMEM((n_cb, seq, CB), BF16),
        pltpu.VMEM((8 + seq, CB), F32),
        pltpu.VMEM((2, 2 * N1 * SP, CB), BF16),
        pltpu.VMEM((2, 2 * N1 * SP, CB), BF16),
        pltpu.VMEM((2 * N2 * SZ, CB), BF16),
        pltpu.VMEM((2 * N2 * SZ, CB), BF16),
        pltpu.VMEM((2 * N1 * ST, CB), BF16),
        pltpu.VMEM((N1 * SY, CB), F32),
        pltpu.VMEM(tf.shape, U32),
        pltpu.VMEM(ti.shape, U32),
        pltpu.VMEM(t2.shape, U32),
        pltpu.VMEM((4, d_model), BF16),
        pltpu.VMEM((n_cb, CB), BF16),
        pltpu.VMEM((n_mem, d_model), BF16),
        pltpu.VMEM((4, d_model), F32),
        pltpu.VMEM((n_cb, CB), F32),
        pltpu.VMEM((3 * n_heads // 2, d_model, d_head), U32),
        pltpu.VMEM((3 * n_heads, d_model // 2, d_head), U32),
        pltpu.VMEM((d_model // 128, n_heads * d_head // 2, 128), U32),
        pltpu.VMEM((seq, d_model), BF16),
        pltpu.VMEM((seq, d_model), BF16),
        pltpu.VMEM((n_seg, seg, 2 * d_model), BF16),
        pltpu.VMEM((n_rows, d_model), F32),
        pltpu.VMEM((n_heads, n_rows, d_head), F32),
        pltpu.VMEM((n_heads, kv_rows, d_head), BF16),
        pltpu.VMEM((n_heads, kv_rows, d_head), BF16),
        pltpu.VMEM((n_rows, n_heads * d_head), F32),
        pltpu.VMEM((n_heads, n_rows, d_head), F32),
        pltpu.VMEM((n_heads, n_rows, d_head), F32),
        pltpu.VMEM((d_model // 128, n_rows, 128), F32),
        pltpu.VMEM((max(_CFG["n_pre"], 2) * 8, d_model), BF16),
        pltpu.VMEM((max(_CFG["n_pre"], 2) * 8, d_model), F32),
        pltpu.VMEM((2, n_heads, max(_CFG["n_pre"], 2) * 8, d_head), F32),
        pltpu.SemaphoreType.DMA((3, n_cb)),
        pltpu.SemaphoreType.DMA((6,)),
        pltpu.SemaphoreType.DMA((3,)),
        pltpu.SemaphoreType.DMA((len(_CFG["first_splits"]) + 1,)),
        pltpu.SemaphoreType.DMA((2,)),
        pltpu.SemaphoreType.DMA(()),
        pltpu.SemaphoreType.DMA((n_seg,)),
        pltpu.SemaphoreType.DMA((n_seg,)),
        pltpu.SemaphoreType.DMA(()),
    ]
    out = pl.pallas_call(
        _make_kernel(n_heads, d_head, d_model, n_mem, seg, n_seg),
        out_shape=jax.ShapeDtypeStruct((seq, 2 * d_model), BF16),
        in_specs=[any_spec] * 15,
        out_specs=any_spec,
        scratch_shapes=scratch,
        compiler_params=pltpu.CompilerParams(vmem_limit_bytes=120 * 1024 * 1024),
    )(shift_k.T, ssm_d.reshape(n_cb, CB), mem0.reshape(n_mem, d_model),
      x.reshape(seq, d_model), wq, wk, wv, wo.reshape(n_heads * d_head, d_model),
      q.reshape(seq, d_model), k.reshape(seq, d_model), v.reshape(seq, d_model), ssm_k,
      tf, ti, t2)
    return out.reshape(1, seq, 2 * d_model)


def pallas_concat_heads__memory_aug_recurrent_mem_tr__ssm_conv_h3__prompt_kernel(
        A_x, A_mem0, A_Wq, A_Wk, A_Wv, A_Wo, A_seg_len, B_q, B_k, B_v, B_shift_k, B_ssm_k, B_ssm_D):
    return _forward(A_x, A_mem0, A_Wq, A_Wk, A_Wv, A_Wo, int(A_seg_len), B_q, B_k, B_v,
                    B_shift_k, B_ssm_k, B_ssm_D)
```

```python
import functools
import math

import jax
import jax.numpy as jnp
import numpy as np
from jax.experimental import pallas as pl
from jax.experimental.pallas import tpu as pltpu

F32 = jnp.float32
BF16 = jnp.bfloat16
U32 = jnp.uint32

N1, N2 = 32, 64
SEQ = N1 * N2
SP = N2 // 2 + 4
SZ = N1 + 4
ST = N2 + 4
SY = N2 + 4
CB = 128


def _dft_tables():
    theta = np.pi / (2 * SEQ)
    lane = np.arange(128)[None, :]
    hi, mid, lo = lane // 64, (lane % 64) // 2, lane % 2
    k1 = np.arange(N1)[:, None]
    fwd = np.zeros((N2 // 4, 2 * N1, 128))
    for g in range(N2 // 4):
        ph = theta * (4 * k1 + 1) * (N2 * mid + 4 * g + 2 * hi + lo)
        fwd[g, 0::2] = np.cos(ph)
        fwd[g, 1::2] = np.sin(ph)
    n1 = np.arange(N1)[:, None]
    inv = np.zeros((N2 // 2, N1, 128))
    for i in range(N2 // 2):
        ph = theta * (4 * mid + 1) * (N2 * n1 + 2 * i + hi)
        inv[i] = np.where(lo == 0, np.cos(ph), np.sin(ph)) / SEQ
    ph = 2 * np.pi * np.arange(N2)[:, None] * np.arange(N2)[None, :] / N2
    c, s = np.cos(ph), np.sin(ph)
    f2 = np.zeros((128, 128))
    f2[:N2, 0::2], f2[:N2, 1::2], f2[N2:, 0::2], f2[N2:, 1::2] = c, -s, s, c
    g2 = np.zeros((128, 128))
    g2[0::2, :N2], g2[0::2, N2:], g2[1::2, :N2], g2[1::2, N2:] = c.T, s.T, -s.T, c.T

    def as_words(a):
        u = a.astype(np.float32).astype(BF16).view(np.uint16).astype(np.uint32)
        return u[..., 0::2, :] | (u[..., 1::2, :] << 16)

    return as_words(fwd), as_words(inv), as_words(np.stack([f2, g2]))


def _to_words(x):
    return pltpu.bitcast(x.astype(BF16), U32)


def _from_words(w):
    return pltpu.bitcast(w, BF16)


_CFG = dict(group=8, lag_s=2, lag_v=3, wo_split=16, gate_at=1, late_first=0, late_per_block=10, prep_early=4, b_group=4, n_early=3, n_first=2, unroll=3, chunk_steps=3, first_splits=(16, 26),
            n_pre=9, pre_unroll=4, pre_rolled=1)


def _step_order(n_heads, n_out_tiles, first=False):
    g, a, b = _CFG["group"], _CFG["lag_s"], _CFG["lag_v"]
    split = _CFG["wo_split"]
    n_groups = n_heads // g
    total = n_groups + a + b
    early = [("W", j, 0, split) for j in range(n_out_tiles)] if split < n_heads else []
    ops = []
    for t in range(total):
        if t < n_groups:
            ops += [("P", h) for h in range(t * g, (t + 1) * g)]
        if t == _CFG["gate_at"]:
            ops.append(("G",))
        if 0 <= t - a < n_groups:
            ops += [("S", h) for h in range((t - a) * g, (t - a + 1) * g)]
        if 0 <= t - a - b < n_groups:
            ops += [("V", h) for h in range((t - a - b) * g, (t - a - b + 1) * g)]
        if early and (t - a - b + 1) * g >= split:
            n = -(-len(early) // (total - t))
            ops += early[:n]
            early = early[n:]
    ops += early
    bounds = [split if split < n_heads else 0]
    if first:
        bounds += [b for b in _CFG["first_splits"] if b > split]
    for lo, hi in zip(bounds, bounds[1:] + [n_heads]):
        ops += [("W", j, lo, hi) for j in range(n_out_tiles)]
    return ops


def _dot(a, b):
    return jnp.dot(a, b, preferred_element_type=F32)


def _dot_nt(a, b):
    return jax.lax.dot_general(a, b, (((1,), (1,)), ((), ())), preferred_element_type=F32)


def _make_kernel(n_heads, d_head, d_model, n_mem, seg, n_seg):
    n_rows = n_mem + seg
    n_cb = d_model // CB
    n_hp = n_heads // 2
    scale = d_head ** (-0.5)
    exp_scale = scale * math.log2(math.e)
    steps_per_chunk = _CFG["chunk_steps"]
    x_chunks = (n_seg - 1) // steps_per_chunk
    x_rows = steps_per_chunk * seg
    assert x_chunks * steps_per_chunk == n_seg - 1 and steps_per_chunk % _CFG["unroll"] == 0
    n_pre = _CFG["n_pre"]
    pre_rows = 8
    assert n_pre % steps_per_chunk == 0
    order = _step_order(n_heads, d_model // 128)
    order_first = _step_order(n_heads, d_model // 128, True)
    wo_bounds = [0] + list(_CFG["first_splits"]) + [n_heads]

    def kernel(sh_hbm, d_hbm, mem_hbm,
               x_hbm, wq_hbm, wk_hbm, wv_hbm, wo_hbm,
               q_hbm, k_hbm, v_hbm, h_hbm, tf_hbm, ti_hbm, t2_hbm,
               out_hbm,
               hs, ks, vs, ob, kf, xp, hp, zx, zh, tt, yp, tf, ti, t2, sh_ref, d_ref, mem_ref, sh32, d32,
               stage, wqkv, wo, xin, qin, ost, hbuf, qbuf, kbuf, vbuf, obuf, pbuf, ibuf, ybuf, xpre, xpre32, qkpre,
               sem_b, sem_t, sem_w, sem_o, sem_h, sem_p, sem_x, sem_q, sem_out):

        n_early = _CFG["n_early"]

        def h_copy(cb):
            c0 = cb * CB if isinstance(cb, int) else pl.multiple_of(cb * CB, CB)
            return pltpu.make_async_copy(h_hbm.at[pl.ds(c0, CB), :], hs.at[cb], sem_b.at[0, cb])

        def kv_copies(cb):
            if isinstance(cb, int):
                c0, width = cb * CB, (CB if cb < n_early else d_model - n_early * CB)
            else:
                c0, width = pl.multiple_of(cb * CB, CB), CB
            return [pltpu.make_async_copy(src.at[:, pl.ds(c0, width)], dst.at[:, pl.ds(c0, width)], sem_b.at[1 + i, cb])
                    for i, (src, dst) in enumerate(((k_hbm, ks), (v_hbm, vs)))]

        def t_copies():
            pairs = ((sh_hbm, sh_ref), (d_hbm, d_ref), (mem_hbm, mem_ref),
                     (tf_hbm, tf), (ti_hbm, ti), (t2_hbm, t2))
            return [pltpu.make_async_copy(src, dst, sem_t.at[i]) for i, (src, dst) in enumerate(pairs)]

        def w_copies(m):
            w32 = (wq_hbm, wk_hbm, wv_hbm)[m].bitcast(U32)
            return [pltpu.make_async_copy(w32.at[:, hp, :], stage.at[m * n_hp + hp], sem_w.at[m])
                    for hp in range(n_hp)]

        def o_copies(i):
            wo32 = wo_hbm.bitcast(U32)
            lo, hi = wo_bounds[i] * d_head // 2, wo_bounds[i + 1] * d_head // 2
            return [pltpu.make_async_copy(wo32.at[pl.ds(lo, hi - lo), pl.ds(j * 128, 128)],
                                          wo.at[j, pl.ds(lo, hi - lo), :], sem_o.at[i])
                    for j in range(d_model // 128)]

        def head_copies():
            return [pltpu.make_async_copy(src.at[pl.ds(0, seg), :], dst.at[pl.ds(0, seg), :], sem_h.at[i])
                    for i, (src, dst) in enumerate(((x_hbm, xin), (q_hbm, qin)))]

        def pre_copies():
            return [pltpu.make_async_copy(x_hbm.at[pl.ds((i + 1) * seg, pre_rows), :],
                                          xpre.at[pl.ds(i * pre_rows, pre_rows), :], sem_p) for i in range(n_pre)]

        def chunk_copies(c):
            r0 = seg + c * x_rows if isinstance(c, int) else pl.multiple_of(seg + c * x_rows, seg)
            return [pltpu.make_async_copy(src.at[pl.ds(r0, x_rows), :], dst.at[pl.ds(r0, x_rows), :], sem.at[c])
                    for src, dst, sem in ((x_hbm, xin, sem_x), (q_hbm, qin, sem_q))]

        def out_copy(s):
            r0 = s * seg if isinstance(s, int) else pl.multiple_of(s * seg, seg)
            return pltpu.make_async_copy(ost.at[s], out_hbm.at[pl.ds(r0, seg), :], sem_out)

        for c in t_copies():
            c.start()
        n_first = _CFG["n_first"]
        for cb in range(n_first):
            for c in [h_copy(cb)] + kv_copies(cb):
                c.start()
        second = []
        for cb in range(n_first, n_early):
            second += [h_copy(cb)] + kv_copies(cb)
        late = kv_copies(n_early) + [h_copy(cb) for cb in range(n_early, n_cb)]
        n_b_late = len(late)
        late += w_copies(0) + pre_copies() + w_copies(1) + w_copies(2) + head_copies()
        for i in range(len(wo_bounds) - 1):
            late += o_copies(i)
        per_block = _CFG["late_per_block"]
        first_block = _CFG["late_first"]

        kf[0:8, :] = jnp.zeros((8, CB), F32)

        group = _CFG["b_group"]

        def put(ref, row, x, slot=()):
            ref[(*slot, pl.ds(2 * row, x.shape[0]), slice(None))] = x.astype(BF16)

        def get(ref, row, n, stride=1, slot=()):
            return ref.bitcast(U32)[(*slot, pl.ds(row, n, stride=stride), slice(None))]

        def wait_inputs(cb):
            h_copy(cb).wait()

            @pl.when(cb < n_early)
            def _():
                for c in kv_copies(cb):
                    c.wait()

            @pl.when(cb == n_early)
            def _():
                for c in kv_copies(n_early):
                    c.wait()

        def prepare(cb, slot, piece):
            c0 = pl.multiple_of(cb * CB, CB)
            for j in range(2 * piece, 2 * piece + 2):
                r = hs[cb, :, j * 128:(j + 1) * 128].astype(F32).T
                put(hp, (2 * j) * SP, r[0:N2], (slot,))
                put(hp, (2 * j + 1) * SP, r[N2:2 * N2], (slot,))
            taps = sh32[:, pl.ds(c0, CB)]
            for n1 in range(4 * piece, 4 * piece + 4):
                kf[pl.ds(8 + n1 * N2, N2), :] = ks[pl.ds(n1 * N2, N2), pl.ds(c0, CB)].astype(F32)
                acc = kf[pl.ds(8 + n1 * N2, N2), :] * taps[0:1]
                for i in range(1, 4):
                    acc = acc + kf[pl.ds(8 - i + n1 * N2, N2), :] * taps[i:i + 1]
                put(xp, n1 * SP, acc * vs[pl.ds(n1 * N2, N2), pl.ds(c0, CB)].astype(F32), (slot,))

        def finish(cb, slot, piece):
            dv = d32[pl.ds(cb, 1), :]
            for n1 in range(4 * piece, 4 * piece + 4):
                kv = _from_words(get(xp, n1 * SP, N2 // 2, 1, (slot,))).astype(F32)
                ob[cb, pl.ds(n1 * N2, N2), :] = (yp[pl.ds(n1 * SY, N2), :] + kv * dv).astype(BF16)

        def b_block(cb, carry):
            @pl.when(cb + 1 < n_cb)
            def _():
                wait_inputs(cb + 1)

            for i in range(n_cb - first_block):
                @pl.when(cb == i + first_block)
                def _(i=i):
                    lo = 0 if i == 0 else n_b_late + i * per_block
                    for c in late[lo:n_b_late + (i + 1) * per_block]:
                        c.start()
            lane = jax.lax.broadcasted_iota(jnp.int32, (1, 128), 1)
            slot = cb % 2
            nxt = jnp.minimum(cb + 1, n_cb - 1)
            prv = jnp.maximum(cb - 1, 0)
            n_pieces = 8

            def side_work(piece):
                finish(prv, 1 - slot, piece)
                prepare(nxt, 1 - slot, piece)

            early_pieces = _CFG["prep_early"]
            for g in range(N2 // 4):
                m = tf[g]
                lhs = _from_words(jnp.concatenate(
                    [jnp.where((lane // 64 == j // 2) & (lane % 2 == j % 2), m, jnp.zeros_like(m))
                     for j in range(4)], axis=0))

                def rhs(ref, g=g):
                    return _from_words(jnp.concatenate(
                        [get(ref, 2 * g, N1, SP, (slot,)), get(ref, 2 * g + 1, N1, SP, (slot,))], axis=0))

                r = _dot(lhs, jnp.concatenate([rhs(xp), rhs(hp)], axis=1))
                for j in range(4):
                    put(zx, (4 * g + j) * SZ, r[2 * N1 * j:2 * N1 * (j + 1), :128])
                    put(zh, (4 * g + j) * SZ, r[2 * N1 * j:2 * N1 * (j + 1), 128:])
                if early_pieces and g % (16 // early_pieces) == 0:
                    side_work(g // (16 // early_pieces))
            f2 = _from_words(t2[0])
            g2 = _from_words(t2[1])

            def stage2(g):
                zz = []
                for k1 in range(g * group, (g + 1) * group):
                    zz += [_from_words(get(zx, k1, N2, SZ)), _from_words(get(zh, k1, N2, SZ))]
                return _dot(f2, jnp.concatenate(zz, axis=1))

            def stage3(g, r):
                ys = []
                for i in range(group):
                    xf = r[:, (2 * i) * 128:(2 * i + 1) * 128]
                    hf = r[:, (2 * i + 1) * 128:(2 * i + 2) * 128]
                    xr, xi, hr, hi = xf[:N2], xf[N2:], hf[:N2], hf[N2:]
                    ys.append(jnp.concatenate([xr * hr - xi * hi, xr * hi + xi * hr], axis=0).astype(BF16))
                t = _dot(g2, jnp.concatenate(ys, axis=1))
                for i in range(group):
                    put(tt, (g * group + i) * ST, t[:, i * 128:(i + 1) * 128])

            n_groups = N1 // group
            late_pieces = list(range(early_pieces, n_pieces))
            r = stage2(0)
            for g in range(n_groups):
                r_next = stage2(g + 1) if g + 1 < n_groups else None
                stage3(g, r)
                r = r_next
                for piece in late_pieces[g::n_groups]:
                    side_work(piece)
            for i in range(N2 // 2):
                m = ti[i]
                lhs = _from_words(jnp.concatenate([jnp.where(lane < 64, m, jnp.zeros_like(m)),
                                                   jnp.where(lane >= 64, m, jnp.zeros_like(m))], axis=0))
                y = _dot(lhs, _from_words(jnp.concatenate(
                    [get(tt, 2 * i, N1, ST), get(tt, 2 * i + 1, N1, ST)], axis=0)))
                yp[pl.ds(2 * i, N1, stride=SY), :] = y[0:N1]
                yp[pl.ds(2 * i + 1, N1, stride=SY), :] = y[N1:2 * N1]
            return carry

        for c in t_copies():
            c.wait()
        sh32[...] = sh_ref[...].astype(F32)
        d32[...] = d_ref[...].astype(F32)
        hbuf[0:n_mem, :] = mem_ref[...].astype(F32)
        wait_inputs(0)
        for c in second:
            c.start()
        for piece in range(8):
            prepare(0, 0, piece)
        jax.lax.fori_loop(0, n_cb, b_block, 0)
        for c in late[n_b_late + (n_cb - first_block) * per_block:]:
            c.start()
        for piece in range(8):
            finish(n_cb - 1, (n_cb - 1) % 2, piece)

        def wtile(ref, i):
            return _from_words(ref[i])

        def precompute():
            per = _CFG["pre_unroll"]

            def body(i, carry):
                xl = xpre32[...]
                for u in range(per):
                    h = i * per + u
                    for m in range(2):
                        qkpre[m, h] = _dot(xl, wtile(wqkv, 3 * h + m))
                return carry

            jax.lax.fori_loop(0, n_heads // per, body, 0)

        for m in range(3):
            if m == 2 and n_pre:
                for c in pre_copies():
                    c.wait()
                xpre32[...] = xpre[...].astype(F32)
                precompute()
            for c in w_copies(m):
                c.wait()

            def relayout(hp, carry, m=m):
                even = stage[m * n_hp + hp, pl.ds(0, d_model // 2, stride=2), :]
                odd = stage[m * n_hp + hp, pl.ds(1, d_model // 2, stride=2), :]
                wqkv[(2 * hp) * 3 + m] = (even & U32(0xFFFF)) | (odd << 16)
                wqkv[(2 * hp + 1) * 3 + m] = (even >> 16) | (odd & U32(0xFFFF0000))
                return carry

            jax.lax.fori_loop(0, n_hp, relayout, 0)

        def step(s, first, pre=False):
            if first:
                for c in head_copies():
                    c.wait()
            row = jax.lax.broadcasted_iota(jnp.int32, (n_rows, n_rows), 0)
            col = jax.lax.broadcasted_iota(jnp.int32, (n_rows, n_rows), 1)
            mask = (row < n_mem) | (row >= col)
            r0 = s * seg if first else pl.multiple_of(s * seg, seg)
            slot = s
            hbuf[n_mem:n_rows, :] = xin[pl.ds(r0, seg), :].astype(F32)
            hl = hbuf[...]
            if pre:
                hr = jnp.concatenate([hl[0:n_mem], hl[n_mem + pre_rows:n_rows]], axis=0)
                p0 = pl.multiple_of((s - 1) * pre_rows, pre_rows)
            waited = [False] * (len(wo_bounds) - 1)
            for op in (order_first if first else order):
                if op[0] == "P":
                    h = op[1]
                    if pre:
                        rq = _dot(hr, wtile(wqkv, 3 * h))
                        qbuf[h] = jnp.concatenate(
                            [rq[0:n_mem], qkpre[0, h, pl.ds(p0, pre_rows), :], rq[n_mem:]], axis=0)
                        rk = _dot(hr, wtile(wqkv, 3 * h + 1))
                        kbuf[h, 0:n_rows] = jnp.concatenate(
                            [rk[0:n_mem], qkpre[1, h, pl.ds(p0, pre_rows), :], rk[n_mem:]], axis=0).astype(BF16)
                    else:
                        qbuf[h] = _dot(hl, wtile(wqkv, 3 * h))
                        kbuf[h, 0:n_rows] = _dot(hl, wtile(wqkv, 3 * h + 1)).astype(BF16)
                    vbuf[h, 0:n_rows] = _dot(hl, wtile(wqkv, 3 * h + 2)).astype(BF16)
                elif op[0] == "S":
                    h = op[1]
                    sc = _dot_nt(qbuf[h], kbuf[h, 0:n_rows])
                    sc = jnp.where(mask, sc, -1e9 / scale)
                    e = jnp.exp2((sc - jnp.max(sc, axis=-1, keepdims=True)) * exp_scale)
                    den = jnp.sum(e, axis=-1, keepdims=True)
                    inv = pl.reciprocal(den, approx=True)
                    pbuf[h, :, 0:n_rows] = e
                    ibuf[h] = jnp.broadcast_to(inv * (2.0 - den * inv), (n_rows, d_head))
                elif op[0] == "V":
                    h = op[1]
                    obuf[:, h * d_head:(h + 1) * d_head] = (
                        _dot(pbuf[h, :, 0:n_rows], vbuf[h, 0:n_rows]) * ibuf[h])
                elif op[0] == "W":
                    _, j, lo, hi = op
                    if first:
                        for i in range(len(waited)):
                            if not waited[i] and hi > wo_bounds[i]:
                                for c in o_copies(i):
                                    c.wait()
                                waited[i] = True
                                if i == len(waited) - 1:
                                    for ch in range(x_chunks):
                                        for c in chunk_copies(ch):
                                            c.start()
                    w = _from_words(wo[j, lo * d_head // 2:hi * d_head // 2, :])
                    y = _dot(obuf[:, lo * d_head:hi * d_head], w)
                    if lo > 0:
                        y = y + ybuf[j]
                    if hi < n_heads:
                        ybuf[j] = y
                    else:
                        hbuf[0:n_mem, j * 128:(j + 1) * 128] = y[0:n_mem]
                        ost[slot, :, j * 128:(j + 1) * 128] = y[n_mem:n_rows].astype(BF16)
                else:
                    for cb in range(n_cb):
                        gate = qin[pl.ds(r0, seg), cb * CB:(cb + 1) * CB].astype(F32)
                        ost[slot, :, d_model + cb * CB:d_model + (cb + 1) * CB] = (
                            ob[cb, pl.ds(r0, seg), :].astype(F32) * gate).astype(BF16)
            out_copy(s).start()

        unroll = _CFG["unroll"]

        def chunk_body(c, carry, pre=False):
            for cp in chunk_copies(c):
                cp.wait()

            def steps_body(i, carry):
                for u in range(unroll):
                    step(1 + c * steps_per_chunk + i * unroll + u, False, pre)
                return carry

            if steps_per_chunk == unroll:
                steps_body(0, 0)
            else:
                jax.lax.fori_loop(0, steps_per_chunk // unroll, steps_body, 0)
            return carry

        step(0, True)
        def pre_step(s, carry):
            @pl.when((s - 1) % steps_per_chunk == 0)
            def _():
                for cp in chunk_copies((s - 1) // steps_per_chunk):
                    cp.wait()

            step(s, False, True)
            return carry

        pre_chunks = n_pre // steps_per_chunk
        if pre_chunks and _CFG["pre_rolled"]:
            jax.lax.fori_loop(1, 1 + n_pre, pre_step, 0)
        elif pre_chunks:
            jax.lax.fori_loop(0, pre_chunks, functools.partial(chunk_body, pre=True), 0)
        jax.lax.fori_loop(pre_chunks, x_chunks, chunk_body, 0)
        for s in range(n_seg):
            out_copy(s).wait()

    return kernel


def _forward(x, mem0, wq, wk, wv, wo, seg_len, q, k, v, shift_k, ssm_k, ssm_d):
    _, seq, d_model = x.shape
    _, n_heads, d_head = wq.shape
    n_mem = mem0.shape[1]
    seg = seg_len
    n_seg = seq // seg
    n_rows = n_mem + seg
    n_cb = d_model // CB
    assert seq == SEQ and d_model == 1024 and d_head == 128 and n_rows % 8 == 0
    tf, ti, t2 = _dft_tables()

    any_spec = pl.BlockSpec(memory_space=pl.ANY)
    kv_rows = -(-n_rows // 16) * 16
    scratch = [
        pltpu.VMEM((n_cb, CB, seq), BF16),
        pltpu.VMEM((seq, d_model), BF16),
        pltpu.VMEM((seq, d_model), BF16),
        pltpu.VMEM((n_cb, seq, CB), BF16),
        pltpu.VMEM((8 + seq, CB), F32),
        pltpu.VMEM((2, 2 * N1 * SP, CB), BF16),
        pltpu.VMEM((2, 2 * N1 * SP, CB), BF16),
        pltpu.VMEM((2 * N2 * SZ, CB), BF16),
        pltpu.VMEM((2 * N2 * SZ, CB), BF16),
        pltpu.VMEM((2 * N1 * ST, CB), BF16),
        pltpu.VMEM((N1 * SY, CB), F32),
        pltpu.VMEM(tf.shape, U32),
        pltpu.VMEM(ti.shape, U32),
        pltpu.VMEM(t2.shape, U32),
        pltpu.VMEM((4, d_model), BF16),
        pltpu.VMEM((n_cb, CB), BF16),
        pltpu.VMEM((n_mem, d_model), BF16),
        pltpu.VMEM((4, d_model), F32),
        pltpu.VMEM((n_cb, CB), F32),
        pltpu.VMEM((3 * n_heads // 2, d_model, d_head), U32),
        pltpu.VMEM((3 * n_heads, d_model // 2, d_head), U32),
        pltpu.VMEM((d_model // 128, n_heads * d_head // 2, 128), U32),
        pltpu.VMEM((seq, d_model), BF16),
        pltpu.VMEM((seq, d_model), BF16),
        pltpu.VMEM((n_seg, seg, 2 * d_model), BF16),
        pltpu.VMEM((n_rows, d_model), F32),
        pltpu.VMEM((n_heads, n_rows, d_head), F32),
        pltpu.VMEM((n_heads, kv_rows, d_head), BF16),
        pltpu.VMEM((n_heads, kv_rows, d_head), BF16),
        pltpu.VMEM((n_rows, n_heads * d_head), F32),
        pltpu.VMEM((n_heads, n_rows, d_head), F32),
        pltpu.VMEM((n_heads, n_rows, d_head), F32),
        pltpu.VMEM((d_model // 128, n_rows, 128), F32),
        pltpu.VMEM((max(_CFG["n_pre"], 2) * 8, d_model), BF16),
        pltpu.VMEM((max(_CFG["n_pre"], 2) * 8, d_model), F32),
        pltpu.VMEM((2, n_heads, max(_CFG["n_pre"], 2) * 8, d_head), F32),
        pltpu.SemaphoreType.DMA((3, n_cb)),
        pltpu.SemaphoreType.DMA((6,)),
        pltpu.SemaphoreType.DMA((3,)),
        pltpu.SemaphoreType.DMA((len(_CFG["first_splits"]) + 1,)),
        pltpu.SemaphoreType.DMA((2,)),
        pltpu.SemaphoreType.DMA(()),
        pltpu.SemaphoreType.DMA((n_seg,)),
        pltpu.SemaphoreType.DMA((n_seg,)),
        pltpu.SemaphoreType.DMA(()),
    ]
    out = pl.pallas_call(
        _make_kernel(n_heads, d_head, d_model, n_mem, seg, n_seg),
        out_shape=jax.ShapeDtypeStruct((seq, 2 * d_model), BF16),
        in_specs=[any_spec] * 15,
        out_specs=any_spec,
        scratch_shapes=scratch,
        compiler_params=pltpu.CompilerParams(vmem_limit_bytes=120 * 1024 * 1024),
    )(shift_k.T, ssm_d.reshape(n_cb, CB), mem0.reshape(n_mem, d_model),
      x.reshape(seq, d_model), wq, wk, wv, wo.reshape(n_heads * d_head, d_model),
      q.reshape(seq, d_model), k.reshape(seq, d_model), v.reshape(seq, d_model), ssm_k,
      tf, ti, t2)
    return out.reshape(1, seq, 2 * d_model)


def pallas_concat_heads__memory_aug_recurrent_mem_tr__ssm_conv_h3__prompt_kernel(
        A_x, A_mem0, A_Wq, A_Wk, A_Wv, A_Wo, A_seg_len, B_q, B_k, B_v, B_shift_k, B_ssm_k, B_ssm_D):
    return _forward(A_x, A_mem0, A_Wq, A_Wk, A_Wv, A_Wo, int(A_seg_len), B_q, B_k, B_v,
                    B_shift_k, B_ssm_k, B_ssm_D)
```

```python
import functools
import math

import jax
import jax.numpy as jnp
import numpy as np
from jax.experimental import pallas as pl
from jax.experimental.pallas import tpu as pltpu

F32 = jnp.float32
BF16 = jnp.bfloat16
U32 = jnp.uint32

N1, N2 = 32, 64
SEQ = N1 * N2
SP = N2 // 2 + 4
SZ = N1 + 4
ST = N2 + 4
SY = N2 + 4
CB = 128


def _dft_tables():
    theta = np.pi / (2 * SEQ)
    lane = np.arange(128)[None, :]
    hi, mid, lo = lane // 64, (lane % 64) // 2, lane % 2
    k1 = np.arange(N1)[:, None]
    fwd = np.zeros((N2 // 4, 2 * N1, 128))
    for g in range(N2 // 4):
        ph = theta * (4 * k1 + 1) * (N2 * mid + 4 * g + 2 * hi + lo)
        fwd[g, 0::2] = np.cos(ph)
        fwd[g, 1::2] = np.sin(ph)
    n1 = np.arange(N1)[:, None]
    inv = np.zeros((N2 // 2, N1, 128))
    for i in range(N2 // 2):
        ph = theta * (4 * mid + 1) * (N2 * n1 + 2 * i + hi)
        inv[i] = np.where(lo == 0, np.cos(ph), np.sin(ph)) / SEQ
    ph = 2 * np.pi * np.arange(N2)[:, None] * np.arange(N2)[None, :] / N2
    c, s = np.cos(ph), np.sin(ph)
    f2 = np.zeros((128, 128))
    f2[:N2, 0::2], f2[:N2, 1::2], f2[N2:, 0::2], f2[N2:, 1::2] = c, -s, s, c
    g2 = np.zeros((128, 128))
    g2[0::2, :N2], g2[0::2, N2:], g2[1::2, :N2], g2[1::2, N2:] = c.T, s.T, -s.T, c.T

    def as_words(a):
        u = a.astype(np.float32).astype(BF16).view(np.uint16).astype(np.uint32)
        return u[..., 0::2, :] | (u[..., 1::2, :] << 16)

    return as_words(fwd), as_words(inv), as_words(np.stack([f2, g2]))


def _to_words(x):
    return pltpu.bitcast(x.astype(BF16), U32)


def _from_words(w):
    return pltpu.bitcast(w, BF16)


_CFG = dict(group=8, lag_s=2, lag_v=3, wo_split=16, gate_at=1, late_first=0, late_per_block=10, prep_early=4, b_group=4, n_early=3, n_first=2, unroll=3, chunk_steps=3, first_splits=(16,),
            n_pre=15, pre_pairs=1, pre_rolled=1, v_fuse=1)


def _step_order(n_heads, n_out_tiles, first=False):
    g, a, b = _CFG["group"], _CFG["lag_s"], _CFG["lag_v"]
    split = _CFG["wo_split"]
    n_groups = n_heads // g
    total = n_groups + a + b
    early = [("W", j, 0, split) for j in range(n_out_tiles)] if split < n_heads else []
    ops = []
    for t in range(total):
        if t < n_groups:
            ops += [("P", h) for h in range(t * g, (t + 1) * g)]
        if t == _CFG["gate_at"]:
            ops.append(("G",))
        if 0 <= t - a < n_groups:
            ops += [("S", h) for h in range((t - a) * g, (t - a + 1) * g)]
        if 0 <= t - a - b < n_groups:
            ops += [("V", h) for h in range((t - a - b) * g, (t - a - b + 1) * g)]
        if early and (t - a - b + 1) * g >= split:
            n = -(-len(early) // (total - t))
            ops += early[:n]
            early = early[n:]
    ops += early
    bounds = [split if split < n_heads else 0]
    if first:
        bounds += [b for b in _CFG["first_splits"] if b > split]
    for lo, hi in zip(bounds, bounds[1:] + [n_heads]):
        ops += [("W", j, lo, hi) for j in range(n_out_tiles)]
    return ops


def _dot(a, b):
    return jnp.dot(a, b, preferred_element_type=F32)


def _dot_nt(a, b):
    return jax.lax.dot_general(a, b, (((1,), (1,)), ((), ())), preferred_element_type=F32)


def _make_kernel(n_heads, d_head, d_model, n_mem, seg, n_seg):
    n_rows = n_mem + seg
    n_cb = d_model // CB
    n_hp = n_heads // 2
    scale = d_head ** (-0.5)
    exp_scale = scale * math.log2(math.e)
    steps_per_chunk = _CFG["chunk_steps"]
    x_chunks = (n_seg - 1) // steps_per_chunk
    x_rows = steps_per_chunk * seg
    assert x_chunks * steps_per_chunk == n_seg - 1 and steps_per_chunk % _CFG["unroll"] == 0
    n_pre = _CFG["n_pre"]
    pre_rows = 8
    assert n_pre % steps_per_chunk == 0
    order = _step_order(n_heads, d_model // 128)
    order_first = _step_order(n_heads, d_model // 128, True)
    wo_bounds = [0] + list(_CFG["first_splits"]) + [n_heads]

    def kernel(sh_hbm, d_hbm, mem_hbm,
               x_hbm, wq_hbm, wk_hbm, wv_hbm, wo_hbm,
               q_hbm, k_hbm, v_hbm, h_hbm, tf_hbm, ti_hbm, t2_hbm,
               out_hbm,
               hs, ks, vs, ob, kf, xp, hp, zx, zh, tt, yp, tf, ti, t2, sh_ref, d_ref, mem_ref, sh32, d32,
               stage, wqkv, wo, xin, qin, ost, hbuf, qbuf, kbuf, vbuf, obuf, pbuf, ibuf, ybuf, xpre, xpre32, qkpre,
               sem_b, sem_t, sem_w, sem_o, sem_h, sem_p, sem_x, sem_q, sem_out):

        n_early = _CFG["n_early"]

        def h_copy(cb):
            c0 = cb * CB if isinstance(cb, int) else pl.multiple_of(cb * CB, CB)
            return pltpu.make_async_copy(h_hbm.at[pl.ds(c0, CB), :], hs.at[cb], sem_b.at[0, cb])

        def kv_copies(cb):
            if isinstance(cb, int):
                c0, width = cb * CB, (CB if cb < n_early else d_model - n_early * CB)
            else:
                c0, width = pl.multiple_of(cb * CB, CB), CB
            return [pltpu.make_async_copy(src.at[:, pl.ds(c0, width)], dst.at[:, pl.ds(c0, width)], sem_b.at[1 + i, cb])
                    for i, (src, dst) in enumerate(((k_hbm, ks), (v_hbm, vs)))]

        def t_copies():
            pairs = ((sh_hbm, sh_ref), (d_hbm, d_ref), (mem_hbm, mem_ref),
                     (tf_hbm, tf), (ti_hbm, ti), (t2_hbm, t2))
            return [pltpu.make_async_copy(src, dst, sem_t.at[i]) for i, (src, dst) in enumerate(pairs)]

        def w_copies(m):
            w32 = (wq_hbm, wk_hbm, wv_hbm)[m].bitcast(U32)
            return [pltpu.make_async_copy(w32.at[:, hp, :], stage.at[m * n_hp + hp], sem_w.at[m])
                    for hp in range(n_hp)]

        def o_copies(i):
            wo32 = wo_hbm.bitcast(U32)
            lo, hi = wo_bounds[i] * d_head // 2, wo_bounds[i + 1] * d_head // 2
            return [pltpu.make_async_copy(wo32.at[pl.ds(lo, hi - lo), pl.ds(j * 128, 128)],
                                          wo.at[j, pl.ds(lo, hi - lo), :], sem_o.at[i])
                    for j in range(d_model // 128)]

        def head_copies():
            return [pltpu.make_async_copy(src.at[pl.ds(0, seg), :], dst.at[pl.ds(0, seg), :], sem_h.at[i])
                    for i, (src, dst) in enumerate(((x_hbm, xin), (q_hbm, qin)))]

        def pre_copies():
            return [pltpu.make_async_copy(x_hbm.at[pl.ds((i + 1) * seg, pre_rows), :],
                                          xpre.at[pl.ds(i * pre_rows, pre_rows), :], sem_p) for i in range(n_pre)]

        def chunk_copies(c):
            r0 = seg + c * x_rows if isinstance(c, int) else pl.multiple_of(seg + c * x_rows, seg)
            return [pltpu.make_async_copy(src.at[pl.ds(r0, x_rows), :], dst.at[pl.ds(r0, x_rows), :], sem.at[c])
                    for src, dst, sem in ((x_hbm, xin, sem_x), (q_hbm, qin, sem_q))]

        def out_copy(s):
            r0 = s * seg if isinstance(s, int) else pl.multiple_of(s * seg, seg)
            return pltpu.make_async_copy(ost.at[s], out_hbm.at[pl.ds(r0, seg), :], sem_out)

        for c in t_copies():
            c.start()
        n_first = _CFG["n_first"]
        for cb in range(n_first):
            for c in [h_copy(cb)] + kv_copies(cb):
                c.start()
        second = []
        for cb in range(n_first, n_early):
            second += [h_copy(cb)] + kv_copies(cb)
        late = kv_copies(n_early) + [h_copy(cb) for cb in range(n_early, n_cb)]
        n_b_late = len(late)
        late += w_copies(0) + pre_copies() + w_copies(1) + w_copies(2) + head_copies()
        for i in range(len(wo_bounds) - 1):
            late += o_copies(i)
        per_block = _CFG["late_per_block"]
        first_block = _CFG["late_first"]

        kf[0:8, :] = jnp.zeros((8, CB), F32)

        group = _CFG["b_group"]

        def put(ref, row, x, slot=()):
            ref[(*slot, pl.ds(2 * row, x.shape[0]), slice(None))] = x.astype(BF16)

        def get(ref, row, n, stride=1, slot=()):
            return ref.bitcast(U32)[(*slot, pl.ds(row, n, stride=stride), slice(None))]

        def wait_inputs(cb):
            h_copy(cb).wait()

            @pl.when(cb < n_early)
            def _():
                for c in kv_copies(cb):
                    c.wait()

            @pl.when(cb == n_early)
            def _():
                for c in kv_copies(n_early):
                    c.wait()

        def prepare(cb, slot, piece):
            c0 = pl.multiple_of(cb * CB, CB)
            for j in range(2 * piece, 2 * piece + 2):
                r = hs[cb, :, j * 128:(j + 1) * 128].astype(F32).T
                put(hp, (2 * j) * SP, r[0:N2], (slot,))
                put(hp, (2 * j + 1) * SP, r[N2:2 * N2], (slot,))
            taps = sh32[:, pl.ds(c0, CB)]
            for n1 in range(4 * piece, 4 * piece + 4):
                kf[pl.ds(8 + n1 * N2, N2), :] = ks[pl.ds(n1 * N2, N2), pl.ds(c0, CB)].astype(F32)
                acc = kf[pl.ds(8 + n1 * N2, N2), :] * taps[0:1]
                for i in range(1, 4):
                    acc = acc + kf[pl.ds(8 - i + n1 * N2, N2), :] * taps[i:i + 1]
                put(xp, n1 * SP, acc * vs[pl.ds(n1 * N2, N2), pl.ds(c0, CB)].astype(F32), (slot,))

        def finish(cb, slot, piece):
            dv = d32[pl.ds(cb, 1), :]
            for n1 in range(4 * piece, 4 * piece + 4):
                kv = _from_words(get(xp, n1 * SP, N2 // 2, 1, (slot,))).astype(F32)
                ob[cb, pl.ds(n1 * N2, N2), :] = (yp[pl.ds(n1 * SY, N2), :] + kv * dv).astype(BF16)

        def b_block(cb, carry):
            @pl.when(cb + 1 < n_cb)
            def _():
                wait_inputs(cb + 1)

            for i in range(n_cb - first_block):
                @pl.when(cb == i + first_block)
                def _(i=i):
                    lo = 0 if i == 0 else n_b_late + i * per_block
                    for c in late[lo:n_b_late + (i + 1) * per_block]:
                        c.start()
            lane = jax.lax.broadcasted_iota(jnp.int32, (1, 128), 1)
            slot = cb % 2
            nxt = jnp.minimum(cb + 1, n_cb - 1)
            prv = jnp.maximum(cb - 1, 0)
            n_pieces = 8

            def side_work(piece):
                finish(prv, 1 - slot, piece)
                prepare(nxt, 1 - slot, piece)

            early_pieces = _CFG["prep_early"]
            for g in range(N2 // 4):
                m = tf[g]
                lhs = _from_words(jnp.concatenate(
                    [jnp.where((lane // 64 == j // 2) & (lane % 2 == j % 2), m, jnp.zeros_like(m))
                     for j in range(4)], axis=0))

                def rhs(ref, g=g):
                    return _from_words(jnp.concatenate(
                        [get(ref, 2 * g, N1, SP, (slot,)), get(ref, 2 * g + 1, N1, SP, (slot,))], axis=0))

                r = _dot(lhs, jnp.concatenate([rhs(xp), rhs(hp)], axis=1))
                for j in range(4):
                    put(zx, (4 * g + j) * SZ, r[2 * N1 * j:2 * N1 * (j + 1), :128])
                    put(zh, (4 * g + j) * SZ, r[2 * N1 * j:2 * N1 * (j + 1), 128:])
                if early_pieces and g % (16 // early_pieces) == 0:
                    side_work(g // (16 // early_pieces))
            f2 = _from_words(t2[0])
            g2 = _from_words(t2[1])

            def stage2(g):
                zz = []
                for k1 in range(g * group, (g + 1) * group):
                    zz += [_from_words(get(zx, k1, N2, SZ)), _from_words(get(zh, k1, N2, SZ))]
                return _dot(f2, jnp.concatenate(zz, axis=1))

            def stage3(g, r):
                ys = []
                for i in range(group):
                    xf = r[:, (2 * i) * 128:(2 * i + 1) * 128]
                    hf = r[:, (2 * i + 1) * 128:(2 * i + 2) * 128]
                    xr, xi, hr, hi = xf[:N2], xf[N2:], hf[:N2], hf[N2:]
                    ys.append(jnp.concatenate([xr * hr - xi * hi, xr * hi + xi * hr], axis=0).astype(BF16))
                t = _dot(g2, jnp.concatenate(ys, axis=1))
                for i in range(group):
                    put(tt, (g * group + i) * ST, t[:, i * 128:(i + 1) * 128])

            n_groups = N1 // group
            late_pieces = list(range(early_pieces, n_pieces))
            r = stage2(0)
            for g in range(n_groups):
                r_next = stage2(g + 1) if g + 1 < n_groups else None
                stage3(g, r)
                r = r_next
                for piece in late_pieces[g::n_groups]:
                    side_work(piece)
            for i in range(N2 // 2):
                m = ti[i]
                lhs = _from_words(jnp.concatenate([jnp.where(lane < 64, m, jnp.zeros_like(m)),
                                                   jnp.where(lane >= 64, m, jnp.zeros_like(m))], axis=0))
                y = _dot(lhs, _from_words(jnp.concatenate(
                    [get(tt, 2 * i, N1, ST), get(tt, 2 * i + 1, N1, ST)], axis=0)))
                yp[pl.ds(2 * i, N1, stride=SY), :] = y[0:N1]
                yp[pl.ds(2 * i + 1, N1, stride=SY), :] = y[N1:2 * N1]
            return carry

        for c in t_copies():
            c.wait()
        sh32[...] = sh_ref[...].astype(F32)
        d32[...] = d_ref[...].astype(F32)
        hbuf[0:n_mem, :] = mem_ref[...].astype(F32)
        wait_inputs(0)
        for c in second:
            c.start()
        for piece in range(8):
            prepare(0, 0, piece)
        jax.lax.fori_loop(0, n_cb, b_block, 0)
        for c in late[n_b_late + (n_cb - first_block) * per_block:]:
            c.start()
        for piece in range(8):
            finish(n_cb - 1, (n_cb - 1) % 2, piece)

        def wtile(ref, i):
            return _from_words(ref[i])

        def relayout(m, hp):
            even = stage[m * n_hp + hp, pl.ds(0, d_model // 2, stride=2), :]
            odd = stage[m * n_hp + hp, pl.ds(1, d_model // 2, stride=2), :]
            wqkv[(2 * hp) * 3 + m] = (even & U32(0xFFFF)) | (odd << 16)
            wqkv[(2 * hp + 1) * 3 + m] = (even >> 16) | (odd & U32(0xFFFF0000))

        for m in range(2):
            for c in w_copies(m):
                c.wait()
        for c in pre_copies():
            c.wait()
        xpre32[...] = xpre[...].astype(F32)
        per = _CFG["pre_pairs"]
        for u in range(per):
            relayout(0, u)
            relayout(1, u)

        def pre_round(i, last):
            xl = xpre32[...]
            for u in range(per):
                for h in (2 * (i * per + u), 2 * (i * per + u) + 1):
                    for m in range(2):
                        qkpre[m, h] = _dot(xl, wtile(wqkv, 3 * h + m))
                if not last:
                    relayout(0, (i + 1) * per + u)
                    relayout(1, (i + 1) * per + u)

        def pre_body(i, carry):
            pre_round(i, False)
            return carry

        jax.lax.fori_loop(0, n_hp // per - 1, pre_body, 0)
        pre_round(n_hp // per - 1, True)
        for c in w_copies(2):
            c.wait()
        if not _CFG["v_fuse"]:
            def v_body(hp, carry):
                relayout(2, hp)
                return carry

            jax.lax.fori_loop(0, n_hp, v_body, 0)

        def step(s, first, pre=False):
            if first:
                for c in head_copies():
                    c.wait()
            row = jax.lax.broadcasted_iota(jnp.int32, (n_rows, n_rows), 0)
            col = jax.lax.broadcasted_iota(jnp.int32, (n_rows, n_rows), 1)
            mask = (row < n_mem) | (row >= col)
            r0 = s * seg if first else pl.multiple_of(s * seg, seg)
            slot = s
            hbuf[n_mem:n_rows, :] = xin[pl.ds(r0, seg), :].astype(F32)
            hl = hbuf[...]
            if pre:
                hr = jnp.concatenate([hl[0:n_mem], hl[n_mem + pre_rows:n_rows]], axis=0)
                p0 = pl.multiple_of((s - 1) * pre_rows, pre_rows)
            waited = [False] * (len(wo_bounds) - 1)
            for op in (order_first if first else order):
                if op[0] == "P":
                    h = op[1]
                    if first and h % 2 == 0 and _CFG["v_fuse"]:
                        if h == 0:
                            relayout(2, 0)
                        if h // 2 + 1 < n_hp:
                            relayout(2, h // 2 + 1)
                    if pre:
                        rq = _dot(hr, wtile(wqkv, 3 * h))
                        qbuf[h] = jnp.concatenate(
                            [rq[0:n_mem], qkpre[0, h, pl.ds(p0, pre_rows), :], rq[n_mem:]], axis=0)
                        rk = _dot(hr, wtile(wqkv, 3 * h + 1))
                        kbuf[h, 0:n_rows] = jnp.concatenate(
                            [rk[0:n_mem], qkpre[1, h, pl.ds(p0, pre_rows), :], rk[n_mem:]], axis=0).astype(BF16)
                    else:
                        qbuf[h] = _dot(hl, wtile(wqkv, 3 * h))
                        kbuf[h, 0:n_rows] = _dot(hl, wtile(wqkv, 3 * h + 1)).astype(BF16)
                    vbuf[h, 0:n_rows] = _dot(hl, wtile(wqkv, 3 * h + 2)).astype(BF16)
                elif op[0] == "S":
                    h = op[1]
                    sc = _dot_nt(qbuf[h], kbuf[h, 0:n_rows])
                    sc = jnp.where(mask, sc, -1e9 / scale)
                    e = jnp.exp2((sc - jnp.max(sc, axis=-1, keepdims=True)) * exp_scale)
                    den = jnp.sum(e, axis=-1, keepdims=True)
                    inv = pl.reciprocal(den, approx=True)
                    pbuf[h, :, 0:n_rows] = e
                    ibuf[h] = jnp.broadcast_to(inv * (2.0 - den * inv), (n_rows, d_head))
                elif op[0] == "V":
                    h = op[1]
                    obuf[:, h * d_head:(h + 1) * d_head] = (
                        _dot(pbuf[h, :, 0:n_rows], vbuf[h, 0:n_rows]) * ibuf[h])
                elif op[0] == "W":
                    _, j, lo, hi = op
                    if first:
                        for i in range(len(waited)):
                            if not waited[i] and hi > wo_bounds[i]:
                                for c in o_copies(i):
                                    c.wait()
                                waited[i] = True
                                if i == len(waited) - 1:
                                    for ch in range(x_chunks):
                                        for c in chunk_copies(ch):
                                            c.start()
                    w = _from_words(wo[j, lo * d_head // 2:hi * d_head // 2, :])
                    y = _dot(obuf[:, lo * d_head:hi * d_head], w)
                    if lo > 0:
                        y = y + ybuf[j]
                    if hi < n_heads:
                        ybuf[j] = y
                    else:
                        hbuf[0:n_mem, j * 128:(j + 1) * 128] = y[0:n_mem]
                        ost[slot, :, j * 128:(j + 1) * 128] = y[n_mem:n_rows].astype(BF16)
                else:
                    for cb in range(n_cb):
                        gate = qin[pl.ds(r0, seg), cb * CB:(cb + 1) * CB].astype(F32)
                        ost[slot, :, d_model + cb * CB:d_model + (cb + 1) * CB] = (
                            ob[cb, pl.ds(r0, seg), :].astype(F32) * gate).astype(BF16)
            out_copy(s).start()

        unroll = _CFG["unroll"]

        def chunk_body(c, carry, pre=False):
            for cp in chunk_copies(c):
                cp.wait()

            def steps_body(i, carry):
                for u in range(unroll):
                    step(1 + c * steps_per_chunk + i * unroll + u, False, pre)
                return carry

            if steps_per_chunk == unroll:
                steps_body(0, 0)
            else:
                jax.lax.fori_loop(0, steps_per_chunk // unroll, steps_body, 0)
            return carry

        step(0, True)
        def pre_step(s, carry):
            @pl.when((s - 1) % steps_per_chunk == 0)
            def _():
                for cp in chunk_copies((s - 1) // steps_per_chunk):
                    cp.wait()

            step(s, False, True)
            return carry

        pre_chunks = n_pre // steps_per_chunk
        if pre_chunks and _CFG["pre_rolled"]:
            jax.lax.fori_loop(1, 1 + n_pre, pre_step, 0)
        elif pre_chunks:
            jax.lax.fori_loop(0, pre_chunks, functools.partial(chunk_body, pre=True), 0)
        jax.lax.fori_loop(pre_chunks, x_chunks, chunk_body, 0)
        for s in range(n_seg):
            out_copy(s).wait()

    return kernel


def _forward(x, mem0, wq, wk, wv, wo, seg_len, q, k, v, shift_k, ssm_k, ssm_d):
    _, seq, d_model = x.shape
    _, n_heads, d_head = wq.shape
    n_mem = mem0.shape[1]
    seg = seg_len
    n_seg = seq // seg
    n_rows = n_mem + seg
    n_cb = d_model // CB
    assert seq == SEQ and d_model == 1024 and d_head == 128 and n_rows % 8 == 0
    tf, ti, t2 = _dft_tables()

    any_spec = pl.BlockSpec(memory_space=pl.ANY)
    kv_rows = -(-n_rows // 16) * 16
    scratch = [
        pltpu.VMEM((n_cb, CB, seq), BF16),
        pltpu.VMEM((seq, d_model), BF16),
        pltpu.VMEM((seq, d_model), BF16),
        pltpu.VMEM((n_cb, seq, CB), BF16),
        pltpu.VMEM((8 + seq, CB), F32),
        pltpu.VMEM((2, 2 * N1 * SP, CB), BF16),
        pltpu.VMEM((2, 2 * N1 * SP, CB), BF16),
        pltpu.VMEM((2 * N2 * SZ, CB), BF16),
        pltpu.VMEM((2 * N2 * SZ, CB), BF16),
        pltpu.VMEM((2 * N1 * ST, CB), BF16),
        pltpu.VMEM((N1 * SY, CB), F32),
        pltpu.VMEM(tf.shape, U32),
        pltpu.VMEM(ti.shape, U32),
        pltpu.VMEM(t2.shape, U32),
        pltpu.VMEM((4, d_model), BF16),
        pltpu.VMEM((n_cb, CB), BF16),
        pltpu.VMEM((n_mem, d_model), BF16),
        pltpu.VMEM((4, d_model), F32),
        pltpu.VMEM((n_cb, CB), F32),
        pltpu.VMEM((3 * n_heads // 2, d_model, d_head), U32),
        pltpu.VMEM((3 * n_heads, d_model // 2, d_head), U32),
        pltpu.VMEM((d_model // 128, n_heads * d_head // 2, 128), U32),
        pltpu.VMEM((seq, d_model), BF16),
        pltpu.VMEM((seq, d_model), BF16),
        pltpu.VMEM((n_seg, seg, 2 * d_model), BF16),
        pltpu.VMEM((n_rows, d_model), F32),
        pltpu.VMEM((n_heads, n_rows, d_head), F32),
        pltpu.VMEM((n_heads, kv_rows, d_head), BF16),
        pltpu.VMEM((n_heads, kv_rows, d_head), BF16),
        pltpu.VMEM((n_rows, n_heads * d_head), F32),
        pltpu.VMEM((n_heads, n_rows, d_head), F32),
        pltpu.VMEM((n_heads, n_rows, d_head), F32),
        pltpu.VMEM((d_model // 128, n_rows, 128), F32),
        pltpu.VMEM((max(_CFG["n_pre"], 2) * 8, d_model), BF16),
        pltpu.VMEM((max(_CFG["n_pre"], 2) * 8, d_model), F32),
        pltpu.VMEM((2, n_heads, max(_CFG["n_pre"], 2) * 8, d_head), F32),
        pltpu.SemaphoreType.DMA((3, n_cb)),
        pltpu.SemaphoreType.DMA((6,)),
        pltpu.SemaphoreType.DMA((3,)),
        pltpu.SemaphoreType.DMA((len(_CFG["first_splits"]) + 1,)),
        pltpu.SemaphoreType.DMA((2,)),
        pltpu.SemaphoreType.DMA(()),
        pltpu.SemaphoreType.DMA((n_seg,)),
        pltpu.SemaphoreType.DMA((n_seg,)),
        pltpu.SemaphoreType.DMA(()),
    ]
    out = pl.pallas_call(
        _make_kernel(n_heads, d_head, d_model, n_mem, seg, n_seg),
        out_shape=jax.ShapeDtypeStruct((seq, 2 * d_model), BF16),
        in_specs=[any_spec] * 15,
        out_specs=any_spec,
        scratch_shapes=scratch,
        compiler_params=pltpu.CompilerParams(vmem_limit_bytes=120 * 1024 * 1024),
    )(shift_k.T, ssm_d.reshape(n_cb, CB), mem0.reshape(n_mem, d_model),
      x.reshape(seq, d_model), wq, wk, wv, wo.reshape(n_heads * d_head, d_model),
      q.reshape(seq, d_model), k.reshape(seq, d_model), v.reshape(seq, d_model), ssm_k,
      tf, ti, t2)
    return out.reshape(1, seq, 2 * d_model)


def pallas_concat_heads__memory_aug_recurrent_mem_tr__ssm_conv_h3__prompt_kernel(
        A_x, A_mem0, A_Wq, A_Wk, A_Wv, A_Wo, A_seg_len, B_q, B_k, B_v, B_shift_k, B_ssm_k, B_ssm_D):
    return _forward(A_x, A_mem0, A_Wq, A_Wk, A_Wv, A_Wo, int(A_seg_len), B_q, B_k, B_v,
                    B_shift_k, B_ssm_k, B_ssm_D)
```

```python
import functools
import math

import jax
import jax.numpy as jnp
import numpy as np
from jax.experimental import pallas as pl
from jax.experimental.pallas import tpu as pltpu

F32 = jnp.float32
BF16 = jnp.bfloat16
U32 = jnp.uint32

N1, N2 = 32, 64
SEQ = N1 * N2
SP = N2 // 2 + 4
SZ = N1 + 4
ST = N2 + 4
SY = N2 + 4
CB = 128


def _dft_tables():
    theta = np.pi / (2 * SEQ)
    lane = np.arange(128)[None, :]
    hi, mid, lo = lane // 64, (lane % 64) // 2, lane % 2
    k1 = np.arange(N1)[:, None]
    fwd = np.zeros((N2 // 4, 2 * N1, 128))
    for g in range(N2 // 4):
        ph = theta * (4 * k1 + 1) * (N2 * mid + 4 * g + 2 * hi + lo)
        fwd[g, 0::2] = np.cos(ph)
        fwd[g, 1::2] = np.sin(ph)
    n1 = np.arange(N1)[:, None]
    inv = np.zeros((N2 // 2, N1, 128))
    for i in range(N2 // 2):
        ph = theta * (4 * mid + 1) * (N2 * n1 + 2 * i + hi)
        inv[i] = np.where(lo == 0, np.cos(ph), np.sin(ph)) / SEQ
    ph = 2 * np.pi * np.arange(N2)[:, None] * np.arange(N2)[None, :] / N2
    c, s = np.cos(ph), np.sin(ph)
    f2 = np.zeros((128, 128))
    f2[:N2, 0::2], f2[:N2, 1::2], f2[N2:, 0::2], f2[N2:, 1::2] = c, -s, s, c
    g2 = np.zeros((128, 128))
    g2[0::2, :N2], g2[0::2, N2:], g2[1::2, :N2], g2[1::2, N2:] = c.T, s.T, -s.T, c.T

    def as_words(a):
        u = a.astype(np.float32).astype(BF16).view(np.uint16).astype(np.uint32)
        return u[..., 0::2, :] | (u[..., 1::2, :] << 16)

    return as_words(fwd), as_words(inv), as_words(np.stack([f2, g2]))


def _to_words(x):
    return pltpu.bitcast(x.astype(BF16), U32)


def _from_words(w):
    return pltpu.bitcast(w, BF16)


_CFG = dict(group=8, lag_s=2, lag_v=3, wo_split=16, gate_at=1, late_first=0, late_per_block=10, prep_early=4, b_group=4, n_early=3, n_first=2, unroll=3, chunk_steps=3, first_splits=(16,),
            n_pre=18, pre_rolled=1)


def _step_order(n_heads, n_out_tiles, first=False):
    g, a, b = _CFG["group"], _CFG["lag_s"], _CFG["lag_v"]
    split = _CFG["wo_split"]
    n_groups = n_heads // g
    total = n_groups + a + b
    early = [("W", j, 0, split) for j in range(n_out_tiles)] if split < n_heads else []
    ops = []
    for t in range(total):
        if t < n_groups:
            ops += [("P", h) for h in range(t * g, (t + 1) * g)]
        if t == _CFG["gate_at"]:
            ops.append(("G",))
        if 0 <= t - a < n_groups:
            ops += [("S", h) for h in range((t - a) * g, (t - a + 1) * g)]
        if 0 <= t - a - b < n_groups:
            ops += [("V", h) for h in range((t - a - b) * g, (t - a - b + 1) * g)]
        if early and (t - a - b + 1) * g >= split:
            n = -(-len(early) // (total - t))
            ops += early[:n]
            early = early[n:]
    ops += early
    bounds = [split if split < n_heads else 0]
    if first:
        bounds += [b for b in _CFG["first_splits"] if b > split]
    for lo, hi in zip(bounds, bounds[1:] + [n_heads]):
        ops += [("W", j, lo, hi) for j in range(n_out_tiles)]
    return ops


def _dot(a, b):
    return jnp.dot(a, b, preferred_element_type=F32)


def _dot_nt(a, b):
    return jax.lax.dot_general(a, b, (((1,), (1,)), ((), ())), preferred_element_type=F32)


def _make_kernel(n_heads, d_head, d_model, n_mem, seg, n_seg):
    n_rows = n_mem + seg
    n_cb = d_model // CB
    n_hp = n_heads // 2
    scale = d_head ** (-0.5)
    exp_scale = scale * math.log2(math.e)
    steps_per_chunk = _CFG["chunk_steps"]
    x_chunks = (n_seg - 1) // steps_per_chunk
    x_rows = steps_per_chunk * seg
    assert x_chunks * steps_per_chunk == n_seg - 1 and steps_per_chunk % _CFG["unroll"] == 0
    n_pre = _CFG["n_pre"]
    pre_rows = 8
    assert n_pre % steps_per_chunk == 0
    order = _step_order(n_heads, d_model // 128)
    order_first = _step_order(n_heads, d_model // 128, True)
    wo_bounds = [0] + list(_CFG["first_splits"]) + [n_heads]

    def kernel(sh_hbm, d_hbm, mem_hbm,
               x_hbm, wq_hbm, wk_hbm, wv_hbm, wo_hbm,
               q_hbm, k_hbm, v_hbm, h_hbm, tf_hbm, ti_hbm, t2_hbm,
               out_hbm,
               hs, ks, vs, ob, kf, xp, hp, zx, zh, tt, yp, tf, ti, t2, sh_ref, d_ref, mem_ref, sh32, d32,
               stage, w_even, w_odd, wo, xin, qin, ost, hbuf, qbuf, kbuf, vbuf, obuf, pbuf, ibuf, ybuf, xpre, xpre32, qkpre,
               sem_b, sem_t, sem_w, sem_o, sem_h, sem_p, sem_x, sem_q, sem_out):

        n_early = _CFG["n_early"]

        def h_copy(cb):
            c0 = cb * CB if isinstance(cb, int) else pl.multiple_of(cb * CB, CB)
            return pltpu.make_async_copy(h_hbm.at[pl.ds(c0, CB), :], hs.at[cb], sem_b.at[0, cb])

        def kv_copies(cb):
            if isinstance(cb, int):
                c0, width = cb * CB, (CB if cb < n_early else d_model - n_early * CB)
            else:
                c0, width = pl.multiple_of(cb * CB, CB), CB
            return [pltpu.make_async_copy(src.at[:, pl.ds(c0, width)], dst.at[:, pl.ds(c0, width)], sem_b.at[1 + i, cb])
                    for i, (src, dst) in enumerate(((k_hbm, ks), (v_hbm, vs)))]

        def t_copies():
            pairs = ((sh_hbm, sh_ref), (d_hbm, d_ref), (mem_hbm, mem_ref),
                     (tf_hbm, tf), (ti_hbm, ti), (t2_hbm, t2))
            return [pltpu.make_async_copy(src, dst, sem_t.at[i]) for i, (src, dst) in enumerate(pairs)]

        def w_copies(m):
            w32 = (wq_hbm, wk_hbm, wv_hbm)[m].bitcast(U32)
            return [pltpu.make_async_copy(w32.at[:, hp, :], stage.at[m * n_hp + hp], sem_w.at[m])
                    for hp in range(n_hp)]

        def o_copies(i):
            wo32 = wo_hbm.bitcast(U32)
            lo, hi = wo_bounds[i] * d_head // 2, wo_bounds[i + 1] * d_head // 2
            return [pltpu.make_async_copy(wo32.at[pl.ds(lo, hi - lo), pl.ds(j * 128, 128)],
                                          wo.at[j, pl.ds(lo, hi - lo), :], sem_o.at[i])
                    for j in range(d_model // 128)]

        def head_copies():
            return [pltpu.make_async_copy(src.at[pl.ds(0, seg), :], dst.at[pl.ds(0, seg), :], sem_h.at[i])
                    for i, (src, dst) in enumerate(((x_hbm, xin), (q_hbm, qin)))]

        def pre_copies():
            return [pltpu.make_async_copy(x_hbm.at[pl.ds(i * seg, pre_rows), :],
                                          xpre.at[pl.ds(i * pre_rows, pre_rows), :], sem_p) for i in range(n_pre + 1)]

        def chunk_copies(c):
            r0 = seg + c * x_rows if isinstance(c, int) else pl.multiple_of(seg + c * x_rows, seg)
            return [pltpu.make_async_copy(src.at[pl.ds(r0, x_rows), :], dst.at[pl.ds(r0, x_rows), :], sem.at[c])
                    for src, dst, sem in ((x_hbm, xin, sem_x), (q_hbm, qin, sem_q))]

        def out_copy(s):
            r0 = s * seg if isinstance(s, int) else pl.multiple_of(s * seg, seg)
            return pltpu.make_async_copy(ost.at[s], out_hbm.at[pl.ds(r0, seg), :], sem_out)

        for c in t_copies():
            c.start()
        n_first = _CFG["n_first"]
        for cb in range(n_first):
            for c in [h_copy(cb)] + kv_copies(cb):
                c.start()
        second = []
        for cb in range(n_first, n_early):
            second += [h_copy(cb)] + kv_copies(cb)
        late = kv_copies(n_early) + [h_copy(cb) for cb in range(n_early, n_cb)]
        n_b_late = len(late)
        late += w_copies(0) + pre_copies() + w_copies(1) + w_copies(2) + head_copies()
        for i in range(len(wo_bounds) - 1):
            late += o_copies(i)
        per_block = _CFG["late_per_block"]
        first_block = _CFG["late_first"]

        kf[0:8, :] = jnp.zeros((8, CB), F32)

        group = _CFG["b_group"]

        def put(ref, row, x, slot=()):
            ref[(*slot, pl.ds(2 * row, x.shape[0]), slice(None))] = x.astype(BF16)

        def get(ref, row, n, stride=1, slot=()):
            return ref.bitcast(U32)[(*slot, pl.ds(row, n, stride=stride), slice(None))]

        def wait_inputs(cb):
            h_copy(cb).wait()

            @pl.when(cb < n_early)
            def _():
                for c in kv_copies(cb):
                    c.wait()

            @pl.when(cb == n_early)
            def _():
                for c in kv_copies(n_early):
                    c.wait()

        def prepare(cb, slot, piece):
            c0 = pl.multiple_of(cb * CB, CB)
            for j in range(2 * piece, 2 * piece + 2):
                r = hs[cb, :, j * 128:(j + 1) * 128].astype(F32).T
                put(hp, (2 * j) * SP, r[0:N2], (slot,))
                put(hp, (2 * j + 1) * SP, r[N2:2 * N2], (slot,))
            taps = sh32[:, pl.ds(c0, CB)]
            for n1 in range(4 * piece, 4 * piece + 4):
                kf[pl.ds(8 + n1 * N2, N2), :] = ks[pl.ds(n1 * N2, N2), pl.ds(c0, CB)].astype(F32)
                acc = kf[pl.ds(8 + n1 * N2, N2), :] * taps[0:1]
                for i in range(1, 4):
                    acc = acc + kf[pl.ds(8 - i + n1 * N2, N2), :] * taps[i:i + 1]
                put(xp, n1 * SP, acc * vs[pl.ds(n1 * N2, N2), pl.ds(c0, CB)].astype(F32), (slot,))

        def finish(cb, slot, piece):
            dv = d32[pl.ds(cb, 1), :]
            for n1 in range(4 * piece, 4 * piece + 4):
                kv = _from_words(get(xp, n1 * SP, N2 // 2, 1, (slot,))).astype(F32)
                ob[cb, pl.ds(n1 * N2, N2), :] = (yp[pl.ds(n1 * SY, N2), :] + kv * dv).astype(BF16)

        def b_block(cb, carry):
            @pl.when(cb + 1 < n_cb)
            def _():
                wait_inputs(cb + 1)

            for i in range(n_cb - first_block):
                @pl.when(cb == i + first_block)
                def _(i=i):
                    lo = 0 if i == 0 else n_b_late + i * per_block
                    for c in late[lo:n_b_late + (i + 1) * per_block]:
                        c.start()
            lane = jax.lax.broadcasted_iota(jnp.int32, (1, 128), 1)
            slot = cb % 2
            nxt = jnp.minimum(cb + 1, n_cb - 1)
            prv = jnp.maximum(cb - 1, 0)
            n_pieces = 8

            def side_work(piece):
                finish(prv, 1 - slot, piece)
                prepare(nxt, 1 - slot, piece)

            early_pieces = _CFG["prep_early"]
            for g in range(N2 // 4):
                m = tf[g]
                lhs = _from_words(jnp.concatenate(
                    [jnp.where((lane // 64 == j // 2) & (lane % 2 == j % 2), m, jnp.zeros_like(m))
                     for j in range(4)], axis=0))

                def rhs(ref, g=g):
                    return _from_words(jnp.concatenate(
                        [get(ref, 2 * g, N1, SP, (slot,)), get(ref, 2 * g + 1, N1, SP, (slot,))], axis=0))

                r = _dot(lhs, jnp.concatenate([rhs(xp), rhs(hp)], axis=1))
                for j in range(4):
                    put(zx, (4 * g + j) * SZ, r[2 * N1 * j:2 * N1 * (j + 1), :128])
                    put(zh, (4 * g + j) * SZ, r[2 * N1 * j:2 * N1 * (j + 1), 128:])
                if early_pieces and g % (16 // early_pieces) == 0:
                    side_work(g // (16 // early_pieces))
            f2 = _from_words(t2[0])
            g2 = _from_words(t2[1])

            def stage2(g):
                zz = []
                for k1 in range(g * group, (g + 1) * group):
                    zz += [_from_words(get(zx, k1, N2, SZ)), _from_words(get(zh, k1, N2, SZ))]
                return _dot(f2, jnp.concatenate(zz, axis=1))

            def stage3(g, r):
                ys = []
                for i in range(group):
                    xf = r[:, (2 * i) * 128:(2 * i + 1) * 128]
                    hf = r[:, (2 * i + 1) * 128:(2 * i + 2) * 128]
                    xr, xi, hr, hi = xf[:N2], xf[N2:], hf[:N2], hf[N2:]
                    ys.append(jnp.concatenate([xr * hr - xi * hi, xr * hi + xi * hr], axis=0).astype(BF16))
                t = _dot(g2, jnp.concatenate(ys, axis=1))
                for i in range(group):
                    put(tt, (g * group + i) * ST, t[:, i * 128:(i + 1) * 128])

            n_groups = N1 // group
            late_pieces = list(range(early_pieces, n_pieces))
            r = stage2(0)
            for g in range(n_groups):
                r_next = stage2(g + 1) if g + 1 < n_groups else None
                stage3(g, r)
                r = r_next
                for piece in late_pieces[g::n_groups]:
                    side_work(piece)
            for i in range(N2 // 2):
                m = ti[i]
                lhs = _from_words(jnp.concatenate([jnp.where(lane < 64, m, jnp.zeros_like(m)),
                                                   jnp.where(lane >= 64, m, jnp.zeros_like(m))], axis=0))
                y = _dot(lhs, _from_words(jnp.concatenate(
                    [get(tt, 2 * i, N1, ST), get(tt, 2 * i + 1, N1, ST)], axis=0)))
                yp[pl.ds(2 * i, N1, stride=SY), :] = y[0:N1]
                yp[pl.ds(2 * i + 1, N1, stride=SY), :] = y[N1:2 * N1]
            return carry

        for c in t_copies():
            c.wait()
        sh32[...] = sh_ref[...].astype(F32)
        d32[...] = d_ref[...].astype(F32)
        hbuf[0:n_mem, :] = mem_ref[...].astype(F32)
        wait_inputs(0)
        for c in second:
            c.start()
        for piece in range(8):
            prepare(0, 0, piece)
        jax.lax.fori_loop(0, n_cb, b_block, 0)
        for c in late[n_b_late + (n_cb - first_block) * per_block:]:
            c.start()
        for piece in range(8):
            finish(n_cb - 1, (n_cb - 1) % 2, piece)

        def w_slot(quad, parity, odd_head, m):
            return (w_even, w_odd)[parity], (2 * quad + odd_head) * 3 + m

        def wtile(h, m):
            ref, i = w_slot(h // 4, (h // 2) % 2, h % 2, m)
            return _from_words(ref[i])

        def relayout(m, quad, parity):
            pair = 2 * quad + parity
            if not isinstance(pair, int):
                pair = jnp.minimum(pair, n_hp - 1)
            src = m * n_hp + pair
            even = stage[src, pl.ds(0, d_model // 2, stride=2), :]
            odd = stage[src, pl.ds(1, d_model // 2, stride=2), :]
            ref, i = w_slot(quad, parity, 0, m)
            ref[i] = (even & U32(0xFFFF)) | (odd << 16)
            ref, i = w_slot(quad, parity, 1, m)
            ref[i] = (even >> 16) | (odd & U32(0xFFFF0000))

        for m in range(2):
            for c in w_copies(m):
                c.wait()
        for c in pre_copies():
            c.wait()
        xpre32[...] = xpre[...].astype(F32)
        relayout(0, 0, 0)
        relayout(1, 0, 0)

        def pre_dots(quad, parity, xl):
            for odd_head in range(2):
                for m in range(2):
                    ref, i = w_slot(quad, parity, odd_head, m)
                    qkpre[m, 4 * quad + 2 * parity + odd_head] = _dot(xl, _from_words(ref[i]))

        def pre_round(quad, carry):
            xl = xpre32[...]
            pre_dots(quad, 0, xl)
            relayout(0, quad, 1)
            relayout(1, quad, 1)
            pre_dots(quad, 1, xl)
            relayout(0, quad + 1, 0)
            relayout(1, quad + 1, 0)
            return carry

        jax.lax.fori_loop(0, n_heads // 4, pre_round, 0)
        for c in w_copies(2):
            c.wait()

        def step(s, first, pre=False):
            if first:
                for c in head_copies():
                    c.wait()
            row = jax.lax.broadcasted_iota(jnp.int32, (n_rows, n_rows), 0)
            col = jax.lax.broadcasted_iota(jnp.int32, (n_rows, n_rows), 1)
            mask = (row < n_mem) | (row >= col)
            r0 = s * seg if first else pl.multiple_of(s * seg, seg)
            slot = s
            hbuf[n_mem:n_rows, :] = xin[pl.ds(r0, seg), :].astype(F32)
            hl = hbuf[...]
            if pre:
                hr = jnp.concatenate([hl[0:n_mem], hl[n_mem + pre_rows:n_rows]], axis=0)
                p0 = s * pre_rows if first else pl.multiple_of(s * pre_rows, pre_rows)
            waited = [False] * (len(wo_bounds) - 1)
            for op in (order_first if first else order):
                if op[0] == "P":
                    h = op[1]
                    if first and h % 2 == 0:
                        if h == 0:
                            relayout(2, 0, 0)
                        if h + 2 < n_heads:
                            relayout(2, (h + 2) // 4, (h // 2 + 1) % 2)
                    if pre:
                        rq = _dot(hr, wtile(h, 0))
                        qbuf[h] = jnp.concatenate(
                            [rq[0:n_mem], qkpre[0, h, pl.ds(p0, pre_rows), :], rq[n_mem:]], axis=0)
                        rk = _dot(hr, wtile(h, 1))
                        kbuf[h, 0:n_rows] = jnp.concatenate(
                            [rk[0:n_mem], qkpre[1, h, pl.ds(p0, pre_rows), :], rk[n_mem:]], axis=0).astype(BF16)
                    else:
                        qbuf[h] = _dot(hl, wtile(h, 0))
                        kbuf[h, 0:n_rows] = _dot(hl, wtile(h, 1)).astype(BF16)
                    vbuf[h, 0:n_rows] = _dot(hl, wtile(h, 2)).astype(BF16)
                elif op[0] == "S":
                    h = op[1]
                    sc = _dot_nt(qbuf[h], kbuf[h, 0:n_rows])
                    sc = jnp.where(mask, sc, -1e9 / scale)
                    e = jnp.exp2((sc - jnp.max(sc, axis=-1, keepdims=True)) * exp_scale)
                    den = jnp.sum(e, axis=-1, keepdims=True)
                    inv = pl.reciprocal(den, approx=True)
                    pbuf[h, :, 0:n_rows] = e
                    ibuf[h] = jnp.broadcast_to(inv * (2.0 - den * inv), (n_rows, d_head))
                elif op[0] == "V":
                    h = op[1]
                    obuf[:, h * d_head:(h + 1) * d_head] = (
                        _dot(pbuf[h, :, 0:n_rows], vbuf[h, 0:n_rows]) * ibuf[h])
                elif op[0] == "W":
                    _, j, lo, hi = op
                    if first:
                        for i in range(len(waited)):
                            if not waited[i] and hi > wo_bounds[i]:
                                for c in o_copies(i):
                                    c.wait()
                                waited[i] = True
                                if i == len(waited) - 1:
                                    for ch in range(x_chunks):
                                        for c in chunk_copies(ch):
                                            c.start()
                    w = _from_words(wo[j, lo * d_head // 2:hi * d_head // 2, :])
                    y = _dot(obuf[:, lo * d_head:hi * d_head], w)
                    if lo > 0:
                        y = y + ybuf[j]
                    if hi < n_heads:
                        ybuf[j] = y
                    else:
                        hbuf[0:n_mem, j * 128:(j + 1) * 128] = y[0:n_mem]
                        ost[slot, :, j * 128:(j + 1) * 128] = y[n_mem:n_rows].astype(BF16)
                else:
                    for cb in range(n_cb):
                        gate = qin[pl.ds(r0, seg), cb * CB:(cb + 1) * CB].astype(F32)
                        ost[slot, :, d_model + cb * CB:d_model + (cb + 1) * CB] = (
                            ob[cb, pl.ds(r0, seg), :].astype(F32) * gate).astype(BF16)
            out_copy(s).start()

        unroll = _CFG["unroll"]

        def chunk_body(c, carry, pre=False):
            for cp in chunk_copies(c):
                cp.wait()

            def steps_body(i, carry):
                for u in range(unroll):
                    step(1 + c * steps_per_chunk + i * unroll + u, False, pre)
                return carry

            if steps_per_chunk == unroll:
                steps_body(0, 0)
            else:
                jax.lax.fori_loop(0, steps_per_chunk // unroll, steps_body, 0)
            return carry

        step(0, True, True)
        def pre_step(s, carry):
            @pl.when((s - 1) % steps_per_chunk == 0)
            def _():
                for cp in chunk_copies((s - 1) // steps_per_chunk):
                    cp.wait()

            step(s, False, True)
            return carry

        pre_chunks = n_pre // steps_per_chunk
        if pre_chunks and _CFG["pre_rolled"]:
            jax.lax.fori_loop(1, 1 + n_pre, pre_step, 0)
        elif pre_chunks:
            jax.lax.fori_loop(0, pre_chunks, functools.partial(chunk_body, pre=True), 0)
        jax.lax.fori_loop(pre_chunks, x_chunks, chunk_body, 0)
        for s in range(n_seg):
            out_copy(s).wait()

    return kernel


def _forward(x, mem0, wq, wk, wv, wo, seg_len, q, k, v, shift_k, ssm_k, ssm_d):
    _, seq, d_model = x.shape
    _, n_heads, d_head = wq.shape
    n_mem = mem0.shape[1]
    seg = seg_len
    n_seg = seq // seg
    n_rows = n_mem + seg
    n_cb = d_model // CB
    assert seq == SEQ and d_model == 1024 and d_head == 128 and n_rows % 8 == 0
    tf, ti, t2 = _dft_tables()

    any_spec = pl.BlockSpec(memory_space=pl.ANY)
    kv_rows = -(-n_rows // 16) * 16
    scratch = [
        pltpu.VMEM((n_cb, CB, seq), BF16),
        pltpu.VMEM((seq, d_model), BF16),
        pltpu.VMEM((seq, d_model), BF16),
        pltpu.VMEM((n_cb, seq, CB), BF16),
        pltpu.VMEM((8 + seq, CB), F32),
        pltpu.VMEM((2, 2 * N1 * SP, CB), BF16),
        pltpu.VMEM((2, 2 * N1 * SP, CB), BF16),
        pltpu.VMEM((2 * N2 * SZ, CB), BF16),
        pltpu.VMEM((2 * N2 * SZ, CB), BF16),
        pltpu.VMEM((2 * N1 * ST, CB), BF16),
        pltpu.VMEM((N1 * SY, CB), F32),
        pltpu.VMEM(tf.shape, U32),
        pltpu.VMEM(ti.shape, U32),
        pltpu.VMEM(t2.shape, U32),
        pltpu.VMEM((4, d_model), BF16),
        pltpu.VMEM((n_cb, CB), BF16),
        pltpu.VMEM((n_mem, d_model), BF16),
        pltpu.VMEM((4, d_model), F32),
        pltpu.VMEM((n_cb, CB), F32),
        pltpu.VMEM((3 * n_heads // 2, d_model, d_head), U32),
        pltpu.VMEM((3 * n_heads // 2 + 6, d_model // 2, d_head), U32),
        pltpu.VMEM((3 * n_heads // 2, d_model // 2, d_head), U32),
        pltpu.VMEM((d_model // 128, n_heads * d_head // 2, 128), U32),
        pltpu.VMEM((seq, d_model), BF16),
        pltpu.VMEM((seq, d_model), BF16),
        pltpu.VMEM((n_seg, seg, 2 * d_model), BF16),
        pltpu.VMEM((n_rows, d_model), F32),
        pltpu.VMEM((n_heads, n_rows, d_head), F32),
        pltpu.VMEM((n_heads, kv_rows, d_head), BF16),
        pltpu.VMEM((n_heads, kv_rows, d_head), BF16),
        pltpu.VMEM((n_rows, n_heads * d_head), F32),
        pltpu.VMEM((n_heads, n_rows, d_head), F32),
        pltpu.VMEM((n_heads, n_rows, d_head), F32),
        pltpu.VMEM((d_model // 128, n_rows, 128), F32),
        pltpu.VMEM(((_CFG["n_pre"] + 1) * 8, d_model), BF16),
        pltpu.VMEM(((_CFG["n_pre"] + 1) * 8, d_model), F32),
        pltpu.VMEM((2, n_heads, (_CFG["n_pre"] + 1) * 8, d_head), F32),
        pltpu.SemaphoreType.DMA((3, n_cb)),
        pltpu.SemaphoreType.DMA((6,)),
        pltpu.SemaphoreType.DMA((3,)),
        pltpu.SemaphoreType.DMA((len(_CFG["first_splits"]) + 1,)),
        pltpu.SemaphoreType.DMA((2,)),
        pltpu.SemaphoreType.DMA(()),
        pltpu.SemaphoreType.DMA((n_seg,)),
        pltpu.SemaphoreType.DMA((n_seg,)),
        pltpu.SemaphoreType.DMA(()),
    ]
    out = pl.pallas_call(
        _make_kernel(n_heads, d_head, d_model, n_mem, seg, n_seg),
        out_shape=jax.ShapeDtypeStruct((seq, 2 * d_model), BF16),
        in_specs=[any_spec] * 15,
        out_specs=any_spec,
        scratch_shapes=scratch,
        compiler_params=pltpu.CompilerParams(vmem_limit_bytes=120 * 1024 * 1024),
    )(shift_k.T, ssm_d.reshape(n_cb, CB), mem0.reshape(n_mem, d_model),
      x.reshape(seq, d_model), wq, wk, wv, wo.reshape(n_heads * d_head, d_model),
      q.reshape(seq, d_model), k.reshape(seq, d_model), v.reshape(seq, d_model), ssm_k,
      tf, ti, t2)
    return out.reshape(1, seq, 2 * d_model)


def pallas_concat_heads__memory_aug_recurrent_mem_tr__ssm_conv_h3__prompt_kernel(
        A_x, A_mem0, A_Wq, A_Wk, A_Wv, A_Wo, A_seg_len, B_q, B_k, B_v, B_shift_k, B_ssm_k, B_ssm_D):
    return _forward(A_x, A_mem0, A_Wq, A_Wk, A_Wv, A_Wo, int(A_seg_len), B_q, B_k, B_v,
                    B_shift_k, B_ssm_k, B_ssm_D)
```

```python
import functools
import math

import jax
import jax.numpy as jnp
import numpy as np
from jax.experimental import pallas as pl
from jax.experimental.pallas import tpu as pltpu

F32 = jnp.float32
BF16 = jnp.bfloat16
U32 = jnp.uint32

N1, N2 = 32, 64
SEQ = N1 * N2
SP = N2 // 2 + 4
SZ = N1 + 4
ST = N2 + 4
SY = N2 + 4
CB = 128


def _dft_tables():
    theta = np.pi / (2 * SEQ)
    lane = np.arange(128)[None, :]
    hi, mid, lo = lane // 64, (lane % 64) // 2, lane % 2
    k1 = np.arange(N1)[:, None]
    fwd = np.zeros((N2 // 4, 2 * N1, 128))
    for g in range(N2 // 4):
        ph = theta * (4 * k1 + 1) * (N2 * mid + 4 * g + 2 * hi + lo)
        fwd[g, 0::2] = np.cos(ph)
        fwd[g, 1::2] = np.sin(ph)
    n1 = np.arange(N1)[:, None]
    inv = np.zeros((N2 // 2, N1, 128))
    for i in range(N2 // 2):
        ph = theta * (4 * mid + 1) * (N2 * n1 + 2 * i + hi)
        inv[i] = np.where(lo == 0, np.cos(ph), np.sin(ph)) / SEQ
    ph = 2 * np.pi * np.arange(N2)[:, None] * np.arange(N2)[None, :] / N2
    c, s = np.cos(ph), np.sin(ph)
    f2 = np.zeros((128, 128))
    f2[:N2, 0::2], f2[:N2, 1::2], f2[N2:, 0::2], f2[N2:, 1::2] = c, -s, s, c
    g2 = np.zeros((128, 128))
    g2[0::2, :N2], g2[0::2, N2:], g2[1::2, :N2], g2[1::2, N2:] = c.T, s.T, -s.T, c.T

    def as_words(a):
        u = a.astype(np.float32).astype(BF16).view(np.uint16).astype(np.uint32)
        return u[..., 0::2, :] | (u[..., 1::2, :] << 16)

    return as_words(fwd), as_words(inv), as_words(np.stack([f2, g2]))


def _to_words(x):
    return pltpu.bitcast(x.astype(BF16), U32)


def _from_words(w):
    return pltpu.bitcast(w, BF16)


_CFG = dict(group=8, lag_s=2, lag_v=3, wo_split=16, gate_at=1, late_first=0, late_per_block=10, b_group=4, n_early=2, unroll=3, chunk_steps=3, first_splits=(16,),
            n_pre=18, pre_rolled=1)


def _step_order(n_heads, n_out_tiles, first=False):
    g, a, b = _CFG["group"], _CFG["lag_s"], _CFG["lag_v"]
    split = _CFG["wo_split"]
    n_groups = n_heads // g
    total = n_groups + a + b
    early = [("W", j, 0, split) for j in range(n_out_tiles)] if split < n_heads else []
    ops = []
    for t in range(total):
        if t < n_groups:
            ops += [("P", h) for h in range(t * g, (t + 1) * g)]
        if t == _CFG["gate_at"]:
            ops.append(("G",))
        if 0 <= t - a < n_groups:
            ops += [("S", h) for h in range((t - a) * g, (t - a + 1) * g)]
        if 0 <= t - a - b < n_groups:
            ops += [("V", h) for h in range((t - a - b) * g, (t - a - b + 1) * g)]
        if early and (t - a - b + 1) * g >= split:
            n = -(-len(early) // (total - t))
            ops += early[:n]
            early = early[n:]
    ops += early
    bounds = [split if split < n_heads else 0]
    if first:
        bounds += [b for b in _CFG["first_splits"] if b > split]
    for lo, hi in zip(bounds, bounds[1:] + [n_heads]):
        ops += [("W", j, lo, hi) for j in range(n_out_tiles)]
    return ops


def _dot(a, b):
    return jnp.dot(a, b, preferred_element_type=F32)


def _dot_nt(a, b):
    return jax.lax.dot_general(a, b, (((1,), (1,)), ((), ())), preferred_element_type=F32)


def _make_kernel(n_heads, d_head, d_model, n_mem, seg, n_seg):
    n_rows = n_mem + seg
    n_cb = d_model // CB
    n_hp = n_heads // 2
    scale = d_head ** (-0.5)
    exp_scale = scale * math.log2(math.e)
    steps_per_chunk = _CFG["chunk_steps"]
    x_chunks = (n_seg - 1) // steps_per_chunk
    x_rows = steps_per_chunk * seg
    assert x_chunks * steps_per_chunk == n_seg - 1 and steps_per_chunk % _CFG["unroll"] == 0
    n_pre = _CFG["n_pre"]
    pre_rows = 8
    assert n_pre % steps_per_chunk == 0
    order = _step_order(n_heads, d_model // 128)
    order_first = _step_order(n_heads, d_model // 128, True)
    wo_bounds = [0] + list(_CFG["first_splits"]) + [n_heads]

    def kernel(sh_hbm, d_hbm, mem_hbm,
               x_hbm, wq_hbm, wk_hbm, wv_hbm, wo_hbm,
               q_hbm, k_hbm, v_hbm, h_hbm, tf_hbm, ti_hbm, t2_hbm,
               out_hbm,
               hs, ks, vs, ob, kf, xp, hp, zx, zh, tt, yp, tf, ti, t2, sh_ref, d_ref, mem_ref, sh32, d32,
               stage, w_even, w_odd, wo, xin, qin, ost, hbuf, qbuf, kbuf, vbuf, obuf, pbuf, ibuf, ybuf, xpre, xpre32, qkpre,
               sem_b, sem_t, sem_w, sem_o, sem_h, sem_p, sem_x, sem_q, sem_out):

        n_early = _CFG["n_early"]

        def h_copy(cb):
            c0 = cb * CB if isinstance(cb, int) else pl.multiple_of(cb * CB, CB)
            return pltpu.make_async_copy(h_hbm.at[pl.ds(c0, CB), :], hs.at[cb], sem_b.at[0, cb])

        def kv_copies(cb):
            if isinstance(cb, int):
                c0, width = cb * CB, (CB if cb < n_early else d_model - n_early * CB)
            else:
                c0, width = pl.multiple_of(cb * CB, CB), CB
            return [pltpu.make_async_copy(src.at[:, pl.ds(c0, width)], dst.at[:, pl.ds(c0, width)], sem_b.at[1 + i, cb])
                    for i, (src, dst) in enumerate(((k_hbm, ks), (v_hbm, vs)))]

        def t_copies():
            pairs = ((sh_hbm, sh_ref), (d_hbm, d_ref), (mem_hbm, mem_ref),
                     (tf_hbm, tf), (ti_hbm, ti), (t2_hbm, t2))
            return [pltpu.make_async_copy(src, dst, sem_t.at[i]) for i, (src, dst) in enumerate(pairs)]

        def w_copies(m):
            w32 = (wq_hbm, wk_hbm, wv_hbm)[m].bitcast(U32)
            return [pltpu.make_async_copy(w32.at[:, hp, :], stage.at[m * n_hp + hp], sem_w.at[m])
                    for hp in range(n_hp)]

        def o_copies(i):
            wo32 = wo_hbm.bitcast(U32)
            lo, hi = wo_bounds[i] * d_head // 2, wo_bounds[i + 1] * d_head // 2
            return [pltpu.make_async_copy(wo32.at[pl.ds(lo, hi - lo), pl.ds(j * 128, 128)],
                                          wo.at[j, pl.ds(lo, hi - lo), :], sem_o.at[i])
                    for j in range(d_model // 128)]

        def head_copies():
            return [pltpu.make_async_copy(src.at[pl.ds(0, seg), :], dst.at[pl.ds(0, seg), :], sem_h.at[i])
                    for i, (src, dst) in enumerate(((x_hbm, xin), (q_hbm, qin)))]

        def pre_copies():
            return [pltpu.make_async_copy(x_hbm.at[pl.ds(i * seg, pre_rows), :],
                                          xpre.at[pl.ds(i * pre_rows, pre_rows), :], sem_p) for i in range(n_pre + 1)]

        def chunk_copies(c):
            r0 = seg + c * x_rows if isinstance(c, int) else pl.multiple_of(seg + c * x_rows, seg)
            return [pltpu.make_async_copy(src.at[pl.ds(r0, x_rows), :], dst.at[pl.ds(r0, x_rows), :], sem.at[c])
                    for src, dst, sem in ((x_hbm, xin, sem_x), (q_hbm, qin, sem_q))]

        def out_copy(s):
            r0 = s * seg if isinstance(s, int) else pl.multiple_of(s * seg, seg)
            return pltpu.make_async_copy(ost.at[s], out_hbm.at[pl.ds(r0, seg), :], sem_out)

        tc = t_copies()
        for c in tc[:3] + kv_copies(0) + [h_copy(0)] + tc[3:]:
            c.start()
        for cb in range(1, n_early):
            for c in [h_copy(cb)] + kv_copies(cb):
                c.start()
        late = kv_copies(n_early) + [h_copy(cb) for cb in range(n_early, n_cb)]
        n_b_late = len(late)
        late += w_copies(0) + pre_copies() + w_copies(1) + w_copies(2) + head_copies()
        for i in range(len(wo_bounds) - 1):
            late += o_copies(i)
        per_block = _CFG["late_per_block"]
        first_block = _CFG["late_first"]

        kf[0:8, :] = jnp.zeros((8, CB), F32)

        group = _CFG["b_group"]

        def put(ref, row, x):
            ref[pl.ds(2 * row, x.shape[0]), :] = x.astype(BF16)

        def get(ref, row, n, stride=1):
            return ref.bitcast(U32)[pl.ds(row, n, stride=stride), :]

        def wait_inputs(cb):
            h_copy(cb).wait()

            @pl.when(cb < n_early)
            def _():
                for c in kv_copies(cb):
                    c.wait()

            @pl.when(cb == n_early)
            def _():
                for c in kv_copies(n_early):
                    c.wait()

        def prepare(cb):
            c0 = pl.multiple_of(cb * CB, CB)
            kf[8:8 + SEQ, :] = ks[:, pl.ds(c0, CB)].astype(F32)
            for j in range(SEQ // 128):
                r = hs[cb, :, j * 128:(j + 1) * 128].astype(F32).T
                put(hp, (2 * j) * SP, r[0:N2])
                put(hp, (2 * j + 1) * SP, r[N2:2 * N2])
            taps = sh32[:, pl.ds(c0, CB)]
            for n1 in range(N1):
                acc = kf[pl.ds(8 + n1 * N2, N2), :] * taps[0:1]
                for i in range(1, 4):
                    acc = acc + kf[pl.ds(8 - i + n1 * N2, N2), :] * taps[i:i + 1]
                put(xp, n1 * SP, acc * vs[pl.ds(n1 * N2, N2), pl.ds(c0, CB)].astype(F32))

        def finish(cb):
            dv = d32[pl.ds(cb, 1), :]
            for n1 in range(N1):
                kv = _from_words(get(xp, n1 * SP, N2 // 2)).astype(F32)
                ob[cb, pl.ds(n1 * N2, N2), :] = (yp[pl.ds(n1 * SY, N2), :] + kv * dv).astype(BF16)

        def b_block(cb, carry):
            wait_inputs(cb)
            for i in range(n_cb - first_block):
                @pl.when(cb == i + first_block)
                def _(i=i):
                    lo = 0 if i == 0 else n_b_late + i * per_block
                    for c in late[lo:n_b_late + (i + 1) * per_block]:
                        c.start()
            lane = jax.lax.broadcasted_iota(jnp.int32, (1, 128), 1)
            prepare(cb)
            for g in range(N2 // 4):
                m = tf[g]
                lhs = _from_words(jnp.concatenate(
                    [jnp.where((lane // 64 == j // 2) & (lane % 2 == j % 2), m, jnp.zeros_like(m))
                     for j in range(4)], axis=0))

                def rhs(ref, g=g):
                    return _from_words(jnp.concatenate(
                        [get(ref, 2 * g, N1, SP), get(ref, 2 * g + 1, N1, SP)], axis=0))

                r = _dot(lhs, jnp.concatenate([rhs(xp), rhs(hp)], axis=1))
                for j in range(4):
                    put(zx, (4 * g + j) * SZ, r[2 * N1 * j:2 * N1 * (j + 1), :128])
                    put(zh, (4 * g + j) * SZ, r[2 * N1 * j:2 * N1 * (j + 1), 128:])
            f2 = _from_words(t2[0])
            g2 = _from_words(t2[1])

            def stage2(g):
                zz = []
                for k1 in range(g * group, (g + 1) * group):
                    zz += [_from_words(get(zx, k1, N2, SZ)), _from_words(get(zh, k1, N2, SZ))]
                return _dot(f2, jnp.concatenate(zz, axis=1))

            def stage3(g, r):
                ys = []
                for i in range(group):
                    xf = r[:, (2 * i) * 128:(2 * i + 1) * 128]
                    hf = r[:, (2 * i + 1) * 128:(2 * i + 2) * 128]
                    xr, xi, hr, hi = xf[:N2], xf[N2:], hf[:N2], hf[N2:]
                    ys.append(jnp.concatenate([xr * hr - xi * hi, xr * hi + xi * hr], axis=0).astype(BF16))
                t = _dot(g2, jnp.concatenate(ys, axis=1))
                for i in range(group):
                    put(tt, (g * group + i) * ST, t[:, i * 128:(i + 1) * 128])

            n_groups = N1 // group
            r = stage2(0)
            for g in range(n_groups):
                r_next = stage2(g + 1) if g + 1 < n_groups else None
                stage3(g, r)
                r = r_next
            for i in range(N2 // 2):
                m = ti[i]
                lhs = _from_words(jnp.concatenate([jnp.where(lane < 64, m, jnp.zeros_like(m)),
                                                   jnp.where(lane >= 64, m, jnp.zeros_like(m))], axis=0))
                y = _dot(lhs, _from_words(jnp.concatenate(
                    [get(tt, 2 * i, N1, ST), get(tt, 2 * i + 1, N1, ST)], axis=0)))
                yp[pl.ds(2 * i, N1, stride=SY), :] = y[0:N1]
                yp[pl.ds(2 * i + 1, N1, stride=SY), :] = y[N1:2 * N1]
            finish(cb)
            return carry

        for c in tc:
            c.wait()
        sh32[...] = sh_ref[...].astype(F32)
        d32[...] = d_ref[...].astype(F32)
        hbuf[0:n_mem, :] = mem_ref[...].astype(F32)
        jax.lax.fori_loop(0, n_cb, b_block, 0)
        for c in late[n_b_late + (n_cb - first_block) * per_block:]:
            c.start()

        def w_slot(quad, parity, odd_head, m):
            return (w_even, w_odd)[parity], (2 * quad + odd_head) * 3 + m

        def wtile(h, m):
            ref, i = w_slot(h // 4, (h // 2) % 2, h % 2, m)
            return _from_words(ref[i])

        def relayout(m, quad, parity):
            pair = 2 * quad + parity
            if not isinstance(pair, int):
                pair = jnp.minimum(pair, n_hp - 1)
            src = m * n_hp + pair
            even = stage[src, pl.ds(0, d_model // 2, stride=2), :]
            odd = stage[src, pl.ds(1, d_model // 2, stride=2), :]
            ref, i = w_slot(quad, parity, 0, m)
            ref[i] = (even & U32(0xFFFF)) | (odd << 16)
            ref, i = w_slot(quad, parity, 1, m)
            ref[i] = (even >> 16) | (odd & U32(0xFFFF0000))

        for m in range(2):
            for c in w_copies(m):
                c.wait()
        for c in pre_copies():
            c.wait()
        xpre32[...] = xpre[...].astype(F32)
        relayout(0, 0, 0)
        relayout(1, 0, 0)

        def pre_dots(quad, parity, xl):
            for odd_head in range(2):
                for m in range(2):
                    ref, i = w_slot(quad, parity, odd_head, m)
                    qkpre[m, 4 * quad + 2 * parity + odd_head] = _dot(xl, _from_words(ref[i]))

        def pre_round(quad, carry):
            xl = xpre32[...]
            pre_dots(quad, 0, xl)
            relayout(0, quad, 1)
            relayout(1, quad, 1)
            pre_dots(quad, 1, xl)
            relayout(0, quad + 1, 0)
            relayout(1, quad + 1, 0)
            return carry

        jax.lax.fori_loop(0, n_heads // 4, pre_round, 0)
        for c in w_copies(2):
            c.wait()

        def step(s, first, pre=False):
            if first:
                for c in head_copies():
                    c.wait()
            row = jax.lax.broadcasted_iota(jnp.int32, (n_rows, n_rows), 0)
            col = jax.lax.broadcasted_iota(jnp.int32, (n_rows, n_rows), 1)
            mask = (row < n_mem) | (row >= col)
            r0 = s * seg if first else pl.multiple_of(s * seg, seg)
            slot = s
            hbuf[n_mem:n_rows, :] = xin[pl.ds(r0, seg), :].astype(F32)
            hl = hbuf[...]
            if pre:
                hr = jnp.concatenate([hl[0:n_mem], hl[n_mem + pre_rows:n_rows]], axis=0)
                p0 = s * pre_rows if first else pl.multiple_of(s * pre_rows, pre_rows)
            waited = [False] * (len(wo_bounds) - 1)
            for op in (order_first if first else order):
                if op[0] == "P":
                    h = op[1]
                    if first and h % 2 == 0:
                        if h == 0:
                            relayout(2, 0, 0)
                        if h + 2 < n_heads:
                            relayout(2, (h + 2) // 4, (h // 2 + 1) % 2)
                    if pre:
                        rq = _dot(hr, wtile(h, 0))
                        qbuf[h] = jnp.concatenate(
                            [rq[0:n_mem], qkpre[0, h, pl.ds(p0, pre_rows), :], rq[n_mem:]], axis=0)
                        rk = _dot(hr, wtile(h, 1))
                        kbuf[h, 0:n_rows] = jnp.concatenate(
                            [rk[0:n_mem], qkpre[1, h, pl.ds(p0, pre_rows), :], rk[n_mem:]], axis=0).astype(BF16)
                    else:
                        qbuf[h] = _dot(hl, wtile(h, 0))
                        kbuf[h, 0:n_rows] = _dot(hl, wtile(h, 1)).astype(BF16)
                    vbuf[h, 0:n_rows] = _dot(hl, wtile(h, 2)).astype(BF16)
                elif op[0] == "S":
                    h = op[1]
                    sc = _dot_nt(qbuf[h], kbuf[h, 0:n_rows])
                    sc = jnp.where(mask, sc, -1e9 / scale)
                    e = jnp.exp2((sc - jnp.max(sc, axis=-1, keepdims=True)) * exp_scale)
                    den = jnp.sum(e, axis=-1, keepdims=True)
                    inv = pl.reciprocal(den, approx=True)
                    pbuf[h, :, 0:n_rows] = e
                    ibuf[h] = jnp.broadcast_to(inv * (2.0 - den * inv), (n_rows, d_head))
                elif op[0] == "V":
                    h = op[1]
                    obuf[:, h * d_head:(h + 1) * d_head] = (
                        _dot(pbuf[h, :, 0:n_rows], vbuf[h, 0:n_rows]) * ibuf[h])
                elif op[0] == "W":
                    _, j, lo, hi = op
                    if first:
                        for i in range(len(waited)):
                            if not waited[i] and hi > wo_bounds[i]:
                                for c in o_copies(i):
                                    c.wait()
                                waited[i] = True
                                if i == len(waited) - 1:
                                    for ch in range(x_chunks):
                                        for c in chunk_copies(ch):
                                            c.start()
                    w = _from_words(wo[j, lo * d_head // 2:hi * d_head // 2, :])
                    y = _dot(obuf[:, lo * d_head:hi * d_head], w)
                    if lo > 0:
                        y = y + ybuf[j]
                    if hi < n_heads:
                        ybuf[j] = y
                    else:
                        hbuf[0:n_mem, j * 128:(j + 1) * 128] = y[0:n_mem]
                        ost[slot, :, j * 128:(j + 1) * 128] = y[n_mem:n_rows].astype(BF16)
                else:
                    for cb in range(n_cb):
                        gate = qin[pl.ds(r0, seg), cb * CB:(cb + 1) * CB].astype(F32)
                        ost[slot, :, d_model + cb * CB:d_model + (cb + 1) * CB] = (
                            ob[cb, pl.ds(r0, seg), :].astype(F32) * gate).astype(BF16)
            out_copy(s).start()

        unroll = _CFG["unroll"]

        def chunk_body(c, carry, pre=False):
            for cp in chunk_copies(c):
                cp.wait()

            def steps_body(i, carry):
                for u in range(unroll):
                    step(1 + c * steps_per_chunk + i * unroll + u, False, pre)
                return carry

            if steps_per_chunk == unroll:
                steps_body(0, 0)
            else:
                jax.lax.fori_loop(0, steps_per_chunk // unroll, steps_body, 0)
            return carry

        step(0, True, True)
        def pre_step(s, carry):
            @pl.when((s - 1) % steps_per_chunk == 0)
            def _():
                for cp in chunk_copies((s - 1) // steps_per_chunk):
                    cp.wait()

            step(s, False, True)
            return carry

        pre_chunks = n_pre // steps_per_chunk
        if pre_chunks and _CFG["pre_rolled"]:
            jax.lax.fori_loop(1, 1 + n_pre, pre_step, 0)
        elif pre_chunks:
            jax.lax.fori_loop(0, pre_chunks, functools.partial(chunk_body, pre=True), 0)
        jax.lax.fori_loop(pre_chunks, x_chunks, chunk_body, 0)
        for s in range(n_seg):
            out_copy(s).wait()

    return kernel


def _forward(x, mem0, wq, wk, wv, wo, seg_len, q, k, v, shift_k, ssm_k, ssm_d):
    _, seq, d_model = x.shape
    _, n_heads, d_head = wq.shape
    n_mem = mem0.shape[1]
    seg = seg_len
    n_seg = seq // seg
    n_rows = n_mem + seg
    n_cb = d_model // CB
    assert seq == SEQ and d_model == 1024 and d_head == 128 and n_rows % 8 == 0
    tf, ti, t2 = _dft_tables()

    any_spec = pl.BlockSpec(memory_space=pl.ANY)
    kv_rows = -(-n_rows // 16) * 16
    scratch = [
        pltpu.VMEM((n_cb, CB, seq), BF16),
        pltpu.VMEM((seq, d_model), BF16),
        pltpu.VMEM((seq, d_model), BF16),
        pltpu.VMEM((n_cb, seq, CB), BF16),
        pltpu.VMEM((8 + seq, CB), F32),
        pltpu.VMEM((2 * N1 * SP, CB), BF16),
        pltpu.VMEM((2 * N1 * SP, CB), BF16),
        pltpu.VMEM((2 * N2 * SZ, CB), BF16),
        pltpu.VMEM((2 * N2 * SZ, CB), BF16),
        pltpu.VMEM((2 * N1 * ST, CB), BF16),
        pltpu.VMEM((N1 * SY, CB), F32),
        pltpu.VMEM(tf.shape, U32),
        pltpu.VMEM(ti.shape, U32),
        pltpu.VMEM(t2.shape, U32),
        pltpu.VMEM((4, d_model), BF16),
        pltpu.VMEM((n_cb, CB), BF16),
        pltpu.VMEM((n_mem, d_model), BF16),
        pltpu.VMEM((4, d_model), F32),
        pltpu.VMEM((n_cb, CB), F32),
        pltpu.VMEM((3 * n_heads // 2, d_model, d_head), U32),
        pltpu.VMEM((3 * n_heads // 2 + 6, d_model // 2, d_head), U32),
        pltpu.VMEM((3 * n_heads // 2, d_model // 2, d_head), U32),
        pltpu.VMEM((d_model // 128, n_heads * d_head // 2, 128), U32),
        pltpu.VMEM((seq, d_model), BF16),
        pltpu.VMEM((seq, d_model), BF16),
        pltpu.VMEM((n_seg, seg, 2 * d_model), BF16),
        pltpu.VMEM((n_rows, d_model), F32),
        pltpu.VMEM((n_heads, n_rows, d_head), F32),
        pltpu.VMEM((n_heads, kv_rows, d_head), BF16),
        pltpu.VMEM((n_heads, kv_rows, d_head), BF16),
        pltpu.VMEM((n_rows, n_heads * d_head), F32),
        pltpu.VMEM((n_heads, n_rows, d_head), F32),
        pltpu.VMEM((n_heads, n_rows, d_head), F32),
        pltpu.VMEM((d_model // 128, n_rows, 128), F32),
        pltpu.VMEM(((_CFG["n_pre"] + 1) * 8, d_model), BF16),
        pltpu.VMEM(((_CFG["n_pre"] + 1) * 8, d_model), F32),
        pltpu.VMEM((2, n_heads, (_CFG["n_pre"] + 1) * 8, d_head), F32),
        pltpu.SemaphoreType.DMA((3, n_cb)),
        pltpu.SemaphoreType.DMA((6,)),
        pltpu.SemaphoreType.DMA((3,)),
        pltpu.SemaphoreType.DMA((len(_CFG["first_splits"]) + 1,)),
        pltpu.SemaphoreType.DMA((2,)),
        pltpu.SemaphoreType.DMA(()),
        pltpu.SemaphoreType.DMA((n_seg,)),
        pltpu.SemaphoreType.DMA((n_seg,)),
        pltpu.SemaphoreType.DMA(()),
    ]
    out = pl.pallas_call(
        _make_kernel(n_heads, d_head, d_model, n_mem, seg, n_seg),
        out_shape=jax.ShapeDtypeStruct((seq, 2 * d_model), BF16),
        in_specs=[any_spec] * 15,
        out_specs=any_spec,
        scratch_shapes=scratch,
        compiler_params=pltpu.CompilerParams(vmem_limit_bytes=120 * 1024 * 1024),
    )(shift_k.T, ssm_d.reshape(n_cb, CB), mem0.reshape(n_mem, d_model),
      x.reshape(seq, d_model), wq, wk, wv, wo.reshape(n_heads * d_head, d_model),
      q.reshape(seq, d_model), k.reshape(seq, d_model), v.reshape(seq, d_model), ssm_k,
      tf, ti, t2)
    return out.reshape(1, seq, 2 * d_model)


def pallas_concat_heads__memory_aug_recurrent_mem_tr__ssm_conv_h3__prompt_kernel(
        A_x, A_mem0, A_Wq, A_Wk, A_Wv, A_Wo, A_seg_len, B_q, B_k, B_v, B_shift_k, B_ssm_k, B_ssm_D):
    return _forward(A_x, A_mem0, A_Wq, A_Wk, A_Wv, A_Wo, int(A_seg_len), B_q, B_k, B_v,
                    B_shift_k, B_ssm_k, B_ssm_D)
```

```python
import functools
import math

import jax
import jax.numpy as jnp
import numpy as np
from jax.experimental import pallas as pl
from jax.experimental.pallas import tpu as pltpu

F32 = jnp.float32
BF16 = jnp.bfloat16
U32 = jnp.uint32

N1, N2 = 32, 64
SEQ = N1 * N2
SP = N2 // 2 + 4
SZ = N1 + 4
ST = N2 + 4
CB = 128


def _dft_tables():
    theta = np.pi / (2 * SEQ)
    lane = np.arange(128)[None, :]
    hi, mid, lo = lane // 64, (lane % 64) // 2, lane % 2
    k1 = np.arange(N1)[:, None]
    fwd = np.zeros((N2 // 4, 2 * N1, 128))
    for g in range(N2 // 4):
        ph = theta * (4 * k1 + 1) * (N2 * mid + 4 * g + 2 * hi + lo)
        fwd[g, 0::2] = np.cos(ph)
        fwd[g, 1::2] = np.sin(ph)
    n1 = np.arange(N1)[:, None]
    inv = np.zeros((N2 // 2, N1, 128))
    for i in range(N2 // 2):
        ph = theta * (4 * mid + 1) * (N2 * n1 + 2 * i + hi)
        inv[i] = np.where(lo == 0, np.cos(ph), np.sin(ph)) / SEQ
    ph = 2 * np.pi * np.arange(N2)[:, None] * np.arange(N2)[None, :] / N2
    c, s = np.cos(ph), np.sin(ph)
    f2 = np.zeros((128, 128))
    f2[:N2, 0::2], f2[:N2, 1::2], f2[N2:, 0::2], f2[N2:, 1::2] = c, -s, s, c
    g2 = np.zeros((128, 128))
    g2[0::2, :N2], g2[0::2, N2:], g2[1::2, :N2], g2[1::2, N2:] = c.T, s.T, -s.T, c.T

    def as_words(a):
        u = a.astype(np.float32).astype(BF16).view(np.uint16).astype(np.uint32)
        return u[..., 0::2, :] | (u[..., 1::2, :] << 16)

    inv = np.repeat(inv, 2, axis=1)
    return as_words(fwd), as_words(inv), as_words(np.stack([f2, g2]))


def _to_words(x):
    return pltpu.bitcast(x.astype(BF16), U32)


def _from_words(w):
    return pltpu.bitcast(w, BF16)


_CFG = dict(group=8, lag_s=2, lag_v=3, wo_split=16, gate_at=1, late_first=0, late_per_block=10, b_group=8, n_early=2, unroll=3, chunk_steps=3, first_splits=(16,),
            n_pre=18, pre_rolled=1)


def _step_order(n_heads, n_out_tiles, first=False):
    g, a, b = _CFG["group"], _CFG["lag_s"], _CFG["lag_v"]
    split = _CFG["wo_split"]
    n_groups = n_heads // g
    total = n_groups + a + b
    early = [("W", j, 0, split) for j in range(n_out_tiles)] if split < n_heads else []
    ops = []
    for t in range(total):
        if t < n_groups:
            ops += [("P", h) for h in range(t * g, (t + 1) * g)]
        if t == _CFG["gate_at"]:
            ops.append(("G",))
        if 0 <= t - a < n_groups:
            ops += [("S", h) for h in range((t - a) * g, (t - a + 1) * g)]
        if 0 <= t - a - b < n_groups:
            ops += [("V", h) for h in range((t - a - b) * g, (t - a - b + 1) * g)]
        if early and (t - a - b + 1) * g >= split:
            n = -(-len(early) // (total - t))
            ops += early[:n]
            early = early[n:]
    ops += early
    bounds = [split if split < n_heads else 0]
    if first:
        bounds += [b for b in _CFG["first_splits"] if b > split]
    for lo, hi in zip(bounds, bounds[1:] + [n_heads]):
        ops += [("W", j, lo, hi) for j in range(n_out_tiles)]
    return ops


def _dot(a, b):
    return jnp.dot(a, b, preferred_element_type=F32)


def _dot_nt(a, b):
    return jax.lax.dot_general(a, b, (((1,), (1,)), ((), ())), preferred_element_type=F32)


def _make_kernel(n_heads, d_head, d_model, n_mem, seg, n_seg):
    n_rows = n_mem + seg
    n_cb = d_model // CB
    n_hp = n_heads // 2
    scale = d_head ** (-0.5)
    exp_scale = scale * math.log2(math.e)
    steps_per_chunk = _CFG["chunk_steps"]
    x_chunks = (n_seg - 1) // steps_per_chunk
    x_rows = steps_per_chunk * seg
    assert x_chunks * steps_per_chunk == n_seg - 1 and steps_per_chunk % _CFG["unroll"] == 0
    n_pre = _CFG["n_pre"]
    pre_rows = 8
    assert n_pre % steps_per_chunk == 0
    order = _step_order(n_heads, d_model // 128)
    order_first = _step_order(n_heads, d_model // 128, True)
    wo_bounds = [0] + list(_CFG["first_splits"]) + [n_heads]

    def kernel(sh_hbm, d_hbm, mem_hbm,
               x_hbm, wq_hbm, wk_hbm, wv_hbm, wo_hbm,
               q_hbm, k_hbm, v_hbm, h_hbm, tf_hbm, ti_hbm, t2_hbm,
               out_hbm,
               hs, ks, vs, ob, kf, xp, hp, zx, zh, tt, tf, ti, t2, sh_ref, d_ref, mem_ref, sh32, d32,
               stage, w_even, w_odd, wo, xin, qin, ost, hbuf, qbuf, kbuf, vbuf, obuf, pbuf, ibuf, ybuf, xpre, xpre32, qkpre,
               sem_b, sem_t, sem_w, sem_o, sem_h, sem_p, sem_x, sem_q, sem_out):

        n_early = _CFG["n_early"]

        def h_copy(cb):
            c0 = cb * CB if isinstance(cb, int) else pl.multiple_of(cb * CB, CB)
            return pltpu.make_async_copy(h_hbm.at[pl.ds(c0, CB), :], hs.at[cb], sem_b.at[0, cb])

        def kv_copies(cb):
            if isinstance(cb, int):
                c0, width = cb * CB, (CB if cb < n_early else d_model - n_early * CB)
            else:
                c0, width = pl.multiple_of(cb * CB, CB), CB
            return [pltpu.make_async_copy(src.at[:, pl.ds(c0, width)], dst.at[:, pl.ds(c0, width)], sem_b.at[1 + i, cb])
                    for i, (src, dst) in enumerate(((k_hbm, ks), (v_hbm, vs)))]

        def t_copies():
            pairs = ((sh_hbm, sh_ref), (d_hbm, d_ref), (mem_hbm, mem_ref),
                     (tf_hbm, tf), (ti_hbm, ti), (t2_hbm, t2))
            return [pltpu.make_async_copy(src, dst, sem_t.at[i]) for i, (src, dst) in enumerate(pairs)]

        def w_copies(m):
            w32 = (wq_hbm, wk_hbm, wv_hbm)[m].bitcast(U32)
            return [pltpu.make_async_copy(w32.at[:, hp, :], stage.at[m * n_hp + hp], sem_w.at[m])
                    for hp in range(n_hp)]

        def o_copies(i):
            wo32 = wo_hbm.bitcast(U32)
            lo, hi = wo_bounds[i] * d_head // 2, wo_bounds[i + 1] * d_head // 2
            return [pltpu.make_async_copy(wo32.at[pl.ds(lo, hi - lo), pl.ds(j * 128, 128)],
                                          wo.at[j, pl.ds(lo, hi - lo), :], sem_o.at[i])
                    for j in range(d_model // 128)]

        def head_copies():
            return [pltpu.make_async_copy(src.at[pl.ds(0, seg), :], dst.at[pl.ds(0, seg), :], sem_h.at[i])
                    for i, (src, dst) in enumerate(((x_hbm, xin), (q_hbm, qin)))]

        def pre_copies():
            return [pltpu.make_async_copy(x_hbm.at[pl.ds(i * seg, pre_rows), :],
                                          xpre.at[pl.ds(i * pre_rows, pre_rows), :], sem_p) for i in range(n_pre + 1)]

        def chunk_copies(c):
            r0 = seg + c * x_rows if isinstance(c, int) else pl.multiple_of(seg + c * x_rows, seg)
            return [pltpu.make_async_copy(src.at[pl.ds(r0, x_rows), :], dst.at[pl.ds(r0, x_rows), :], sem.at[c])
                    for src, dst, sem in ((x_hbm, xin, sem_x), (q_hbm, qin, sem_q))]

        def out_copy(s):
            r0 = s * seg if isinstance(s, int) else pl.multiple_of(s * seg, seg)
            return pltpu.make_async_copy(ost.at[s], out_hbm.at[pl.ds(r0, seg), :], sem_out)

        tc = t_copies()
        for c in tc[:3] + kv_copies(0) + [h_copy(0)] + tc[3:]:
            c.start()
        for cb in range(1, n_early):
            for c in [h_copy(cb)] + kv_copies(cb):
                c.start()
        late = kv_copies(n_early) + [h_copy(cb) for cb in range(n_early, n_cb)]
        n_b_late = len(late)
        late += w_copies(0) + pre_copies() + w_copies(1) + w_copies(2) + head_copies()
        for i in range(len(wo_bounds) - 1):
            late += o_copies(i)
        per_block = _CFG["late_per_block"]
        first_block = _CFG["late_first"]

        kf[0:8, :] = jnp.zeros((8, CB), F32)

        group = _CFG["b_group"]

        def put(ref, row, x):
            ref[pl.ds(2 * row, x.shape[0]), :] = x.astype(BF16)

        def get(ref, row, n, stride=1):
            return ref.bitcast(U32)[pl.ds(row, n, stride=stride), :]

        def wait_inputs(cb):
            h_copy(cb).wait()

            @pl.when(cb < n_early)
            def _():
                for c in kv_copies(cb):
                    c.wait()

            @pl.when(cb == n_early)
            def _():
                for c in kv_copies(n_early):
                    c.wait()

        def prepare(cb):
            c0 = pl.multiple_of(cb * CB, CB)
            kf[8:8 + SEQ, :] = ks[:, pl.ds(c0, CB)].astype(F32)
            for j in range(SEQ // 128):
                r = hs[cb, :, j * 128:(j + 1) * 128].astype(F32).T
                put(hp, (2 * j) * SP, r[0:N2])
                put(hp, (2 * j + 1) * SP, r[N2:2 * N2])
            taps = sh32[:, pl.ds(c0, CB)]
            for n1 in range(N1):
                acc = kf[pl.ds(8 + n1 * N2, N2), :] * taps[0:1]
                for i in range(1, 4):
                    acc = acc + kf[pl.ds(8 - i + n1 * N2, N2), :] * taps[i:i + 1]
                put(xp, n1 * SP, acc * vs[pl.ds(n1 * N2, N2), pl.ds(c0, CB)].astype(F32))

        def b_block(cb, carry):
            wait_inputs(cb)
            for i in range(n_cb - first_block):
                @pl.when(cb == i + first_block)
                def _(i=i):
                    lo = 0 if i == 0 else n_b_late + i * per_block
                    for c in late[lo:n_b_late + (i + 1) * per_block]:
                        c.start()
            lane = jax.lax.broadcasted_iota(jnp.int32, (1, 128), 1)
            prepare(cb)
            for g in range(N2 // 4):
                m = tf[g]
                lhs = _from_words(jnp.concatenate(
                    [jnp.where((lane // 64 == j // 2) & (lane % 2 == j % 2), m, jnp.zeros_like(m))
                     for j in range(4)], axis=0))

                def rhs(ref, g=g):
                    return _from_words(jnp.concatenate(
                        [get(ref, 2 * g, N1, SP), get(ref, 2 * g + 1, N1, SP)], axis=0))

                r = _dot(lhs, jnp.concatenate([rhs(xp), rhs(hp)], axis=1))
                for j in range(4):
                    put(zx, (4 * g + j) * SZ, r[2 * N1 * j:2 * N1 * (j + 1), :128])
                    put(zh, (4 * g + j) * SZ, r[2 * N1 * j:2 * N1 * (j + 1), 128:])
            f2 = _from_words(t2[0])
            g2 = _from_words(t2[1])

            def stage2(g):
                zz = []
                for k1 in range(g * group, (g + 1) * group):
                    zz += [_from_words(get(zx, k1, N2, SZ)), _from_words(get(zh, k1, N2, SZ))]
                return _dot(f2, jnp.concatenate(zz, axis=1))

            def stage3(g, r):
                ys = []
                for i in range(group):
                    xf = r[:, (2 * i) * 128:(2 * i + 1) * 128]
                    hf = r[:, (2 * i + 1) * 128:(2 * i + 2) * 128]
                    xr, xi, hr, hi = xf[:N2], xf[N2:], hf[:N2], hf[N2:]
                    ys.append(jnp.concatenate([xr * hr - xi * hi, xr * hi + xi * hr], axis=0).astype(BF16))
                t = _dot(g2, jnp.concatenate(ys, axis=1))
                for i in range(group):
                    put(tt, (g * group + i) * ST, t[:, i * 128:(i + 1) * 128])

            n_groups = N1 // group
            r = stage2(0)
            for g in range(n_groups):
                r_next = stage2(g + 1) if g + 1 < n_groups else None
                stage3(g, r)
                r = r_next
            half_mask = jnp.where(lane < 64, U32(0x0000FFFF), U32(0xFFFF0000))
            dv = d32[pl.ds(cb, 1), :]
            for i in range(N2 // 2):
                y = _dot(_from_words(ti[i] & half_mask), _from_words(jnp.concatenate(
                    [get(tt, 2 * i, N1, ST), get(tt, 2 * i + 1, N1, ST)], axis=0)))
                kv = _from_words(get(xp, i, N1, SP)).astype(F32)
                ob[cb, pl.ds(i, N1, stride=SP), :] = _to_words(y + kv * dv)
            return carry

        for c in tc:
            c.wait()
        sh32[...] = sh_ref[...].astype(F32)
        d32[...] = d_ref[...].astype(F32)
        hbuf[0:n_mem, :] = mem_ref[...].astype(F32)
        jax.lax.fori_loop(0, n_cb, b_block, 0)
        for c in late[n_b_late + (n_cb - first_block) * per_block:]:
            c.start()

        def w_slot(quad, parity, odd_head, m):
            return (w_even, w_odd)[parity], (2 * quad + odd_head) * 3 + m

        def wtile(h, m):
            ref, i = w_slot(h // 4, (h // 2) % 2, h % 2, m)
            return _from_words(ref[i])

        def relayout(m, quad, parity):
            pair = 2 * quad + parity
            if not isinstance(pair, int):
                pair = jnp.minimum(pair, n_hp - 1)
            src = m * n_hp + pair
            even = stage[src, pl.ds(0, d_model // 2, stride=2), :]
            odd = stage[src, pl.ds(1, d_model // 2, stride=2), :]
            ref, i = w_slot(quad, parity, 0, m)
            ref[i] = (even & U32(0xFFFF)) | (odd << 16)
            ref, i = w_slot(quad, parity, 1, m)
            ref[i] = (even >> 16) | (odd & U32(0xFFFF0000))

        for m in range(2):
            for c in w_copies(m):
                c.wait()
        for c in pre_copies():
            c.wait()
        xpre32[...] = xpre[...].astype(F32)
        relayout(0, 0, 0)
        relayout(1, 0, 0)

        def pre_dots(quad, parity, xl):
            for odd_head in range(2):
                for m in range(2):
                    ref, i = w_slot(quad, parity, odd_head, m)
                    qkpre[m, 4 * quad + 2 * parity + odd_head] = _dot(xl, _from_words(ref[i]))

        def pre_round(quad, carry):
            xl = xpre32[...]
            pre_dots(quad, 0, xl)
            relayout(0, quad, 1)
            relayout(1, quad, 1)
            pre_dots(quad, 1, xl)
            relayout(0, quad + 1, 0)
            relayout(1, quad + 1, 0)
            return carry

        jax.lax.fori_loop(0, n_heads // 4, pre_round, 0)
        for c in w_copies(2):
            c.wait()

        def step(s, first, pre=False):
            if first:
                for c in head_copies():
                    c.wait()
            row = jax.lax.broadcasted_iota(jnp.int32, (n_rows, n_rows), 0)
            col = jax.lax.broadcasted_iota(jnp.int32, (n_rows, n_rows), 1)
            mask = (row < n_mem) | (row >= col)
            r0 = s * seg if first else pl.multiple_of(s * seg, seg)
            slot = s
            y0 = (s * seg // N2) * SP + (s * seg % N2) // 2
            if not first:
                y0 = pl.multiple_of(y0, 4)
            hbuf[n_mem:n_rows, :] = xin[pl.ds(r0, seg), :].astype(F32)
            hl = hbuf[...]
            if pre:
                hr = jnp.concatenate([hl[0:n_mem], hl[n_mem + pre_rows:n_rows]], axis=0)
                p0 = s * pre_rows if first else pl.multiple_of(s * pre_rows, pre_rows)
            waited = [False] * (len(wo_bounds) - 1)
            for op in (order_first if first else order):
                if op[0] == "P":
                    h = op[1]
                    if first and h % 2 == 0:
                        if h == 0:
                            relayout(2, 0, 0)
                        if h + 2 < n_heads:
                            relayout(2, (h + 2) // 4, (h // 2 + 1) % 2)
                    if pre:
                        rq = _dot(hr, wtile(h, 0))
                        qbuf[h] = jnp.concatenate(
                            [rq[0:n_mem], qkpre[0, h, pl.ds(p0, pre_rows), :], rq[n_mem:]], axis=0)
                        rk = _dot(hr, wtile(h, 1))
                        kbuf[h, 0:n_rows] = jnp.concatenate(
                            [rk[0:n_mem], qkpre[1, h, pl.ds(p0, pre_rows), :], rk[n_mem:]], axis=0).astype(BF16)
                    else:
                        qbuf[h] = _dot(hl, wtile(h, 0))
                        kbuf[h, 0:n_rows] = _dot(hl, wtile(h, 1)).astype(BF16)
                    vbuf[h, 0:n_rows] = _dot(hl, wtile(h, 2)).astype(BF16)
                elif op[0] == "S":
                    h = op[1]
                    sc = _dot_nt(qbuf[h], kbuf[h, 0:n_rows])
                    sc = jnp.where(mask, sc, -1e9 / scale)
                    e = jnp.exp2((sc - jnp.max(sc, axis=-1, keepdims=True)) * exp_scale)
                    den = jnp.sum(e, axis=-1, keepdims=True)
                    inv = pl.reciprocal(den, approx=True)
                    pbuf[h, :, 0:n_rows] = e
                    ibuf[h] = jnp.broadcast_to(inv * (2.0 - den * inv), (n_rows, d_head))
                elif op[0] == "V":
                    h = op[1]
                    obuf[:, h * d_head:(h + 1) * d_head] = (
                        _dot(pbuf[h, :, 0:n_rows], vbuf[h, 0:n_rows]) * ibuf[h])
                elif op[0] == "W":
                    _, j, lo, hi = op
                    if first:
                        for i in range(len(waited)):
                            if not waited[i] and hi > wo_bounds[i]:
                                for c in o_copies(i):
                                    c.wait()
                                waited[i] = True
                                if i == len(waited) - 1:
                                    for ch in range(x_chunks):
                                        for c in chunk_copies(ch):
                                            c.start()
                    w = _from_words(wo[j, lo * d_head // 2:hi * d_head // 2, :])
                    y = _dot(obuf[:, lo * d_head:hi * d_head], w)
                    if lo > 0:
                        y = y + ybuf[j]
                    if hi < n_heads:
                        ybuf[j] = y
                    else:
                        hbuf[0:n_mem, j * 128:(j + 1) * 128] = y[0:n_mem]
                        ost[slot, :, j * 128:(j + 1) * 128] = y[n_mem:n_rows].astype(BF16)
                else:
                    for cb in range(n_cb):
                        gate = qin[pl.ds(r0, seg), cb * CB:(cb + 1) * CB].astype(F32)
                        ost[slot, :, d_model + cb * CB:d_model + (cb + 1) * CB] = (
                            _from_words(ob[cb, pl.ds(y0, seg // 2), :]).astype(F32) * gate).astype(BF16)
            out_copy(s).start()

        unroll = _CFG["unroll"]

        def chunk_body(c, carry, pre=False):
            for cp in chunk_copies(c):
                cp.wait()

            def steps_body(i, carry):
                for u in range(unroll):
                    step(1 + c * steps_per_chunk + i * unroll + u, False, pre)
                return carry

            if steps_per_chunk == unroll:
                steps_body(0, 0)
            else:
                jax.lax.fori_loop(0, steps_per_chunk // unroll, steps_body, 0)
            return carry

        step(0, True, True)
        def pre_step(s, carry):
            @pl.when((s - 1) % steps_per_chunk == 0)
            def _():
                for cp in chunk_copies((s - 1) // steps_per_chunk):
                    cp.wait()

            step(s, False, True)
            return carry

        pre_chunks = n_pre // steps_per_chunk
        if pre_chunks and _CFG["pre_rolled"]:
            jax.lax.fori_loop(1, 1 + n_pre, pre_step, 0)
        elif pre_chunks:
            jax.lax.fori_loop(0, pre_chunks, functools.partial(chunk_body, pre=True), 0)
        jax.lax.fori_loop(pre_chunks, x_chunks, chunk_body, 0)
        for s in range(n_seg):
            out_copy(s).wait()

    return kernel


def _forward(x, mem0, wq, wk, wv, wo, seg_len, q, k, v, shift_k, ssm_k, ssm_d):
    _, seq, d_model = x.shape
    _, n_heads, d_head = wq.shape
    n_mem = mem0.shape[1]
    seg = seg_len
    n_seg = seq // seg
    n_rows = n_mem + seg
    n_cb = d_model // CB
    assert seq == SEQ and d_model == 1024 and d_head == 128 and n_rows % 8 == 0
    tf, ti, t2 = _dft_tables()

    any_spec = pl.BlockSpec(memory_space=pl.ANY)
    kv_rows = -(-n_rows // 16) * 16
    scratch = [
        pltpu.VMEM((n_cb, CB, seq), BF16),
        pltpu.VMEM((seq, d_model), BF16),
        pltpu.VMEM((seq, d_model), BF16),
        pltpu.VMEM((n_cb, N1 * SP, CB), U32),
        pltpu.VMEM((8 + seq, CB), F32),
        pltpu.VMEM((2 * N1 * SP, CB), BF16),
        pltpu.VMEM((2 * N1 * SP, CB), BF16),
        pltpu.VMEM((2 * N2 * SZ, CB), BF16),
        pltpu.VMEM((2 * N2 * SZ, CB), BF16),
        pltpu.VMEM((2 * N1 * ST, CB), BF16),
        pltpu.VMEM(tf.shape, U32),
        pltpu.VMEM(ti.shape, U32),
        pltpu.VMEM(t2.shape, U32),
        pltpu.VMEM((4, d_model), BF16),
        pltpu.VMEM((n_cb, CB), BF16),
        pltpu.VMEM((n_mem, d_model), BF16),
        pltpu.VMEM((4, d_model), F32),
        pltpu.VMEM((n_cb, CB), F32),
        pltpu.VMEM((3 * n_heads // 2, d_model, d_head), U32),
        pltpu.VMEM((3 * n_heads // 2 + 6, d_model // 2, d_head), U32),
        pltpu.VMEM((3 * n_heads // 2, d_model // 2, d_head), U32),
        pltpu.VMEM((d_model // 128, n_heads * d_head // 2, 128), U32),
        pltpu.VMEM((seq, d_model), BF16),
        pltpu.VMEM((seq, d_model), BF16),
        pltpu.VMEM((n_seg, seg, 2 * d_model), BF16),
        pltpu.VMEM((n_rows, d_model), F32),
        pltpu.VMEM((n_heads, n_rows, d_head), F32),
        pltpu.VMEM((n_heads, kv_rows, d_head), BF16),
        pltpu.VMEM((n_heads, kv_rows, d_head), BF16),
        pltpu.VMEM((n_rows, n_heads * d_head), F32),
        pltpu.VMEM((n_heads, n_rows, d_head), F32),
        pltpu.VMEM((n_heads, n_rows, d_head), F32),
        pltpu.VMEM((d_model // 128, n_rows, 128), F32),
        pltpu.VMEM(((_CFG["n_pre"] + 1) * 8, d_model), BF16),
        pltpu.VMEM(((_CFG["n_pre"] + 1) * 8, d_model), F32),
        pltpu.VMEM((2, n_heads, (_CFG["n_pre"] + 1) * 8, d_head), F32),
        pltpu.SemaphoreType.DMA((3, n_cb)),
        pltpu.SemaphoreType.DMA((6,)),
        pltpu.SemaphoreType.DMA((3,)),
        pltpu.SemaphoreType.DMA((len(_CFG["first_splits"]) + 1,)),
        pltpu.SemaphoreType.DMA((2,)),
        pltpu.SemaphoreType.DMA(()),
        pltpu.SemaphoreType.DMA((n_seg,)),
        pltpu.SemaphoreType.DMA((n_seg,)),
        pltpu.SemaphoreType.DMA(()),
    ]
    out = pl.pallas_call(
        _make_kernel(n_heads, d_head, d_model, n_mem, seg, n_seg),
        out_shape=jax.ShapeDtypeStruct((seq, 2 * d_model), BF16),
        in_specs=[any_spec] * 15,
        out_specs=any_spec,
        scratch_shapes=scratch,
        compiler_params=pltpu.CompilerParams(vmem_limit_bytes=120 * 1024 * 1024),
    )(shift_k.T, ssm_d.reshape(n_cb, CB), mem0.reshape(n_mem, d_model),
      x.reshape(seq, d_model), wq, wk, wv, wo.reshape(n_heads * d_head, d_model),
      q.reshape(seq, d_model), k.reshape(seq, d_model), v.reshape(seq, d_model), ssm_k,
      tf, ti, t2)
    return out.reshape(1, seq, 2 * d_model)


def pallas_concat_heads__memory_aug_recurrent_mem_tr__ssm_conv_h3__prompt_kernel(
        A_x, A_mem0, A_Wq, A_Wk, A_Wv, A_Wo, A_seg_len, B_q, B_k, B_v, B_shift_k, B_ssm_k, B_ssm_D):
    return _forward(A_x, A_mem0, A_Wq, A_Wk, A_Wv, A_Wo, int(A_seg_len), B_q, B_k, B_v,
                    B_shift_k, B_ssm_k, B_ssm_D)
```

```python
import math

import jax
import jax.numpy as jnp
import numpy as np
from jax.experimental import pallas as pl
from jax.experimental.pallas import tpu as pltpu

F32 = jnp.float32
BF16 = jnp.bfloat16
U32 = jnp.uint32

N1, N2 = 32, 64
SEQ = N1 * N2
SP = N2 // 2 + 4
SZ = N1 + 4
ST = N2 + 4
CB = 128


def _dft_tables():
    theta = np.pi / (2 * SEQ)
    lane = np.arange(128)[None, :]
    hi, mid, lo = lane // 64, (lane % 64) // 2, lane % 2
    k1 = np.arange(N1)[:, None]
    fwd = np.zeros((N2 // 4, 2 * N1, 128))
    for g in range(N2 // 4):
        ph = theta * (4 * k1 + 1) * (N2 * mid + 4 * g + 2 * hi + lo)
        fwd[g, 0::2] = np.cos(ph)
        fwd[g, 1::2] = np.sin(ph)
    n1 = np.arange(N1)[:, None]
    inv = np.zeros((N2 // 2, N1, 128))
    for i in range(N2 // 2):
        ph = theta * (4 * mid + 1) * (N2 * n1 + 2 * i + hi)
        inv[i] = np.where(lo == 0, np.cos(ph), np.sin(ph)) / SEQ
    ph = 2 * np.pi * np.arange(N2)[:, None] * np.arange(N2)[None, :] / N2
    c, s = np.cos(ph), np.sin(ph)
    f2 = np.zeros((128, 128))
    f2[:N2, 0::2], f2[:N2, 1::2], f2[N2:, 0::2], f2[N2:, 1::2] = c, -s, s, c
    g2 = np.zeros((128, 128))
    g2[0::2, :N2], g2[0::2, N2:], g2[1::2, :N2], g2[1::2, N2:] = c.T, s.T, -s.T, c.T

    def as_words(a):
        u = a.astype(np.float32).astype(BF16).view(np.uint16).astype(np.uint32)
        return u[..., 0::2, :] | (u[..., 1::2, :] << 16)

    inv = np.repeat(inv, 2, axis=1)
    return as_words(fwd), as_words(inv), as_words(np.stack([f2, g2]))


def _to_words(x):
    return pltpu.bitcast(x.astype(BF16), U32)


def _from_words(w):
    return pltpu.bitcast(w, BF16)


_CFG = dict(
    group=8, lag_s=2, lag_v=3, wo_split=16, gate_at=1,
    first_splits=(16,),
    unroll=3,
    chunk_steps=3,
    n_pre=18,
    n_early=2,
    late_per_block=10,
    b_group=8,
)


def _step_order(n_heads, n_out_tiles, first=False):
    g, a, b = _CFG["group"], _CFG["lag_s"], _CFG["lag_v"]
    split = _CFG["wo_split"]
    n_groups = n_heads // g
    total = n_groups + a + b
    early = [("W", j, 0, split) for j in range(n_out_tiles)] if split < n_heads else []
    ops = []
    for t in range(total):
        if t < n_groups:
            ops += [("P", h) for h in range(t * g, (t + 1) * g)]
        if t == _CFG["gate_at"]:
            ops.append(("G",))
        if 0 <= t - a < n_groups:
            ops += [("S", h) for h in range((t - a) * g, (t - a + 1) * g)]
        if 0 <= t - a - b < n_groups:
            ops += [("V", h) for h in range((t - a - b) * g, (t - a - b + 1) * g)]
        if early and (t - a - b + 1) * g >= split:
            n = -(-len(early) // (total - t))
            ops += early[:n]
            early = early[n:]
    ops += early
    bounds = [split if split < n_heads else 0]
    if first:
        bounds += [b for b in _CFG["first_splits"] if b > split]
    for lo, hi in zip(bounds, bounds[1:] + [n_heads]):
        ops += [("W", j, lo, hi) for j in range(n_out_tiles)]
    return ops


def _dot(a, b):
    return jnp.dot(a, b, preferred_element_type=F32)


def _dot_nt(a, b):
    return jax.lax.dot_general(a, b, (((1,), (1,)), ((), ())), preferred_element_type=F32)


def _make_kernel(n_heads, d_head, d_model, n_mem, seg, n_seg):
    n_rows = n_mem + seg
    n_cb = d_model // CB
    n_hp = n_heads // 2
    scale = d_head ** (-0.5)
    exp_scale = scale * math.log2(math.e)
    steps_per_chunk = _CFG["chunk_steps"]
    x_chunks = (n_seg - 1) // steps_per_chunk
    x_rows = steps_per_chunk * seg
    assert x_chunks * steps_per_chunk == n_seg - 1 and steps_per_chunk % _CFG["unroll"] == 0
    n_pre = _CFG["n_pre"]
    pre_rows = 8
    assert n_pre % steps_per_chunk == 0
    order = _step_order(n_heads, d_model // 128)
    order_first = _step_order(n_heads, d_model // 128, True)
    wo_bounds = [0] + list(_CFG["first_splits"]) + [n_heads]

    def kernel(sh_hbm, d_hbm, mem_hbm,
               x_hbm, wq_hbm, wk_hbm, wv_hbm, wo_hbm,
               q_hbm, k_hbm, v_hbm, h_hbm, tf_hbm, ti_hbm, t2_hbm,
               out_hbm,
               hs, ks, vs, ob, kf, xp, hp, zx, zh, tt, tf, ti, t2, sh_ref, d_ref, mem_ref, sh32, d32,
               stage, w_even, w_odd, wo, xin, qin, ost, hbuf, qbuf, kbuf, vbuf, obuf, pbuf, ibuf, ybuf, xpre, xpre32, qkpre,
               sem_b, sem_t, sem_w, sem_o, sem_h, sem_p, sem_x, sem_q, sem_out):

        n_early = _CFG["n_early"]

        def h_copy(cb):
            c0 = cb * CB if isinstance(cb, int) else pl.multiple_of(cb * CB, CB)
            return pltpu.make_async_copy(h_hbm.at[pl.ds(c0, CB), :], hs.at[cb], sem_b.at[0, cb])

        def kv_copies(cb):
            if isinstance(cb, int):
                c0, width = cb * CB, (CB if cb < n_early else d_model - n_early * CB)
            else:
                c0, width = pl.multiple_of(cb * CB, CB), CB
            return [pltpu.make_async_copy(src.at[:, pl.ds(c0, width)], dst.at[:, pl.ds(c0, width)], sem_b.at[1 + i, cb])
                    for i, (src, dst) in enumerate(((k_hbm, ks), (v_hbm, vs)))]

        def t_copies():
            pairs = ((sh_hbm, sh_ref), (d_hbm, d_ref), (mem_hbm, mem_ref),
                     (tf_hbm, tf), (ti_hbm, ti), (t2_hbm, t2))
            return [pltpu.make_async_copy(src, dst, sem_t.at[i]) for i, (src, dst) in enumerate(pairs)]

        def w_copies(m):
            w32 = (wq_hbm, wk_hbm, wv_hbm)[m].bitcast(U32)
            return [pltpu.make_async_copy(w32.at[:, hp, :], stage.at[m * n_hp + hp], sem_w.at[m])
                    for hp in range(n_hp)]

        def o_copies(i):
            wo32 = wo_hbm.bitcast(U32)
            lo, hi = wo_bounds[i] * d_head // 2, wo_bounds[i + 1] * d_head // 2
            return [pltpu.make_async_copy(wo32.at[pl.ds(lo, hi - lo), pl.ds(j * 128, 128)],
                                          wo.at[j, pl.ds(lo, hi - lo), :], sem_o.at[i])
                    for j in range(d_model // 128)]

        def head_copies():
            return [pltpu.make_async_copy(src.at[pl.ds(0, seg), :], dst.at[pl.ds(0, seg), :], sem_h.at[i])
                    for i, (src, dst) in enumerate(((x_hbm, xin), (q_hbm, qin)))]

        def pre_copies():
            return [pltpu.make_async_copy(x_hbm.at[pl.ds(i * seg, pre_rows), :],
                                          xpre.at[pl.ds(i * pre_rows, pre_rows), :], sem_p) for i in range(n_pre + 1)]

        def chunk_copies(c):
            r0 = seg + c * x_rows if isinstance(c, int) else pl.multiple_of(seg + c * x_rows, seg)
            return [pltpu.make_async_copy(src.at[pl.ds(r0, x_rows), :], dst.at[pl.ds(r0, x_rows), :], sem.at[c])
                    for src, dst, sem in ((x_hbm, xin, sem_x), (q_hbm, qin, sem_q))]

        def out_copy(s):
            r0 = s * seg if isinstance(s, int) else pl.multiple_of(s * seg, seg)
            return pltpu.make_async_copy(ost.at[s], out_hbm.at[pl.ds(r0, seg), :], sem_out)

        tc = t_copies()
        for c in tc[:3] + kv_copies(0) + [h_copy(0)] + tc[3:]:
            c.start()
        for cb in range(1, n_early):
            for c in [h_copy(cb)] + kv_copies(cb):
                c.start()
        late = kv_copies(n_early) + [h_copy(cb) for cb in range(n_early, n_cb)]
        n_b_late = len(late)
        late += w_copies(0) + pre_copies() + w_copies(1) + w_copies(2) + head_copies()
        for i in range(len(wo_bounds) - 1):
            late += o_copies(i)
        per_block = _CFG["late_per_block"]

        kf[0:8, :] = jnp.zeros((8, CB), F32)

        group = _CFG["b_group"]

        def put(ref, row, x):
            ref[pl.ds(2 * row, x.shape[0]), :] = x.astype(BF16)

        def get(ref, row, n, stride=1):
            return ref.bitcast(U32)[pl.ds(row, n, stride=stride), :]

        def wait_inputs(cb):
            h_copy(cb).wait()

            @pl.when(cb < n_early)
            def _():
                for c in kv_copies(cb):
                    c.wait()

            @pl.when(cb == n_early)
            def _():
                for c in kv_copies(n_early):
                    c.wait()

        def prepare(cb):
            c0 = pl.multiple_of(cb * CB, CB)
            kf[8:8 + SEQ, :] = ks[:, pl.ds(c0, CB)].astype(F32)
            for j in range(SEQ // 128):
                r = hs[cb, :, j * 128:(j + 1) * 128].astype(F32).T
                put(hp, (2 * j) * SP, r[0:N2])
                put(hp, (2 * j + 1) * SP, r[N2:2 * N2])
            taps = sh32[:, pl.ds(c0, CB)]
            for n1 in range(N1):
                acc = kf[pl.ds(8 + n1 * N2, N2), :] * taps[0:1]
                for i in range(1, 4):
                    acc = acc + kf[pl.ds(8 - i + n1 * N2, N2), :] * taps[i:i + 1]
                put(xp, n1 * SP, acc * vs[pl.ds(n1 * N2, N2), pl.ds(c0, CB)].astype(F32))

        def b_block(cb, carry):
            wait_inputs(cb)
            for i in range(n_cb):
                @pl.when(cb == i)
                def _(i=i):
                    lo = 0 if i == 0 else n_b_late + i * per_block
                    for c in late[lo:n_b_late + (i + 1) * per_block]:
                        c.start()
            lane = jax.lax.broadcasted_iota(jnp.int32, (1, 128), 1)
            prepare(cb)
            for g in range(N2 // 4):
                m = tf[g]
                lhs = _from_words(jnp.concatenate(
                    [jnp.where((lane // 64 == j // 2) & (lane % 2 == j % 2), m, jnp.zeros_like(m))
                     for j in range(4)], axis=0))

                def rhs(ref, g=g):
                    return _from_words(jnp.concatenate(
                        [get(ref, 2 * g, N1, SP), get(ref, 2 * g + 1, N1, SP)], axis=0))

                r = _dot(lhs, jnp.concatenate([rhs(xp), rhs(hp)], axis=1))
                for j in range(4):
                    put(zx, (4 * g + j) * SZ, r[2 * N1 * j:2 * N1 * (j + 1), :128])
                    put(zh, (4 * g + j) * SZ, r[2 * N1 * j:2 * N1 * (j + 1), 128:])
            f2 = _from_words(t2[0])
            g2 = _from_words(t2[1])

            def stage2(g):
                zz = []
                for k1 in range(g * group, (g + 1) * group):
                    zz += [_from_words(get(zx, k1, N2, SZ)), _from_words(get(zh, k1, N2, SZ))]
                return _dot(f2, jnp.concatenate(zz, axis=1))

            def stage3(g, r):
                ys = []
                for i in range(group):
                    xf = r[:, (2 * i) * 128:(2 * i + 1) * 128]
                    hf = r[:, (2 * i + 1) * 128:(2 * i + 2) * 128]
                    xr, xi, hr, hi = xf[:N2], xf[N2:], hf[:N2], hf[N2:]
                    ys.append(jnp.concatenate([xr * hr - xi * hi, xr * hi + xi * hr], axis=0).astype(BF16))
                t = _dot(g2, jnp.concatenate(ys, axis=1))
                for i in range(group):
                    put(tt, (g * group + i) * ST, t[:, i * 128:(i + 1) * 128])

            n_groups = N1 // group
            r = stage2(0)
            for g in range(n_groups):
                r_next = stage2(g + 1) if g + 1 < n_groups else None
                stage3(g, r)
                r = r_next
            half_mask = jnp.where(lane < 64, U32(0x0000FFFF), U32(0xFFFF0000))
            dv = d32[pl.ds(cb, 1), :]
            for i in range(N2 // 2):
                y = _dot(_from_words(ti[i] & half_mask), _from_words(jnp.concatenate(
                    [get(tt, 2 * i, N1, ST), get(tt, 2 * i + 1, N1, ST)], axis=0)))
                kv = _from_words(get(xp, i, N1, SP)).astype(F32)
                ob[cb, pl.ds(i, N1, stride=SP), :] = _to_words(y + kv * dv)
            return carry

        for c in tc:
            c.wait()
        sh32[...] = sh_ref[...].astype(F32)
        d32[...] = d_ref[...].astype(F32)
        hbuf[0:n_mem, :] = mem_ref[...].astype(F32)
        jax.lax.fori_loop(0, n_cb, b_block, 0)
        for c in late[n_b_late + n_cb * per_block:]:
            c.start()

        def w_slot(quad, parity, odd_head, m):
            return (w_even, w_odd)[parity], (2 * quad + odd_head) * 3 + m

        def wtile(h, m):
            ref, i = w_slot(h // 4, (h // 2) % 2, h % 2, m)
            return _from_words(ref[i])

        def relayout(m, quad, parity):
            pair = 2 * quad + parity
            if not isinstance(pair, int):
                pair = jnp.minimum(pair, n_hp - 1)
            src = m * n_hp + pair
            even = stage[src, pl.ds(0, d_model // 2, stride=2), :]
            odd = stage[src, pl.ds(1, d_model // 2, stride=2), :]
            ref, i = w_slot(quad, parity, 0, m)
            ref[i] = (even & U32(0xFFFF)) | (odd << 16)
            ref, i = w_slot(quad, parity, 1, m)
            ref[i] = (even >> 16) | (odd & U32(0xFFFF0000))

        for m in range(2):
            for c in w_copies(m):
                c.wait()
        for c in pre_copies():
            c.wait()
        xpre32[...] = xpre[...].astype(F32)
        relayout(0, 0, 0)
        relayout(1, 0, 0)

        def pre_dots(quad, parity, xl):
            for odd_head in range(2):
                for m in range(2):
                    ref, i = w_slot(quad, parity, odd_head, m)
                    qkpre[m, 4 * quad + 2 * parity + odd_head] = _dot(xl, _from_words(ref[i]))

        def pre_round(quad, carry):
            xl = xpre32[...]
            pre_dots(quad, 0, xl)
            relayout(0, quad, 1)
            relayout(1, quad, 1)
            pre_dots(quad, 1, xl)
            relayout(0, quad + 1, 0)
            relayout(1, quad + 1, 0)
            return carry

        jax.lax.fori_loop(0, n_heads // 4, pre_round, 0)
        for c in w_copies(2):
            c.wait()

        def step(s, first, pre=False):
            if first:
                for c in head_copies():
                    c.wait()
            row = jax.lax.broadcasted_iota(jnp.int32, (n_rows, n_rows), 0)
            col = jax.lax.broadcasted_iota(jnp.int32, (n_rows, n_rows), 1)
            mask = (row < n_mem) | (row >= col)
            r0 = s * seg if first else pl.multiple_of(s * seg, seg)
            slot = s
            y0 = (s * seg // N2) * SP + (s * seg % N2) // 2
            if not first:
                y0 = pl.multiple_of(y0, 4)
            hbuf[n_mem:n_rows, :] = xin[pl.ds(r0, seg), :].astype(F32)
            hl = hbuf[...]
            if pre:
                hr = jnp.concatenate([hl[0:n_mem], hl[n_mem + pre_rows:n_rows]], axis=0)
                p0 = s * pre_rows if first else pl.multiple_of(s * pre_rows, pre_rows)
            waited = [False] * (len(wo_bounds) - 1)
            for op in (order_first if first else order):
                if op[0] == "P":
                    h = op[1]
                    if first and h % 2 == 0:
                        if h == 0:
                            relayout(2, 0, 0)
                        if h + 2 < n_heads:
                            relayout(2, (h + 2) // 4, (h // 2 + 1) % 2)
                    if pre:
                        rq = _dot(hr, wtile(h, 0))
                        qbuf[h] = jnp.concatenate(
                            [rq[0:n_mem], qkpre[0, h, pl.ds(p0, pre_rows), :], rq[n_mem:]], axis=0)
                        rk = _dot(hr, wtile(h, 1))
                        kbuf[h, 0:n_rows] = jnp.concatenate(
                            [rk[0:n_mem], qkpre[1, h, pl.ds(p0, pre_rows), :], rk[n_mem:]], axis=0).astype(BF16)
                    else:
                        qbuf[h] = _dot(hl, wtile(h, 0))
                        kbuf[h, 0:n_rows] = _dot(hl, wtile(h, 1)).astype(BF16)
                    vbuf[h, 0:n_rows] = _dot(hl, wtile(h, 2)).astype(BF16)
                elif op[0] == "S":
                    h = op[1]
                    sc = _dot_nt(qbuf[h], kbuf[h, 0:n_rows])
                    sc = jnp.where(mask, sc, -1e9 / scale)
                    e = jnp.exp2((sc - jnp.max(sc, axis=-1, keepdims=True)) * exp_scale)
                    den = jnp.sum(e, axis=-1, keepdims=True)
                    inv = pl.reciprocal(den, approx=True)
                    pbuf[h, :, 0:n_rows] = e
                    ibuf[h] = jnp.broadcast_to(inv * (2.0 - den * inv), (n_rows, d_head))
                elif op[0] == "V":
                    h = op[1]
                    obuf[:, h * d_head:(h + 1) * d_head] = (
                        _dot(pbuf[h, :, 0:n_rows], vbuf[h, 0:n_rows]) * ibuf[h])
                elif op[0] == "W":
                    _, j, lo, hi = op
                    if first:
                        for i in range(len(waited)):
                            if not waited[i] and hi > wo_bounds[i]:
                                for c in o_copies(i):
                                    c.wait()
                                waited[i] = True
                                if i == len(waited) - 1:
                                    for ch in range(x_chunks):
                                        for c in chunk_copies(ch):
                                            c.start()
                    w = _from_words(wo[j, lo * d_head // 2:hi * d_head // 2, :])
                    y = _dot(obuf[:, lo * d_head:hi * d_head], w)
                    if lo > 0:
                        y = y + ybuf[j]
                    if hi < n_heads:
                        ybuf[j] = y
                    else:
                        hbuf[0:n_mem, j * 128:(j + 1) * 128] = y[0:n_mem]
                        ost[slot, :, j * 128:(j + 1) * 128] = y[n_mem:n_rows].astype(BF16)
                else:
                    for cb in range(n_cb):
                        gate = qin[pl.ds(r0, seg), cb * CB:(cb + 1) * CB].astype(F32)
                        ost[slot, :, d_model + cb * CB:d_model + (cb + 1) * CB] = (
                            _from_words(ob[cb, pl.ds(y0, seg // 2), :]).astype(F32) * gate).astype(BF16)
            out_copy(s).start()

        unroll = _CFG["unroll"]

        def pre_step(s, carry):
            @pl.when((s - 1) % steps_per_chunk == 0)
            def _():
                for cp in chunk_copies((s - 1) // steps_per_chunk):
                    cp.wait()

            step(s, False, True)
            return carry

        def chunk_body(c, carry):
            for cp in chunk_copies(c):
                cp.wait()

            def steps_body(i, carry):
                for u in range(unroll):
                    step(1 + c * steps_per_chunk + i * unroll + u, False)
                return carry

            if steps_per_chunk == unroll:
                steps_body(0, 0)
            else:
                jax.lax.fori_loop(0, steps_per_chunk // unroll, steps_body, 0)
            return carry

        step(0, True, True)
        jax.lax.fori_loop(1, 1 + n_pre, pre_step, 0)
        jax.lax.fori_loop(n_pre // steps_per_chunk, x_chunks, chunk_body, 0)
        for s in range(n_seg):
            out_copy(s).wait()

    return kernel


def _forward(x, mem0, wq, wk, wv, wo, seg_len, q, k, v, shift_k, ssm_k, ssm_d):
    _, seq, d_model = x.shape
    _, n_heads, d_head = wq.shape
    n_mem = mem0.shape[1]
    seg = seg_len
    n_seg = seq // seg
    n_rows = n_mem + seg
    n_cb = d_model // CB
    assert seq == SEQ and d_model == 1024 and d_head == 128 and n_rows % 8 == 0
    tf, ti, t2 = _dft_tables()

    any_spec = pl.BlockSpec(memory_space=pl.ANY)
    kv_rows = -(-n_rows // 16) * 16
    scratch = [
        pltpu.VMEM((n_cb, CB, seq), BF16),
        pltpu.VMEM((seq, d_model), BF16),
        pltpu.VMEM((seq, d_model), BF16),
        pltpu.VMEM((n_cb, N1 * SP, CB), U32),
        pltpu.VMEM((8 + seq, CB), F32),
        pltpu.VMEM((2 * N1 * SP, CB), BF16),
        pltpu.VMEM((2 * N1 * SP, CB), BF16),
        pltpu.VMEM((2 * N2 * SZ, CB), BF16),
        pltpu.VMEM((2 * N2 * SZ, CB), BF16),
        pltpu.VMEM((2 * N1 * ST, CB), BF16),
        pltpu.VMEM(tf.shape, U32),
        pltpu.VMEM(ti.shape, U32),
        pltpu.VMEM(t2.shape, U32),
        pltpu.VMEM((4, d_model), BF16),
        pltpu.VMEM((n_cb, CB), BF16),
        pltpu.VMEM((n_mem, d_model), BF16),
        pltpu.VMEM((4, d_model), F32),
        pltpu.VMEM((n_cb, CB), F32),
        pltpu.VMEM((3 * n_heads // 2, d_model, d_head), U32),
        pltpu.VMEM((3 * n_heads // 2 + 6, d_model // 2, d_head), U32),
        pltpu.VMEM((3 * n_heads // 2, d_model // 2, d_head), U32),
        pltpu.VMEM((d_model // 128, n_heads * d_head // 2, 128), U32),
        pltpu.VMEM((seq, d_model), BF16),
        pltpu.VMEM((seq, d_model), BF16),
        pltpu.VMEM((n_seg, seg, 2 * d_model), BF16),
        pltpu.VMEM((n_rows, d_model), F32),
        pltpu.VMEM((n_heads, n_rows, d_head), F32),
        pltpu.VMEM((n_heads, kv_rows, d_head), BF16),
        pltpu.VMEM((n_heads, kv_rows, d_head), BF16),
        pltpu.VMEM((n_rows, n_heads * d_head), F32),
        pltpu.VMEM((n_heads, n_rows, d_head), F32),
        pltpu.VMEM((n_heads, n_rows, d_head), F32),
        pltpu.VMEM((d_model // 128, n_rows, 128), F32),
        pltpu.VMEM(((_CFG["n_pre"] + 1) * 8, d_model), BF16),
        pltpu.VMEM(((_CFG["n_pre"] + 1) * 8, d_model), F32),
        pltpu.VMEM((2, n_heads, (_CFG["n_pre"] + 1) * 8, d_head), F32),
        pltpu.SemaphoreType.DMA((3, n_cb)),
        pltpu.SemaphoreType.DMA((6,)),
        pltpu.SemaphoreType.DMA((3,)),
        pltpu.SemaphoreType.DMA((len(_CFG["first_splits"]) + 1,)),
        pltpu.SemaphoreType.DMA((2,)),
        pltpu.SemaphoreType.DMA(()),
        pltpu.SemaphoreType.DMA((n_seg,)),
        pltpu.SemaphoreType.DMA((n_seg,)),
        pltpu.SemaphoreType.DMA(()),
    ]
    out = pl.pallas_call(
        _make_kernel(n_heads, d_head, d_model, n_mem, seg, n_seg),
        out_shape=jax.ShapeDtypeStruct((seq, 2 * d_model), BF16),
        in_specs=[any_spec] * 15,
        out_specs=any_spec,
        scratch_shapes=scratch,
        compiler_params=pltpu.CompilerParams(vmem_limit_bytes=120 * 1024 * 1024),
    )(shift_k.T, ssm_d.reshape(n_cb, CB), mem0.reshape(n_mem, d_model),
      x.reshape(seq, d_model), wq, wk, wv, wo.reshape(n_heads * d_head, d_model),
      q.reshape(seq, d_model), k.reshape(seq, d_model), v.reshape(seq, d_model), ssm_k,
      tf, ti, t2)
    return out.reshape(1, seq, 2 * d_model)


def pallas_concat_heads__memory_aug_recurrent_mem_tr__ssm_conv_h3__prompt_kernel(
        A_x, A_mem0, A_Wq, A_Wk, A_Wv, A_Wo, A_seg_len, B_q, B_k, B_v, B_shift_k, B_ssm_k, B_ssm_D):
    return _forward(A_x, A_mem0, A_Wq, A_Wk, A_Wv, A_Wo, int(A_seg_len), B_q, B_k, B_v,
                    B_shift_k, B_ssm_k, B_ssm_D)
```

```python
import math

import jax
import jax.numpy as jnp
import numpy as np
from jax.experimental import pallas as pl
from jax.experimental.pallas import tpu as pltpu

F32 = jnp.float32
BF16 = jnp.bfloat16
U32 = jnp.uint32

N1, N2 = 32, 64
SEQ = N1 * N2
SP = N2 // 2 + 4
SZ = N1 + 4
ST = N2 + 4
CB = 128


def _dft_tables():
    theta = np.pi / (2 * SEQ)
    lane = np.arange(128)[None, :]
    hi, mid, lo = lane // 64, (lane % 64) // 2, lane % 2
    k1 = np.arange(N1)[:, None]
    fwd = np.zeros((N2 // 4, 2 * N1, 128))
    for g in range(N2 // 4):
        ph = theta * (4 * k1 + 1) * (N2 * mid + 4 * g + 2 * hi + lo)
        fwd[g, 0::2] = np.cos(ph)
        fwd[g, 1::2] = np.sin(ph)
    n1 = np.arange(N1)[:, None]
    inv = np.zeros((N2 // 2, N1, 128))
    for i in range(N2 // 2):
        ph = theta * (4 * mid + 1) * (N2 * n1 + 2 * i + hi)
        inv[i] = np.where(lo == 0, np.cos(ph), np.sin(ph)) / SEQ
    ph = 2 * np.pi * np.arange(N2)[:, None] * np.arange(N2)[None, :] / N2
    c, s = np.cos(ph), np.sin(ph)
    f2 = np.zeros((128, 128))
    f2[:N2, 0::2], f2[:N2, 1::2], f2[N2:, 0::2], f2[N2:, 1::2] = c, -s, s, c
    g2 = np.zeros((128, 128))
    g2[0::2, :N2], g2[0::2, N2:], g2[1::2, :N2], g2[1::2, N2:] = c.T, s.T, -s.T, c.T

    def as_words(a):
        u = a.astype(np.float32).astype(BF16).view(np.uint16).astype(np.uint32)
        return u[..., 0::2, :] | (u[..., 1::2, :] << 16)

    inv = np.repeat(inv, 2, axis=1)
    return as_words(fwd), as_words(inv), as_words(np.stack([f2, g2]))


def _to_words(x):
    return pltpu.bitcast(x.astype(BF16), U32)


def _from_words(w):
    return pltpu.bitcast(w, BF16)


_CFG = dict(
    group=8, lag_s=2, lag_v=3, wo_split=16, gate_at=1,
    first_splits=(16,),
    unroll=3,
    chunk_steps=3,
    n_pre=18,
    n_early=2,
    late_per_block=10,
    b_group=8,
)


def _step_order(n_heads, n_out_tiles, first=False):
    g, a, b = _CFG["group"], _CFG["lag_s"], _CFG["lag_v"]
    split = _CFG["wo_split"]
    n_groups = n_heads // g
    total = n_groups + a + b
    early = [("W", j, 0, split) for j in range(n_out_tiles)] if split < n_heads else []
    ops = []
    for t in range(total):
        if t < n_groups:
            ops += [("P", h) for h in range(t * g, (t + 1) * g)]
        if t == _CFG["gate_at"]:
            ops.append(("G",))
        if 0 <= t - a < n_groups:
            ops += [("S", h) for h in range((t - a) * g, (t - a + 1) * g)]
        if 0 <= t - a - b < n_groups:
            ops += [("V", h) for h in range((t - a - b) * g, (t - a - b + 1) * g)]
        if early and (t - a - b + 1) * g >= split:
            n = -(-len(early) // (total - t))
            ops += early[:n]
            early = early[n:]
    ops += early
    bounds = [split if split < n_heads else 0]
    if first:
        bounds += [b for b in _CFG["first_splits"] if b > split]
    for lo, hi in zip(bounds, bounds[1:] + [n_heads]):
        ops += [("W", j, lo, hi) for j in range(n_out_tiles)]
    return ops


def _dot(a, b):
    return jnp.dot(a, b, preferred_element_type=F32)


def _dot_nt(a, b):
    return jax.lax.dot_general(a, b, (((1,), (1,)), ((), ())), preferred_element_type=F32)


def _make_kernel(n_heads, d_head, d_model, n_mem, seg, n_seg):
    n_rows = n_mem + seg
    n_cb = d_model // CB
    n_hp = n_heads // 2
    scale = d_head ** (-0.5)
    exp_scale = scale * math.log2(math.e)
    steps_per_chunk = _CFG["chunk_steps"]
    x_chunks = (n_seg - 1) // steps_per_chunk
    x_rows = steps_per_chunk * seg
    assert x_chunks * steps_per_chunk == n_seg - 1 and steps_per_chunk % _CFG["unroll"] == 0
    n_pre = _CFG["n_pre"]
    pre_rows = 8
    assert n_pre % steps_per_chunk == 0
    order = _step_order(n_heads, d_model // 128)
    order_first = _step_order(n_heads, d_model // 128, True)
    wo_bounds = [0] + list(_CFG["first_splits"]) + [n_heads]

    def kernel(sh_hbm, d_hbm, mem_hbm,
               x_hbm, wq_hbm, wk_hbm, wv_hbm, wo_hbm,
               q_hbm, k_hbm, v_hbm, h_hbm, tf_hbm, ti_hbm, t2_hbm,
               out_hbm,
               hs, ks, vs, ob, kf, xp, hp, zx, zh, tt, tf, ti, t2, sh_ref, d_ref, mem_ref, sh32, d32,
               stage, w_even, w_odd, wo, xin, qin, ost, hbuf, qbuf, kbuf, vbuf, obuf, pbuf, ibuf, ybuf, xpre, xpre32, qkpre,
               sem_b, sem_t, sem_w, sem_o, sem_h, sem_p, sem_x, sem_q, sem_out):

        n_early = _CFG["n_early"]

        def h_copy(cb):
            c0 = cb * CB if isinstance(cb, int) else pl.multiple_of(cb * CB, CB)
            return pltpu.make_async_copy(h_hbm.at[pl.ds(c0, CB), :], hs.at[cb], sem_b.at[0, cb])

        def kv_copies(cb):
            if isinstance(cb, int):
                c0, width = cb * CB, (CB if cb < n_early else d_model - n_early * CB)
            else:
                c0, width = pl.multiple_of(cb * CB, CB), CB
            return [pltpu.make_async_copy(src.at[:, pl.ds(c0, width)], dst.at[:, pl.ds(c0, width)], sem_b.at[1 + i, cb])
                    for i, (src, dst) in enumerate(((k_hbm, ks), (v_hbm, vs)))]

        def t_copies():
            pairs = ((sh_hbm, sh_ref), (d_hbm, d_ref), (mem_hbm, mem_ref),
                     (tf_hbm, tf), (ti_hbm, ti), (t2_hbm, t2))
            return [pltpu.make_async_copy(src, dst, sem_t.at[i]) for i, (src, dst) in enumerate(pairs)]

        def w_copies(m):
            w32 = (wq_hbm, wk_hbm, wv_hbm)[m].bitcast(U32)
            return [pltpu.make_async_copy(w32.at[:, hp, :], stage.at[m * n_hp + hp, pl.ds(0, d_model), :], sem_w.at[m])
                    for hp in range(n_hp)]

        def o_copies(i):
            wo32 = wo_hbm.bitcast(U32)
            lo, hi = wo_bounds[i] * d_head // 2, wo_bounds[i + 1] * d_head // 2
            return [pltpu.make_async_copy(wo32.at[pl.ds(lo, hi - lo), pl.ds(j * 128, 128)],
                                          wo.at[j, pl.ds(lo, hi - lo), :], sem_o.at[i])
                    for j in range(d_model // 128)]

        def head_copies():
            return [pltpu.make_async_copy(src.at[pl.ds(0, seg), :], dst.at[pl.ds(0, seg), :], sem_h.at[i])
                    for i, (src, dst) in enumerate(((x_hbm, xin), (q_hbm, qin)))]

        def pre_copies():
            return [pltpu.make_async_copy(x_hbm.at[pl.ds(i * seg, pre_rows), :],
                                          xpre.at[pl.ds(i * pre_rows, pre_rows), :], sem_p) for i in range(n_pre + 1)]

        def chunk_copies(c):
            r0 = seg + c * x_rows if isinstance(c, int) else pl.multiple_of(seg + c * x_rows, seg)
            return [pltpu.make_async_copy(src.at[pl.ds(r0, x_rows), :], dst.at[pl.ds(r0, x_rows), :], sem.at[c])
                    for src, dst, sem in ((x_hbm, xin, sem_x), (q_hbm, qin, sem_q))]

        def out_copy(s):
            r0 = s * seg if isinstance(s, int) else pl.multiple_of(s * seg, seg)
            return pltpu.make_async_copy(ost.at[s], out_hbm.at[pl.ds(r0, seg), :], sem_out)

        tc = t_copies()
        for c in tc[:3] + kv_copies(0) + [h_copy(0)] + tc[3:]:
            c.start()
        for cb in range(1, n_early):
            for c in [h_copy(cb)] + kv_copies(cb):
                c.start()
        late = kv_copies(n_early) + [h_copy(cb) for cb in range(n_early, n_cb)]
        n_b_late = len(late)
        late += w_copies(0) + pre_copies() + w_copies(1) + w_copies(2) + head_copies()
        for i in range(len(wo_bounds) - 1):
            late += o_copies(i)
        per_block = _CFG["late_per_block"]

        kf[0:8, :] = jnp.zeros((8, CB), F32)

        group = _CFG["b_group"]

        def put(ref, row, x):
            ref[pl.ds(2 * row, x.shape[0]), :] = x.astype(BF16)

        def get(ref, row, n, stride=1):
            return ref.bitcast(U32)[pl.ds(row, n, stride=stride), :]

        def wait_inputs(cb):
            h_copy(cb).wait()

            @pl.when(cb < n_early)
            def _():
                for c in kv_copies(cb):
                    c.wait()

            @pl.when(cb == n_early)
            def _():
                for c in kv_copies(n_early):
                    c.wait()

        def prepare(cb):
            c0 = pl.multiple_of(cb * CB, CB)
            kf[8:8 + SEQ, :] = ks[:, pl.ds(c0, CB)].astype(F32)
            for j in range(SEQ // 128):
                r = hs[cb, :, j * 128:(j + 1) * 128].astype(F32).T
                put(hp, (2 * j) * SP, r[0:N2])
                put(hp, (2 * j + 1) * SP, r[N2:2 * N2])
            taps = sh32[:, pl.ds(c0, CB)]
            for n1 in range(N1):
                acc = kf[pl.ds(8 + n1 * N2, N2), :] * taps[0:1]
                for i in range(1, 4):
                    acc = acc + kf[pl.ds(8 - i + n1 * N2, N2), :] * taps[i:i + 1]
                put(xp, n1 * SP, acc * vs[pl.ds(n1 * N2, N2), pl.ds(c0, CB)].astype(F32))

        def b_block(cb, carry):
            wait_inputs(cb)
            for i in range(n_cb):
                @pl.when(cb == i)
                def _(i=i):
                    lo = 0 if i == 0 else n_b_late + i * per_block
                    for c in late[lo:n_b_late + (i + 1) * per_block]:
                        c.start()
            lane = jax.lax.broadcasted_iota(jnp.int32, (1, 128), 1)
            prepare(cb)
            for g in range(N2 // 4):
                m = tf[g]
                lhs = _from_words(jnp.concatenate(
                    [jnp.where((lane // 64 == j // 2) & (lane % 2 == j % 2), m, jnp.zeros_like(m))
                     for j in range(4)], axis=0))

                def rhs(ref, g=g):
                    return _from_words(jnp.concatenate(
                        [get(ref, 2 * g, N1, SP), get(ref, 2 * g + 1, N1, SP)], axis=0))

                r = _dot(lhs, jnp.concatenate([rhs(xp), rhs(hp)], axis=1))
                for j in range(4):
                    put(zx, (4 * g + j) * SZ, r[2 * N1 * j:2 * N1 * (j + 1), :128])
                    put(zh, (4 * g + j) * SZ, r[2 * N1 * j:2 * N1 * (j + 1), 128:])
            f2 = _from_words(t2[0])
            g2 = _from_words(t2[1])

            def stage2(g):
                zz = []
                for k1 in range(g * group, (g + 1) * group):
                    zz += [_from_words(get(zx, k1, N2, SZ)), _from_words(get(zh, k1, N2, SZ))]
                return _dot(f2, jnp.concatenate(zz, axis=1))

            def stage3(g, r):
                ys = []
                for i in range(group):
                    xf = r[:, (2 * i) * 128:(2 * i + 1) * 128]
                    hf = r[:, (2 * i + 1) * 128:(2 * i + 2) * 128]
                    xr, xi, hr, hi = xf[:N2], xf[N2:], hf[:N2], hf[N2:]
                    ys.append(jnp.concatenate([xr * hr - xi * hi, xr * hi + xi * hr], axis=0).astype(BF16))
                t = _dot(g2, jnp.concatenate(ys, axis=1))
                for i in range(group):
                    put(tt, (g * group + i) * ST, t[:, i * 128:(i + 1) * 128])

            n_groups = N1 // group
            r = stage2(0)
            for g in range(n_groups):
                r_next = stage2(g + 1) if g + 1 < n_groups else None
                stage3(g, r)
                r = r_next
            half_mask = jnp.where(lane < 64, U32(0x0000FFFF), U32(0xFFFF0000))
            dv = d32[pl.ds(cb, 1), :]
            for i in range(N2 // 2):
                y = _dot(_from_words(ti[i] & half_mask), _from_words(jnp.concatenate(
                    [get(tt, 2 * i, N1, ST), get(tt, 2 * i + 1, N1, ST)], axis=0)))
                kv = _from_words(get(xp, i, N1, SP)).astype(F32)
                ob[cb, pl.ds(i, N1, stride=SP), :] = _to_words(y + kv * dv)
            return carry

        for c in tc:
            c.wait()
        sh32[...] = sh_ref[...].astype(F32)
        d32[...] = d_ref[...].astype(F32)
        hbuf[0:n_mem, :] = mem_ref[...].astype(F32)
        jax.lax.fori_loop(0, n_cb, b_block, 0)
        for c in late[n_b_late + n_cb * per_block:]:
            c.start()

        def w_slot(quad, parity, odd_head, m):
            return (w_even, w_odd)[parity], (2 * quad + odd_head) * 3 + m

        def wtile(h, m):
            ref, i = w_slot(h // 4, (h // 2) % 2, h % 2, m)
            return _from_words(ref[i])

        def relayout(m, quad, parity):
            pair = 2 * quad + parity
            if not isinstance(pair, int):
                pair = jnp.minimum(pair, n_hp - 1)
            src = m * n_hp + pair
            even = stage[src, pl.ds(0, d_model // 2, stride=2), :]
            odd = stage[src, pl.ds(1, d_model // 2, stride=2), :]
            ref, i = w_slot(quad, parity, 0, m)
            ref[i] = (even & U32(0xFFFF)) | (odd << 16)
            ref, i = w_slot(quad, parity, 1, m)
            ref[i] = (even >> 16) | (odd & U32(0xFFFF0000))

        for m in range(2):
            for c in w_copies(m):
                c.wait()
        for c in pre_copies():
            c.wait()
        xpre32[...] = xpre[...].astype(F32)
        relayout(0, 0, 0)
        relayout(1, 0, 0)

        def pre_dots(quad, parity, xl):
            for odd_head in range(2):
                for m in range(2):
                    ref, i = w_slot(quad, parity, odd_head, m)
                    qkpre[m, 4 * quad + 2 * parity + odd_head] = _dot(xl, _from_words(ref[i]))

        def pre_round(quad, carry):
            xl = xpre32[...]
            pre_dots(quad, 0, xl)
            relayout(0, quad, 1)
            relayout(1, quad, 1)
            pre_dots(quad, 1, xl)
            relayout(0, quad + 1, 0)
            relayout(1, quad + 1, 0)
            return carry

        jax.lax.fori_loop(0, n_heads // 4, pre_round, 0)
        for c in w_copies(2):
            c.wait()

        def step(s, first, pre=False):
            if first:
                for c in head_copies():
                    c.wait()
            row = jax.lax.broadcasted_iota(jnp.int32, (n_rows, n_rows), 0)
            col = jax.lax.broadcasted_iota(jnp.int32, (n_rows, n_rows), 1)
            mask = (row < n_mem) | (row >= col)
            r0 = s * seg if first else pl.multiple_of(s * seg, seg)
            slot = s
            y0 = (s * seg // N2) * SP + (s * seg % N2) // 2
            if not first:
                y0 = pl.multiple_of(y0, 4)
            hbuf[n_mem:n_rows, :] = xin[pl.ds(r0, seg), :].astype(F32)
            hl = hbuf[...]
            if pre:
                hr = jnp.concatenate([hl[0:n_mem], hl[n_mem + pre_rows:n_rows]], axis=0)
                p0 = s * pre_rows if first else pl.multiple_of(s * pre_rows, pre_rows)
            waited = [False] * (len(wo_bounds) - 1)
            for op in (order_first if first else order):
                if op[0] == "P":
                    h = op[1]
                    if first and h % 2 == 0:
                        if h == 0:
                            relayout(2, 0, 0)
                        if h + 2 < n_heads:
                            relayout(2, (h + 2) // 4, (h // 2 + 1) % 2)
                    if pre:
                        rq = _dot(hr, wtile(h, 0))
                        qbuf[h] = jnp.concatenate(
                            [rq[0:n_mem], qkpre[0, h, pl.ds(p0, pre_rows), :], rq[n_mem:]], axis=0)
                        rk = _dot(hr, wtile(h, 1))
                        kbuf[h, 0:n_rows] = jnp.concatenate(
                            [rk[0:n_mem], qkpre[1, h, pl.ds(p0, pre_rows), :], rk[n_mem:]], axis=0).astype(BF16)
                    else:
                        qbuf[h] = _dot(hl, wtile(h, 0))
                        kbuf[h, 0:n_rows] = _dot(hl, wtile(h, 1)).astype(BF16)
                    vbuf[h, 0:n_rows] = _dot(hl, wtile(h, 2)).astype(BF16)
                elif op[0] == "S":
                    h = op[1]
                    sc = _dot_nt(qbuf[h], kbuf[h, 0:n_rows])
                    sc = jnp.where(mask, sc, -1e9 / scale)
                    e = jnp.exp2((sc - jnp.max(sc, axis=-1, keepdims=True)) * exp_scale)
                    den = jnp.sum(e, axis=-1, keepdims=True)
                    inv = pl.reciprocal(den, approx=True)
                    pbuf[h, :, 0:n_rows] = e
                    ibuf[h] = jnp.broadcast_to(inv * (2.0 - den * inv), (n_rows, d_head))
                elif op[0] == "V":
                    h = op[1]
                    obuf[:, h * d_head:(h + 1) * d_head] = (
                        _dot(pbuf[h, :, 0:n_rows], vbuf[h, 0:n_rows]) * ibuf[h])
                elif op[0] == "W":
                    _, j, lo, hi = op
                    if first:
                        for i in range(len(waited)):
                            if not waited[i] and hi > wo_bounds[i]:
                                for c in o_copies(i):
                                    c.wait()
                                waited[i] = True
                                if i == len(waited) - 1:
                                    for ch in range(x_chunks):
                                        for c in chunk_copies(ch):
                                            c.start()
                    w = _from_words(wo[j, lo * d_head // 2:hi * d_head // 2, :])
                    y = _dot(obuf[:, lo * d_head:hi * d_head], w)
                    if lo > 0:
                        y = y + ybuf[j]
                    if hi < n_heads:
                        ybuf[j] = y
                    else:
                        hbuf[0:n_mem, j * 128:(j + 1) * 128] = y[0:n_mem]
                        ost[slot, :, j * 128:(j + 1) * 128] = y[n_mem:n_rows].astype(BF16)
                else:
                    for cb in range(n_cb):
                        gate = qin[pl.ds(r0, seg), cb * CB:(cb + 1) * CB].astype(F32)
                        ost[slot, :, d_model + cb * CB:d_model + (cb + 1) * CB] = (
                            _from_words(ob[cb, pl.ds(y0, seg // 2), :]).astype(F32) * gate).astype(BF16)
            out_copy(s).start()

        unroll = _CFG["unroll"]

        def pre_step(s, carry):
            @pl.when((s - 1) % steps_per_chunk == 0)
            def _():
                for cp in chunk_copies((s - 1) // steps_per_chunk):
                    cp.wait()

            step(s, False, True)
            return carry

        def chunk_body(c, carry):
            for cp in chunk_copies(c):
                cp.wait()

            def steps_body(i, carry):
                for u in range(unroll):
                    step(1 + c * steps_per_chunk + i * unroll + u, False)
                return carry

            if steps_per_chunk == unroll:
                steps_body(0, 0)
            else:
                jax.lax.fori_loop(0, steps_per_chunk // unroll, steps_body, 0)
            return carry

        step(0, True, True)
        jax.lax.fori_loop(1, 1 + n_pre, pre_step, 0)
        jax.lax.fori_loop(n_pre // steps_per_chunk, x_chunks, chunk_body, 0)
        pltpu.make_async_copy(ost, ost, sem_out).wait()

    return kernel


def _forward(x, mem0, wq, wk, wv, wo, seg_len, q, k, v, shift_k, ssm_k, ssm_d):
    _, seq, d_model = x.shape
    _, n_heads, d_head = wq.shape
    n_mem = mem0.shape[1]
    seg = seg_len
    n_seg = seq // seg
    n_rows = n_mem + seg
    n_cb = d_model // CB
    assert seq == SEQ and d_model == 1024 and d_head == 128 and n_rows % 8 == 0
    tf, ti, t2 = _dft_tables()

    any_spec = pl.BlockSpec(memory_space=pl.ANY)
    kv_rows = -(-n_rows // 16) * 16
    scratch = [
        pltpu.VMEM((n_cb, CB, seq), BF16),
        pltpu.VMEM((seq, d_model), BF16),
        pltpu.VMEM((seq, d_model), BF16),
        pltpu.VMEM((n_cb, N1 * SP + 64, CB), U32),
        pltpu.VMEM((8 + seq, CB), F32),
        pltpu.VMEM((2 * (N1 * SP + 64), CB), BF16),
        pltpu.VMEM((2 * (N1 * SP + 64), CB), BF16),
        pltpu.VMEM((2 * (N2 * SZ + 64), CB), BF16),
        pltpu.VMEM((2 * (N2 * SZ + 64), CB), BF16),
        pltpu.VMEM((2 * (N1 * ST + 96), CB), BF16),
        pltpu.VMEM(tf.shape, U32),
        pltpu.VMEM(ti.shape, U32),
        pltpu.VMEM(t2.shape, U32),
        pltpu.VMEM((4, d_model), BF16),
        pltpu.VMEM((n_cb, CB), BF16),
        pltpu.VMEM((n_mem, d_model), BF16),
        pltpu.VMEM((4, d_model), F32),
        pltpu.VMEM((n_cb, CB), F32),
        pltpu.VMEM((3 * n_heads // 2, d_model + 8, d_head), U32),
        pltpu.VMEM((3 * n_heads // 2 + 6, d_model // 2, d_head), U32),
        pltpu.VMEM((3 * n_heads // 2, d_model // 2, d_head), U32),
        pltpu.VMEM((d_model // 128, n_heads * d_head // 2, 128), U32),
        pltpu.VMEM((seq, d_model), BF16),
        pltpu.VMEM((seq, d_model), BF16),
        pltpu.VMEM((n_seg, seg, 2 * d_model), BF16),
        pltpu.VMEM((n_rows, d_model), F32),
        pltpu.VMEM((n_heads, n_rows, d_head), F32),
        pltpu.VMEM((n_heads, kv_rows, d_head), BF16),
        pltpu.VMEM((n_heads, kv_rows, d_head), BF16),
        pltpu.VMEM((n_rows, n_heads * d_head), F32),
        pltpu.VMEM((n_heads, n_rows, d_head), F32),
        pltpu.VMEM((n_heads, n_rows, d_head), F32),
        pltpu.VMEM((d_model // 128, n_rows, 128), F32),
        pltpu.VMEM(((_CFG["n_pre"] + 1) * 8, d_model), BF16),
        pltpu.VMEM(((_CFG["n_pre"] + 1) * 8, d_model), F32),
        pltpu.VMEM((2, n_heads, (_CFG["n_pre"] + 1) * 8, d_head), F32),
        pltpu.SemaphoreType.DMA((3, n_cb)),
        pltpu.SemaphoreType.DMA((6,)),
        pltpu.SemaphoreType.DMA((3,)),
        pltpu.SemaphoreType.DMA((len(_CFG["first_splits"]) + 1,)),
        pltpu.SemaphoreType.DMA((2,)),
        pltpu.SemaphoreType.DMA(()),
        pltpu.SemaphoreType.DMA((n_seg,)),
        pltpu.SemaphoreType.DMA((n_seg,)),
        pltpu.SemaphoreType.DMA(()),
    ]
    out = pl.pallas_call(
        _make_kernel(n_heads, d_head, d_model, n_mem, seg, n_seg),
        out_shape=jax.ShapeDtypeStruct((seq, 2 * d_model), BF16),
        in_specs=[any_spec] * 15,
        out_specs=any_spec,
        scratch_shapes=scratch,
        compiler_params=pltpu.CompilerParams(vmem_limit_bytes=120 * 1024 * 1024),
    )(shift_k.T, ssm_d.reshape(n_cb, CB), mem0.reshape(n_mem, d_model),
      x.reshape(seq, d_model), wq, wk, wv, wo.reshape(n_heads * d_head, d_model),
      q.reshape(seq, d_model), k.reshape(seq, d_model), v.reshape(seq, d_model), ssm_k,
      tf, ti, t2)
    return out.reshape(1, seq, 2 * d_model)


def pallas_concat_heads__memory_aug_recurrent_mem_tr__ssm_conv_h3__prompt_kernel(
        A_x, A_mem0, A_Wq, A_Wk, A_Wv, A_Wo, A_seg_len, B_q, B_k, B_v, B_shift_k, B_ssm_k, B_ssm_D):
    return _forward(A_x, A_mem0, A_Wq, A_Wk, A_Wv, A_Wo, int(A_seg_len), B_q, B_k, B_v,
                    B_shift_k, B_ssm_k, B_ssm_D)
```
